```python
import jax
import jax.numpy as jnp

def _softmax(x, axis=-1):
    return jax.nn.softmax(x, axis=axis)

def _gelu(x):
    return jax.nn.gelu(x, approximate=True)

def _silu(x):
    return jax.nn.silu(x)

def _sigmoid(x):
    return jax.nn.sigmoid(x)

def _layernorm(x, axis=-1, eps=1e-05):
    m = jnp.mean(x, axis=axis, keepdims=True)
    v = jnp.var(x, axis=axis, keepdims=True)
    return (x - m) / jnp.sqrt(v + eps)

def _scatter_add(tgt, idx, src, axis=0):
    return tgt.at[idx].add(src)

def _segment_sum(src, seg, n):
    return jax.ops.segment_sum(src, seg, n)

class _Rng:

    def __init__(self, key):
        self._k = key

    def _next(self):
        self._k, sub = jax.random.split(self._k)
        return sub

    def normal(self, shape):
        return jax.random.normal(self._next(), shape, dtype=jnp.bfloat16)

    def randint(self, lo, hi, shape):
        return jax.random.randint(self._next(), shape, lo, hi, dtype=jnp.int32)

    def uniform(self, shape, lo=0.0, hi=1.0):
        return jax.random.uniform(self._next(), shape, jnp.bfloat16, lo, hi)

    def permutation(self, n):
        return jax.random.permutation(self._next(), n)
kernel_name = 'interleave_layers__memory_aug_recurrent_mem_tr__glu_gated_glu__prompt'

def setup_inputs():
    _rng = _Rng(jax.random.key(int.from_bytes(__import__("os").urandom(4), "little")))
    _w = lambda a: (lambda t: t.astype(jnp.bfloat16) if jnp.issubdtype(t.dtype, jnp.floating) else t)(jnp.asarray(a))

    def _A_setup():
        B, S, Dm = (1, 2048, 1024)
        H, Dh = (32, 128)
        M, seg = (8, 32)
        seg = min(seg, S)
        S = S // seg * seg
        return {'x': _w((lambda *s: _rng.normal(s) * 0.05)(B, S, Dm)), 'mem0': _w((lambda *s: _rng.normal(s) * 0.05)(B, M, Dm)), 'Wq': _w((lambda *s: _rng.normal(s) * 0.05)(Dm, H, Dh) * Dm ** (-0.5)), 'Wk': _w((lambda *s: _rng.normal(s) * 0.05)(Dm, H, Dh) * Dm ** (-0.5)), 'Wv': _w((lambda *s: _rng.normal(s) * 0.05)(Dm, H, Dh) * Dm ** (-0.5)), 'Wo': _w((lambda *s: _rng.normal(s) * 0.05)(H, Dh, Dm) * (H * Dh) ** (-0.5)), 'seg_len': seg}
    _A_in = _A_setup()

    def _B_setup():
        B, S, D, F = (1, 2048, 1024, 3584)
        return {'x': _w((lambda *s: _rng.normal(s) * 0.05)(B, S, D)), 'w_gate': _w((lambda *s: _rng.normal(s) * 0.05)(D, F)), 'w_up': _w((lambda *s: _rng.normal(s) * 0.05)(D, F)), 'w_down': _w((lambda *s: _rng.normal(s) * 0.05)(F, D))}
    _B_in = _B_setup()
    return {'A_x': _A_in['x'], 'A_mem0': _A_in['mem0'], 'A_Wq': _A_in['Wq'], 'A_Wk': _A_in['Wk'], 'A_Wv': _A_in['Wv'], 'A_Wo': _A_in['Wo'], 'A_seg_len': _A_in['seg_len'], 'B_x': _B_in['x'], 'B_w_gate': _B_in['w_gate'], 'B_w_up': _B_in['w_up'], 'B_w_down': _B_in['w_down']}

def reference(A_x, A_mem0, A_Wq, A_Wk, A_Wv, A_Wo, A_seg_len, B_x, B_w_gate, B_w_up, B_w_down):

    def _A_ref(x, mem0, Wq, Wk, Wv, Wo, seg_len):
        B, S, Dm = x.shape
        H, Dh = (Wq.shape[1], Wq.shape[2])
        M = mem0.shape[1]
        scale = Dh ** (-0.5)
        n_seg = S // seg_len
        L = M + seg_len
        idx = jnp.arange(L)
        mask = (idx[:, None] < M) | (idx[:, None] >= idx[None, :])
        mem = mem0
        outs = []
        for s in range(n_seg):
            xs = x[:, s * seg_len:(s + 1) * seg_len, :].copy()
            h = jnp.concatenate([mem, xs], axis=1)
            q = jnp.einsum('btd,dhe->bhte', h, Wq)
            k = jnp.einsum('btd,dhe->bhte', h, Wk)
            v = jnp.einsum('btd,dhe->bhte', h, Wv)
            scores = jnp.einsum('bhqe,bhke->bhqk', q, k) * scale
            scores = jnp.where(mask[None, None], scores, -1000000000.0)
            p = _softmax(scores, axis=-1)
            o = jnp.einsum('bhqk,bhke->bhqe', p, v)
            o = jnp.einsum('bhte,hed->btd', o, Wo)
            mem = o[:, :M, :].copy()
            outs.append(o[:, M:, :])
        return jnp.concatenate(outs, axis=1)

    def _B_ref(x, w_gate, w_up, w_down):
        g = jnp.einsum('bsd,df->bsf', x, w_gate)
        u = jnp.einsum('bsd,df->bsf', x, w_up)
        h = _sigmoid(g) * u
        return jnp.einsum('bsf,fd->bsd', h, w_down)
    x = A_x
    x = x + _A_ref(_layernorm(x, axis=-1), A_mem0, A_Wq, A_Wk, A_Wv, A_Wo, A_seg_len)
    x = x + _B_ref(_layernorm(x, axis=-1), B_w_gate, B_w_up, B_w_down)
    x = x + _A_ref(_layernorm(x, axis=-1), A_mem0, A_Wq, A_Wk, A_Wv, A_Wo, A_seg_len)
    x = x + _B_ref(_layernorm(x, axis=-1), B_w_gate, B_w_up, B_w_down)
    return x
```

```python
import functools

import jax
import jax.numpy as jnp
from jax import lax
import jax.experimental.pallas as pl
import jax.experimental.pallas.tpu as pltpu

F32 = jnp.float32
BF16 = jnp.bfloat16
LAG = 2
HEAD_GROUP = 4
FF_CHUNK = 512
RAW_CHUNK = 128


def _layernorm(x):
    m = jnp.mean(x, axis=-1, keepdims=True)
    d = x - m
    v = jnp.mean(d * d, axis=-1, keepdims=True)
    return d * lax.rsqrt(v + 1e-5)


def _dot(a, b):
    return jnp.dot(a, b, preferred_element_type=F32)


def _kernel(x_hbm, mem0_ref, wq_hbm, wk_hbm, wv_hbm, wo_hbm, wg_hbm, wu_hbm, wd_hbm,
            out_hbm,
            x_v, out_v, raw, wqkv, wo, wg, wu, wd,
            h_in, xa, attn, xb, hb, act, dacc, bias,
            sem_x, sem_raw, sem_w, sem_out, *, seg):
    S, D = x_v.shape
    M = mem0_ref.shape[0]
    H, Dh = wq_hbm.shape[1], wq_hbm.shape[2]
    F = wg.shape[1]
    n_seg = S // seg
    R = 2 * (M + seg)
    G = HEAD_GROUP
    scale = Dh ** -0.5
    n_raw = D // RAW_CHUNK

    x_copy = pltpu.make_async_copy(x_hbm, x_v, sem_x)
    x_copy.start()

    def raw_copy(c, i):
        src = (wq_hbm, wk_hbm, wv_hbm)[i]
        rows = pl.ds(c * RAW_CHUNK, RAW_CHUNK)
        return pltpu.make_async_copy(src.at[rows], raw.at[i, rows], sem_raw.at[i, c])

    for c in range(n_raw):
        for i in range(3):
            raw_copy(c, i).start()
    w_copies = [pltpu.make_async_copy(s, d, sem_w.at[i]) for i, (s, d) in enumerate(
        ((wo_hbm, wo), (wg_hbm, wg), (wu_hbm, wu), (wd_hbm, wd)))]
    for cp in w_copies:
        cp.start()

    r = lax.broadcasted_iota(jnp.int32, (R, R), 0)
    c = lax.broadcasted_iota(jnp.int32, (R, R), 1)

    def second(i):
        return ((i >= M) & (i < 2 * M)) | (i >= 2 * M + seg)

    visible = (r < 2 * M) | (r >= c)
    bias[...] = jnp.where(second(r) == second(c),
                          jnp.where(visible, 0.0, -1e9), -jnp.inf).astype(F32)

    raw32 = raw.bitcast(jnp.uint32)

    def relayout(c, carry):
        base = pl.multiple_of(c * RAW_CHUNK, RAW_CHUNK)
        for i in range(3):
            raw_copy(c, i).wait()
            for j in range(H // 2):
                even = raw32[i, pl.ds(base, RAW_CHUNK // 2, stride=2), j, :]
                odd = raw32[i, pl.ds(base + 1, RAW_CHUNK // 2, stride=2), j, :]
                lo = (even & 0xFFFF) | (odd << 16)
                hi = (even >> 16) | (odd & jnp.uint32(0xFFFF0000))
                for head, word in ((2 * j, lo), (2 * j + 1, hi)):
                    col = (i * G + head % G) * Dh
                    wqkv[head // G, pl.ds(base, RAW_CHUNK), col:col + Dh] = (
                        pltpu.bitcast(word, BF16))
        return carry

    lax.fori_loop(0, n_raw, relayout, 0)

    x_copy.wait()
    mem0 = mem0_ref[...].astype(F32)

    def load_segment(s):
        rows = pl.ds(pl.multiple_of(s * seg, seg), seg)
        xs = x_v[rows, :].astype(F32)
        xa[0:seg, :] = xs
        h_in[2 * M:2 * M + seg, :] = _layernorm(xs).astype(BF16)

    h_in[0:2 * M, :] = jnp.concatenate([mem0, mem0], axis=0).astype(BF16)
    h_in[2 * M + seg:R, :] = jnp.zeros((seg, D), BF16)
    xa[seg:2 * seg, :] = jnp.zeros((seg, D), F32)
    xb[...] = jnp.zeros(xb.shape, F32)
    act[...] = jnp.zeros(act.shape, BF16)
    load_segment(0)
    for cp in w_copies:
        cp.wait()

    def project(g):
        return _dot(h_in[...], wqkv[g]).astype(BF16)

    def attend(g, qkv):
        for i in range(G):
            q = qkv[:, i * Dh:(i + 1) * Dh]
            k = qkv[:, (G + i) * Dh:(G + i + 1) * Dh]
            v = qkv[:, (2 * G + i) * Dh:(2 * G + i + 1) * Dh]
            s = lax.dot_general(q, k, (((1,), (1,)), ((), ())),
                                preferred_element_type=F32)
            b = bias[...]
            s = jnp.where(b == 0.0, s * scale, b)
            e = jnp.exp(s - jnp.max(s, axis=-1, keepdims=True))
            p = e * (1.0 / jnp.sum(e, axis=-1, keepdims=True))
            head = g * G + i
            attn[:, head * Dh:(head + 1) * Dh] = _dot(p.astype(BF16), v).astype(BF16)

    def attention():
        n_groups = H // G
        qkv = project(0)
        for g in range(n_groups):
            nxt = project(g + 1) if g + 1 < n_groups else None
            attend(g, qkv)
            qkv = nxt

    def down_first():
        dacc[...] = xb[...] + _dot(act[:, :F // 2], wd[:F // 2, :])

    def down_second():
        return dacc[...] + _dot(act[:, F // 2:], wd[F // 2:, :])

    def out_proj(t):
        o = _dot(attn[...], wo[...])
        mem2 = jnp.where(t < LAG, mem0, o[M:2 * M])
        h_in[0:2 * M, :] = jnp.concatenate([o[0:M], mem2], axis=0).astype(BF16)
        x1 = xa[...] + o[2 * M:]
        xb[...] = x1
        hb[...] = _layernorm(x1).astype(BF16)

    def gate_up():
        for f in range(0, F, FF_CHUNK):
            g = _dot(hb[...], wg[:, f:f + FF_CHUNK])
            u = _dot(hb[...], wu[:, f:f + FF_CHUNK])
            act[:, f:f + FF_CHUNK] = (jax.nn.sigmoid(g) * u).astype(BF16)

    def out_copy(s):
        rows = pl.ds(pl.multiple_of(s * seg, seg), seg)
        return pltpu.make_async_copy(out_v.at[rows], out_hbm.at[rows], sem_out)

    def step(t, carry):
        @pl.when(t >= LAG + 2)
        def _():
            out_copy(t - LAG - 2).start()

        attention()
        down_first()
        out_proj(t)
        x2 = down_second()
        xa[seg:2 * seg, :] = x2[0:seg]
        h_in[2 * M + seg:R, :] = _layernorm(x2[0:seg]).astype(BF16)
        done = jnp.maximum(t - LAG - 1, 0)
        out_v[pl.ds(pl.multiple_of(done * seg, seg), seg), :] = x2[seg:].astype(out_v.dtype)
        load_segment(jnp.minimum(t + 1, n_seg - 1))
        gate_up()
        return carry

    lax.fori_loop(0, n_seg + LAG, step, 0)

    out_copy(n_seg - 2).start()
    last = xb[seg:, :] + _dot(act[seg:, :], wd[...])
    out_v[(n_seg - 1) * seg:, :] = last.astype(out_v.dtype)
    out_copy(n_seg - 1).start()
    pltpu.make_async_copy(out_v, out_hbm, sem_out).wait()


@functools.partial(jax.jit, static_argnames=("A_seg_len",))
def pallas_interleave_layers__memory_aug_recurrent_mem_tr__glu_gated_glu__prompt_kernel(
    A_x, A_mem0, A_Wq, A_Wk, A_Wv, A_Wo, A_seg_len, B_x, B_w_gate, B_w_up, B_w_down,
):
    del B_x
    B, S, D = A_x.shape
    M = A_mem0.shape[1]
    _, H, Dh = A_Wq.shape
    F = B_w_gate.shape[1]
    seg = int(A_seg_len)
    assert B == 1 and S % seg == 0
    R = 2 * (M + seg)
    hbm = pl.BlockSpec(memory_space=pl.ANY)
    out = pl.pallas_call(
        functools.partial(_kernel, seg=seg),
        out_shape=jax.ShapeDtypeStruct((S, D), A_x.dtype),
        in_specs=[hbm, pl.BlockSpec(memory_space=pltpu.VMEM)] + [hbm] * 7,
        out_specs=hbm,
        scratch_shapes=[
            pltpu.VMEM((S, D), BF16),
            pltpu.VMEM((S, D), A_x.dtype),
            pltpu.VMEM((3, D, H, Dh), BF16),
            pltpu.VMEM((H // HEAD_GROUP, D, 3 * HEAD_GROUP * Dh), BF16),
            pltpu.VMEM((H * Dh, D), BF16),
            pltpu.VMEM((D, F), BF16),
            pltpu.VMEM((D, F), BF16),
            pltpu.VMEM((F, D), BF16),
            pltpu.VMEM((R, D), BF16),
            pltpu.VMEM((2 * seg, D), F32),
            pltpu.VMEM((R, H * Dh), BF16),
            pltpu.VMEM((2 * seg, D), F32),
            pltpu.VMEM((2 * seg, D), BF16),
            pltpu.VMEM((2 * seg, F), BF16),
            pltpu.VMEM((2 * seg, D), F32),
            pltpu.VMEM((R, R), F32),
            pltpu.SemaphoreType.DMA(()),
            pltpu.SemaphoreType.DMA((3, D // RAW_CHUNK)),
            pltpu.SemaphoreType.DMA((4,)),
            pltpu.SemaphoreType.DMA(()),
        ],
        compiler_params=pltpu.CompilerParams(vmem_limit_bytes=110 * 2**20),
    )(A_x.reshape(S, D), A_mem0.reshape(M, D), A_Wq, A_Wk, A_Wv,
      A_Wo.reshape(H * Dh, D), B_w_gate, B_w_up, B_w_down)
    return out.reshape(B, S, D)
```

```python
import functools

import jax
import jax.numpy as jnp
from jax import lax
import jax.experimental.pallas as pl
import jax.experimental.pallas.tpu as pltpu

F32 = jnp.float32
BF16 = jnp.bfloat16
LAG = 3
RING = 4
HEAD_GROUP = 4
FF_CHUNK = 512
RAW_CHUNK = 128
RAW_AHEAD = 1
X_HEAD = 8


def _layernorm(x):
    m = jnp.mean(x, axis=-1, keepdims=True)
    d = x - m
    v = jnp.mean(d * d, axis=-1, keepdims=True)
    return d * lax.rsqrt(v + 1e-5)


def _dot(a, b):
    return jnp.dot(a, b, preferred_element_type=F32)


def _kernel(x_hbm, mem0_ref, wq_hbm, wk_hbm, wv_hbm, wo_hbm, wg_hbm, wu_hbm, wd_hbm,
            out_hbm,
            x_v, out_v, raw, wqkv, wo, wg, wu, wd,
            h_in, xa, attn, xb, hb, act, dacc, ring, bias,
            sem_x, sem_raw, sem_w, sem_out, *, seg):
    S, D = x_v.shape
    M = mem0_ref.shape[0]
    Dh = wq_hbm.shape[1]
    H = wq_hbm.shape[0] // D
    F = wg.shape[1]
    n_seg = S // seg
    R = 2 * (M + seg)
    MEM, TOK2 = seg, seg + 2 * M
    G = HEAD_GROUP
    scale = Dh ** -0.5
    n_raw = D // RAW_CHUNK

    def seg_rows(s, n=1):
        start = s * seg
        return pl.ds(start if isinstance(start, int) else pl.multiple_of(start, seg), n * seg)

    x_head = pltpu.make_async_copy(
        x_hbm.at[seg_rows(0, X_HEAD)], x_v.at[seg_rows(0, X_HEAD)], sem_x.at[0])
    x_tail = pltpu.make_async_copy(
        x_hbm.at[seg_rows(X_HEAD, n_seg - X_HEAD)],
        x_v.at[seg_rows(X_HEAD, n_seg - X_HEAD)], sem_x.at[1])

    def raw_copy(c, i):
        n = RAW_CHUNK * H
        return pltpu.make_async_copy((wq_hbm, wk_hbm, wv_hbm)[i].at[pl.ds(c * n, n)],
                                     raw.at[3 * c + i], sem_raw.at[i, c])

    wo_copy, wg_copy, wu_copy, wd_copy = (
        pltpu.make_async_copy(s, d, sem_w.at[i]) for i, (s, d) in enumerate(
            ((wo_hbm, wo), (wg_hbm, wg), (wu_hbm, wu), (wd_hbm, wd))))

    for c in range(RAW_AHEAD):
        for i in range(3):
            raw_copy(c, i).start()
    x_head.start()

    r = lax.broadcasted_iota(jnp.int32, (R, R), 0)
    c = lax.broadcasted_iota(jnp.int32, (R, R), 1)

    def is_mem(i):
        return (i >= MEM) & (i < TOK2)

    visible = is_mem(r) | is_mem(c) | (r >= c)
    mask = jnp.where((r >= seg + M) == (c >= seg + M),
                     jnp.where(visible, 0.0, -1e9), -jnp.inf).astype(F32)
    bias[0] = mask
    bias[1, :, 0:R - MEM] = mask[:, MEM:]

    raw32 = raw.bitcast(jnp.uint32)

    def relayout(c, carry):
        base = pl.multiple_of(c * RAW_CHUNK, RAW_CHUNK)
        for i in range(3):
            raw_copy(c, i).wait()

            @pl.when(c + RAW_AHEAD < n_raw)
            def _():
                raw_copy(c + RAW_AHEAD, i).start()

            if i == 0:
                @pl.when(c + RAW_AHEAD == n_raw)
                def _():
                    wo_copy.start()

            for j in range(H // 2):
                even = raw32[3 * c + i, pl.ds(j, RAW_CHUNK // 2, stride=H), :]
                odd = raw32[3 * c + i, pl.ds(H // 2 + j, RAW_CHUNK // 2, stride=H), :]
                lo = (even & 0xFFFF) | (odd << 16)
                hi = (even >> 16) | (odd & jnp.uint32(0xFFFF0000))
                for head, word in ((2 * j, lo), (2 * j + 1, hi)):
                    col = (i * G + head % G) * Dh
                    wqkv[head // G, pl.ds(base, RAW_CHUNK), col:col + Dh] = (
                        pltpu.bitcast(word, BF16))
        return carry

    lax.fori_loop(0, n_raw, relayout, 0)

    mem0 = mem0_ref[...].astype(F32)

    def feed_layer1(s):
        xs = x_v[seg_rows(s), :].astype(F32)
        xa[0:seg, :] = xs
        h_in[0:seg, :] = _layernorm(xs).astype(BF16)

    def feed_layer2(s):
        xs = ring[s % RING]
        xa[seg:2 * seg, :] = xs
        h_in[TOK2:R, :] = _layernorm(xs).astype(BF16)

    def attention(lo, hi, fillers=(None, None)):
        def project(g, i):
            w = wqkv[g, :, i * G * Dh:(i + 1) * G * Dh]
            y = _dot(h_in[lo:hi, :], w).astype(BF16)
            return [y[:, j * Dh:(j + 1) * Dh] for j in range(G)]

        def probabilities(q, k):
            s = lax.dot_general(q, k, (((1,), (1,)), ((), ())), preferred_element_type=F32)
            b = bias[int(lo > 0), lo:hi, 0:hi - lo]
            s = jnp.where(b == 0.0, s * scale, b)
            e = jnp.exp(s - jnp.max(s, axis=-1, keepdims=True))
            return (e * (1.0 / jnp.sum(e, axis=-1, keepdims=True))).astype(BF16)

        q, k = project(0, 0), project(0, 1)
        for g in range(H // G):
            last = g + 1 == H // G
            v = project(g, 2)
            p = [probabilities(q[j], k[j]) for j in range(G)]
            if not last:
                q = project(g + 1, 0)
            elif fillers[0]:
                fillers[0]()
            for j in range(G):
                head = g * G + j
                attn[lo:hi, head * Dh:(head + 1) * Dh] = _dot(p[j], v[j]).astype(BF16)
            if not last:
                k = project(g + 1, 1)
            elif fillers[1]:
                fillers[1]()

    def feed_ffn(rows, x1):
        xb[rows, :] = x1
        hb[rows, :] = _layernorm(x1).astype(BF16)

    def gate_up(n):
        for f in range(0, F, FF_CHUNK):
            g = _dot(hb[0:n, :], wg[:, f:f + FF_CHUNK])
            u = _dot(hb[0:n, :], wu[:, f:f + FF_CHUNK])
            act[0:n, f:f + FF_CHUNK] = (jax.nn.sigmoid(g) * u).astype(BF16)

    def down(lo, hi):
        return xb[lo:hi, :] + _dot(act[lo:hi, :], wd[...])

    def out_copy(s, n=1):
        return pltpu.make_async_copy(
            out_v.at[seg_rows(s, n)], out_hbm.at[seg_rows(s, n)], sem_out)

    x_head.wait()
    h_in[MEM:TOK2, :] = jnp.concatenate([mem0, mem0], axis=0).astype(BF16)
    feed_layer1(0)

    def fill(t, carry):
        attention(0, TOK2)

        @pl.when(t == 0)
        def _():
            wg_copy.start()
            wo_copy.wait()
            wu_copy.start()

        @pl.when(t == LAG - 1)
        def _():
            wd_copy.start()

        o = _dot(attn[0:TOK2, :], wo[...])
        h_in[MEM:TOK2, :] = jnp.concatenate([o[MEM:MEM + M], mem0], axis=0).astype(BF16)
        feed_ffn(seg_rows((t + 1) % LAG), xa[0:seg, :] + o[0:seg])
        feed_layer1(t + 1)
        return carry

    lax.fori_loop(0, LAG, fill, 0)
    wg_copy.wait()
    wu_copy.wait()
    gate_up(LAG * seg)
    wd_copy.wait()
    x_tail.start()
    x2 = down(seg, LAG * seg)
    for s in range(LAG - 1):
        ring[s] = x2[s * seg:(s + 1) * seg]
    feed_layer2(0)

    def step(t, carry):
        @pl.when(t >= LAG + 2)
        def _():
            out_copy(t - LAG - 2).start()

        @pl.when(t == X_HEAD - 1)
        def _():
            x_tail.wait()

        def down_part(src, i):
            cols = slice(i * F // 4, (i + 1) * F // 4)
            dacc[...] = src[0:2 * seg, :] + _dot(act[0:2 * seg, cols], wd[cols, :])

        attention(0, R, (lambda: down_part(xb, 0), lambda: down_part(dacc, 1)))
        o = _dot(attn[...], wo[...])
        h_in[MEM:TOK2, :] = o[MEM:TOK2].astype(BF16)
        feed_ffn(seg_rows(0, 2),
                 xa[...] + jnp.concatenate([o[0:seg], o[TOK2:R]], axis=0))
        x2 = dacc[...] + _dot(act[0:2 * seg, F // 2:], wd[F // 2:, :])
        ring[(t - 1) % RING] = x2[0:seg]
        out_v[seg_rows(jnp.maximum(t - LAG - 1, 0)), :] = x2[seg:].astype(out_v.dtype)
        feed_layer1(jnp.minimum(t + 1, n_seg - 1))
        feed_layer2(t + 1 - LAG)
        gate_up(2 * seg)
        return carry

    lax.fori_loop(LAG, n_seg, step, 0)

    x2 = down(0, 2 * seg)
    ring[(n_seg - 1) % RING] = x2[0:seg]
    out_v[seg_rows(n_seg - LAG - 1), :] = x2[seg:].astype(out_v.dtype)
    out_copy(n_seg - LAG - 2, 2).start()

    def drain(i, carry):
        attention(MEM, R)
        o = _dot(attn[MEM:R, :], wo[...])
        h_in[MEM:TOK2, :] = jnp.concatenate([mem0, o[M:2 * M]], axis=0).astype(BF16)
        feed_ffn(seg_rows(i), xa[seg:, :] + o[2 * M:])
        feed_layer2(jnp.minimum(n_seg - LAG + i + 1, n_seg - 1))
        return carry

    lax.fori_loop(0, LAG, drain, 0)
    gate_up(LAG * seg)
    out_v[seg_rows(n_seg - LAG, LAG), :] = down(0, LAG * seg).astype(out_v.dtype)
    out_copy(n_seg - LAG, LAG).start()
    pltpu.make_async_copy(out_v, out_hbm, sem_out).wait()


@functools.partial(jax.jit, static_argnames=("A_seg_len",))
def pallas_interleave_layers__memory_aug_recurrent_mem_tr__glu_gated_glu__prompt_kernel(
    A_x, A_mem0, A_Wq, A_Wk, A_Wv, A_Wo, A_seg_len, B_x, B_w_gate, B_w_up, B_w_down,
):
    del B_x
    B, S, D = A_x.shape
    M = A_mem0.shape[1]
    _, H, Dh = A_Wq.shape
    F = B_w_gate.shape[1]
    seg = int(A_seg_len)
    assert B == 1 and S % seg == 0
    R = 2 * (M + seg)
    hbm = pl.BlockSpec(memory_space=pl.ANY)
    out = pl.pallas_call(
        functools.partial(_kernel, seg=seg),
        out_shape=jax.ShapeDtypeStruct((S, D), A_x.dtype),
        in_specs=[hbm, pl.BlockSpec(memory_space=pltpu.VMEM)] + [hbm] * 7,
        out_specs=hbm,
        scratch_shapes=[
            pltpu.VMEM((S, D), BF16),
            pltpu.VMEM((S, D), A_x.dtype),
            pltpu.VMEM((3 * D // RAW_CHUNK, RAW_CHUNK * H, Dh), BF16),
            pltpu.VMEM((H // HEAD_GROUP, D, 3 * HEAD_GROUP * Dh), BF16),
            pltpu.VMEM((H * Dh, D), BF16),
            pltpu.VMEM((D, F), BF16),
            pltpu.VMEM((D, F), BF16),
            pltpu.VMEM((F, D), BF16),
            pltpu.VMEM((R, D), BF16),
            pltpu.VMEM((2 * seg, D), F32),
            pltpu.VMEM((R, H * Dh), BF16),
            pltpu.VMEM((LAG * seg, D), F32),
            pltpu.VMEM((LAG * seg, D), BF16),
            pltpu.VMEM((LAG * seg, F), BF16),
            pltpu.VMEM((2 * seg, D), F32),
            pltpu.VMEM((RING, seg, D), F32),
            pltpu.VMEM((2, R, R), F32),
            pltpu.SemaphoreType.DMA((2,)),
            pltpu.SemaphoreType.DMA((3, D // RAW_CHUNK)),
            pltpu.SemaphoreType.DMA((4,)),
            pltpu.SemaphoreType.DMA(()),
        ],
        compiler_params=pltpu.CompilerParams(vmem_limit_bytes=110 * 2**20),
    )(A_x.reshape(S, D), A_mem0.reshape(M, D), A_Wq.reshape(D * H, Dh),
      A_Wk.reshape(D * H, Dh), A_Wv.reshape(D * H, Dh),
      A_Wo.reshape(H * Dh, D), B_w_gate, B_w_up, B_w_down)
    return out.reshape(B, S, D)
```

```python
import functools

import jax
import jax.numpy as jnp
from jax import lax
import jax.experimental.pallas as pl
import jax.experimental.pallas.tpu as pltpu

F32 = jnp.float32
BF16 = jnp.bfloat16
LAG = 3
RING = 4
HEAD_GROUP = 4
FF_CHUNK = 512
RAW_CHUNK = 128
RAW_AHEAD = 1
PRE_ROWS = 16
PRE_STEPS = 16
X_HEAD = LAG + PRE_STEPS + 1


def _layernorm(x):
    m = jnp.mean(x, axis=-1, keepdims=True)
    d = x - m
    v = jnp.mean(d * d, axis=-1, keepdims=True)
    return d * lax.rsqrt(v + 1e-5)


def _dot(a, b):
    return jnp.dot(a, b, preferred_element_type=F32)


def _kernel(x_hbm, mem0_ref, wq_hbm, wk_hbm, wv_hbm, wo_hbm, wg_hbm, wu_hbm, wd_hbm,
            out_hbm,
            x_v, out_v, raw, wqkv, wo, wg, wu, wd,
            h_in, xa, attn, xb, hb, act, dacc, ring, bias, pre_in, pre,
            sem_x, sem_raw, sem_w, sem_out, *, seg):
    S, D = x_v.shape
    M = mem0_ref.shape[0]
    Dh = wq_hbm.shape[1]
    H = wq_hbm.shape[0] // D
    F = wg.shape[1]
    n_seg = S // seg
    R = 2 * (M + seg)
    MEM, TOK2 = seg, seg + 2 * M
    G = HEAD_GROUP
    scale = Dh ** -0.5
    n_raw = D // RAW_CHUNK

    def seg_rows(s, n=1):
        start = s * seg
        return pl.ds(start if isinstance(start, int) else pl.multiple_of(start, seg), n * seg)

    x_head = pltpu.make_async_copy(
        x_hbm.at[seg_rows(0, X_HEAD)], x_v.at[seg_rows(0, X_HEAD)], sem_x.at[0])
    x_tail = pltpu.make_async_copy(
        x_hbm.at[seg_rows(X_HEAD, n_seg - X_HEAD)],
        x_v.at[seg_rows(X_HEAD, n_seg - X_HEAD)], sem_x.at[1])

    def raw_copy(c, i):
        n = RAW_CHUNK * H
        return pltpu.make_async_copy((wq_hbm, wk_hbm, wv_hbm)[i].at[pl.ds(c * n, n)],
                                     raw.at[3 * c + i], sem_raw.at[i, c])

    wo_copy, wg_copy, wu_copy, wd_copy = (
        pltpu.make_async_copy(s, d, sem_w.at[i]) for i, (s, d) in enumerate(
            ((wo_hbm, wo), (wg_hbm, wg), (wu_hbm, wu), (wd_hbm, wd))))

    x_head.start()
    for c in range(RAW_AHEAD):
        for i in range(3):
            raw_copy(c, i).start()

    r = lax.broadcasted_iota(jnp.int32, (R, R), 0)
    c = lax.broadcasted_iota(jnp.int32, (R, R), 1)

    def is_mem(i):
        return (i >= MEM) & (i < TOK2)

    visible = is_mem(r) | is_mem(c) | (r >= c)
    mask = jnp.where((r >= seg + M) == (c >= seg + M),
                     jnp.where(visible, 0.0, -1e9), -jnp.inf).astype(F32)
    bias[0] = mask
    bias[1, :, 0:R - MEM] = mask[:, MEM:]

    raw32 = raw.bitcast(jnp.uint32)
    pre[...] = jnp.zeros(pre.shape, F32)
    x_head.wait()
    for n in range(PRE_STEPS):
        start = (LAG + n) * seg
        hs = _layernorm(x_v[start:start + PRE_ROWS, :].astype(F32)).astype(BF16)
        for c in range(n_raw):
            pre_in[c, n * PRE_ROWS:(n + 1) * PRE_ROWS, :] = (
                hs[:, c * RAW_CHUNK:(c + 1) * RAW_CHUNK])

    def relayout(c, carry):
        base = pl.multiple_of(c * RAW_CHUNK, RAW_CHUNK)
        for i in range(3):
            raw_copy(c, i).wait()

            @pl.when(c + RAW_AHEAD < n_raw)
            def _():
                raw_copy(c + RAW_AHEAD, i).start()

            if i == 0:
                @pl.when(c + RAW_AHEAD == n_raw)
                def _():
                    wo_copy.start()

            cols = slice(i * G * Dh, (i + 1) * G * Dh)
            for g in range(H // G):
                tiles = []
                for j in range(g * G // 2, (g + 1) * G // 2):
                    even = raw32[3 * c + i, pl.ds(j, RAW_CHUNK // 2, stride=H), :]
                    odd = raw32[3 * c + i, pl.ds(H // 2 + j, RAW_CHUNK // 2, stride=H), :]
                    tiles.append((even & 0xFFFF) | (odd << 16))
                    tiles.append((even >> 16) | (odd & jnp.uint32(0xFFFF0000)))
                w = pltpu.bitcast(jnp.concatenate(tiles, axis=1), BF16)
                wqkv[g, pl.ds(base, RAW_CHUNK), cols] = w
                pre[g, :, cols] += _dot(pre_in[c], w)
        return carry

    lax.fori_loop(0, n_raw, relayout, 0)

    mem0 = mem0_ref[...].astype(F32)

    def feed_layer1(s):
        xs = x_v[seg_rows(s), :].astype(F32)
        xa[0:seg, :] = xs
        h_in[0:seg, :] = _layernorm(xs).astype(BF16)

    def feed_layer2(s):
        xs = ring[s % RING]
        xa[seg:2 * seg, :] = xs
        h_in[TOK2:R, :] = _layernorm(xs).astype(BF16)

    def attention(lo, hi, fillers=(None, None), pre_rows=None):
        def project(g, i):
            cols = slice(i * G * Dh, (i + 1) * G * Dh)
            if pre_rows is None:
                y = _dot(h_in[lo:hi, :], wqkv[g, :, cols])
            else:
                y = jnp.concatenate(
                    [pre[g, pre_rows, cols],
                     _dot(h_in[lo + PRE_ROWS:hi, :], wqkv[g, :, cols])], axis=0)
            y = y.astype(BF16)
            return [y[:, j * Dh:(j + 1) * Dh] for j in range(G)]

        def probabilities(q, k):
            s = lax.dot_general(q, k, (((1,), (1,)), ((), ())), preferred_element_type=F32)
            b = bias[int(lo > 0), lo:hi, 0:hi - lo]
            s = jnp.where(b == 0.0, s * scale, b)
            e = jnp.exp(s - jnp.max(s, axis=-1, keepdims=True))
            return (e * (1.0 / jnp.sum(e, axis=-1, keepdims=True))).astype(BF16)

        q, k = project(0, 0), project(0, 1)
        for g in range(H // G):
            last = g + 1 == H // G
            v = project(g, 2)
            p = [probabilities(q[j], k[j]) for j in range(G)]
            if not last:
                q = project(g + 1, 0)
            elif fillers[0]:
                fillers[0]()
            for j in range(G):
                head = g * G + j
                attn[lo:hi, head * Dh:(head + 1) * Dh] = _dot(p[j], v[j]).astype(BF16)
            if not last:
                k = project(g + 1, 1)
            elif fillers[1]:
                fillers[1]()

    def feed_ffn(rows, x1):
        xb[rows, :] = x1
        hb[rows, :] = _layernorm(x1).astype(BF16)

    def gate_up(n):
        for f in range(0, F, FF_CHUNK):
            g = _dot(hb[0:n, :], wg[:, f:f + FF_CHUNK])
            u = _dot(hb[0:n, :], wu[:, f:f + FF_CHUNK])
            act[0:n, f:f + FF_CHUNK] = (jax.nn.sigmoid(g) * u).astype(BF16)

    def down(lo, hi):
        return xb[lo:hi, :] + _dot(act[lo:hi, :], wd[...])

    def out_copy(s, n=1):
        return pltpu.make_async_copy(
            out_v.at[seg_rows(s, n)], out_hbm.at[seg_rows(s, n)], sem_out)

    h_in[MEM:TOK2, :] = jnp.concatenate([mem0, mem0], axis=0).astype(BF16)
    feed_layer1(0)

    def fill(t, carry):
        attention(0, TOK2)

        @pl.when(t == 0)
        def _():
            wg_copy.start()
            wo_copy.wait()
            wu_copy.start()

        @pl.when(t == LAG - 1)
        def _():
            wd_copy.start()

        o = _dot(attn[0:TOK2, :], wo[...])
        h_in[MEM:TOK2, :] = jnp.concatenate([o[MEM:MEM + M], mem0], axis=0).astype(BF16)
        feed_ffn(seg_rows((t + 1) % LAG), xa[0:seg, :] + o[0:seg])
        feed_layer1(t + 1)
        return carry

    lax.fori_loop(0, LAG, fill, 0)
    wg_copy.wait()
    wu_copy.wait()
    gate_up(LAG * seg)
    wd_copy.wait()
    x_tail.start()
    x2 = down(seg, LAG * seg)
    for s in range(LAG - 1):
        ring[s] = x2[s * seg:(s + 1) * seg]
    feed_layer2(0)

    def step(t, carry, *, use_pre):
        @pl.when(t >= LAG + 2)
        def _():
            out_copy(t - LAG - 2).start()


        def down_part(src, i):
            cols = slice(i * F // 4, (i + 1) * F // 4)
            dacc[...] = src[0:2 * seg, :] + _dot(act[0:2 * seg, cols], wd[cols, :])

        pre_rows = None
        if use_pre:
            pre_rows = pl.ds(pl.multiple_of((t - LAG) * PRE_ROWS, PRE_ROWS), PRE_ROWS)
        attention(0, R, (lambda: down_part(xb, 0), lambda: down_part(dacc, 1)), pre_rows)
        o = _dot(attn[...], wo[...])
        h_in[MEM:TOK2, :] = o[MEM:TOK2].astype(BF16)
        feed_ffn(seg_rows(0, 2),
                 xa[...] + jnp.concatenate([o[0:seg], o[TOK2:R]], axis=0))
        x2 = dacc[...] + _dot(act[0:2 * seg, F // 2:], wd[F // 2:, :])
        ring[(t - 1) % RING] = x2[0:seg]
        out_v[seg_rows(jnp.maximum(t - LAG - 1, 0)), :] = x2[seg:].astype(out_v.dtype)
        feed_layer1(jnp.minimum(t + 1, n_seg - 1))
        feed_layer2(t + 1 - LAG)
        gate_up(2 * seg)
        return carry

    lax.fori_loop(LAG, LAG + PRE_STEPS, functools.partial(step, use_pre=True), 0)
    x_tail.wait()
    lax.fori_loop(LAG + PRE_STEPS, n_seg, functools.partial(step, use_pre=False), 0)

    x2 = down(0, 2 * seg)
    ring[(n_seg - 1) % RING] = x2[0:seg]
    out_v[seg_rows(n_seg - LAG - 1), :] = x2[seg:].astype(out_v.dtype)
    out_copy(n_seg - LAG - 2, 2).start()

    def drain(i, carry):
        attention(MEM, R)
        o = _dot(attn[MEM:R, :], wo[...])
        h_in[MEM:TOK2, :] = jnp.concatenate([mem0, o[M:2 * M]], axis=0).astype(BF16)
        feed_ffn(seg_rows(i), xa[seg:, :] + o[2 * M:])
        feed_layer2(jnp.minimum(n_seg - LAG + i + 1, n_seg - 1))
        return carry

    lax.fori_loop(0, LAG, drain, 0)
    gate_up(LAG * seg)
    out_v[seg_rows(n_seg - LAG, LAG), :] = down(0, LAG * seg).astype(out_v.dtype)
    out_copy(n_seg - LAG, LAG).start()
    pltpu.make_async_copy(out_v, out_hbm, sem_out).wait()


@functools.partial(jax.jit, static_argnames=("A_seg_len",))
def pallas_interleave_layers__memory_aug_recurrent_mem_tr__glu_gated_glu__prompt_kernel(
    A_x, A_mem0, A_Wq, A_Wk, A_Wv, A_Wo, A_seg_len, B_x, B_w_gate, B_w_up, B_w_down,
):
    del B_x
    B, S, D = A_x.shape
    M = A_mem0.shape[1]
    _, H, Dh = A_Wq.shape
    F = B_w_gate.shape[1]
    seg = int(A_seg_len)
    assert B == 1 and S % seg == 0
    R = 2 * (M + seg)
    hbm = pl.BlockSpec(memory_space=pl.ANY)
    out = pl.pallas_call(
        functools.partial(_kernel, seg=seg),
        out_shape=jax.ShapeDtypeStruct((S, D), A_x.dtype),
        in_specs=[hbm, pl.BlockSpec(memory_space=pltpu.VMEM)] + [hbm] * 7,
        out_specs=hbm,
        scratch_shapes=[
            pltpu.VMEM((S, D), BF16),
            pltpu.VMEM((S, D), A_x.dtype),
            pltpu.VMEM((3 * D // RAW_CHUNK, RAW_CHUNK * H, Dh), BF16),
            pltpu.VMEM((H // HEAD_GROUP, D, 3 * HEAD_GROUP * Dh), BF16),
            pltpu.VMEM((H * Dh, D), BF16),
            pltpu.VMEM((D, F), BF16),
            pltpu.VMEM((D, F), BF16),
            pltpu.VMEM((F, D), BF16),
            pltpu.VMEM((R, D), BF16),
            pltpu.VMEM((2 * seg, D), F32),
            pltpu.VMEM((R, H * Dh), BF16),
            pltpu.VMEM((LAG * seg, D), F32),
            pltpu.VMEM((LAG * seg, D), BF16),
            pltpu.VMEM((LAG * seg, F), BF16),
            pltpu.VMEM((2 * seg, D), F32),
            pltpu.VMEM((RING, seg, D), F32),
            pltpu.VMEM((2, R, R), F32),
            pltpu.VMEM((D // RAW_CHUNK, PRE_STEPS * PRE_ROWS, RAW_CHUNK), BF16),
            pltpu.VMEM((H // HEAD_GROUP, PRE_STEPS * PRE_ROWS, 3 * HEAD_GROUP * Dh), F32),
            pltpu.SemaphoreType.DMA((2,)),
            pltpu.SemaphoreType.DMA((3, D // RAW_CHUNK)),
            pltpu.SemaphoreType.DMA((4,)),
            pltpu.SemaphoreType.DMA(()),
        ],
        compiler_params=pltpu.CompilerParams(vmem_limit_bytes=120 * 2**20),
    )(A_x.reshape(S, D), A_mem0.reshape(M, D), A_Wq.reshape(D * H, Dh),
      A_Wk.reshape(D * H, Dh), A_Wv.reshape(D * H, Dh),
      A_Wo.reshape(H * Dh, D), B_w_gate, B_w_up, B_w_down)
    return out.reshape(B, S, D)
```

```python
import functools

import jax
import jax.numpy as jnp
from jax import lax
import jax.experimental.pallas as pl
import jax.experimental.pallas.tpu as pltpu

F32 = jnp.float32
BF16 = jnp.bfloat16
LANES = 128
LAG = 3
RING = 4
GROUP = 4
RAW_SLOTS = 3
PRE_ROWS = 16
PRE_STEPS = 16
X_HEAD = LAG + PRE_STEPS + 1
OUT_SLOTS = 4
B11, B12, B21, B22 = 1, 2, 3, 4


def _layernorm(x):
    m = jnp.mean(x, axis=-1, keepdims=True)
    d = x - m
    v = jnp.mean(d * d, axis=-1, keepdims=True)
    return d * lax.rsqrt(v + 1e-5)


def _dot(a, b):
    return lax.dot_general(a, b, (((1,), (0,)), ((), ())), preferred_element_type=F32)


def _weight_sums(b11, b12, b21, b22):
    b11, b12, b21, b22 = (b.astype(F32) for b in (b11, b12, b21, b22))
    sums = {0: b11 + b22, 2: b12 - b22, 3: b21 - b11, 5: b11 + b12, 6: b21 + b22}
    return {p: s.astype(BF16) for p, s in sums.items()}


def _row_sums(a11, a12, a21=None, a22=None):
    if a21 is None:
        return {0: a11, 2: a11, 4: a11 + a12, 6: a12}
    return {0: a11 + a22, 1: a21 + a22, 2: a11, 3: a22,
            4: a11 + a12, 5: a21 - a11, 6: a12 - a22}


def _left(m):
    if 1 not in m:
        return [m[0] - m[4] + m[6]]
    return [m[0] + m[3] - m[4] + m[6], m[1] + m[3]]


def _right(m):
    if 1 not in m:
        return [m[2] + m[4]]
    return [m[2] + m[4], m[0] - m[1] + m[2] + m[5]]


def _tile(x, j):
    return x[:, j * LANES:(j + 1) * LANES]


def _kernel(x_hbm, mem0_ref, wq_hbm, wk_hbm, wv_hbm, wo_hbm, wg_hbm, wu_hbm, wd_hbm,
            out_hbm,
            x_v, out_v, raw, wqkv, wo, wgu, wd,
            lhs_h, lhs_o, lhs_b, lhs_d, dacc, xa, xb, ring, bias, pre_in, pre,
            sem_x, sem_raw, sem_w, sem_out, *, seg):
    S, D = x_v.shape
    M = mem0_ref.shape[0]
    Dh = LANES
    H = wq_hbm.shape[0] // D
    n_seg = S // seg
    L = M + seg
    half = D // 2
    n_kt = half // LANES
    n_ff = wd.shape[2]
    n_groups = H // (2 * GROUP)
    scale = Dh ** -0.5
    ONE, BOTH = (0, 2, 4, 6), (0, 1, 2, 3, 4, 5, 6)

    def seg_rows(s, n=1):
        start = s * seg
        return pl.ds(start if isinstance(start, int) else pl.multiple_of(start, seg), n * seg)

    x_head = pltpu.make_async_copy(
        x_hbm.at[seg_rows(0, X_HEAD)], x_v.at[seg_rows(0, X_HEAD)], sem_x.at[0])
    x_tail = pltpu.make_async_copy(
        x_hbm.at[seg_rows(X_HEAD, n_seg - X_HEAD)],
        x_v.at[seg_rows(X_HEAD, n_seg - X_HEAD)], sem_x.at[1])

    def raw_copies(n, src):
        slot = n % RAW_SLOTS
        return [pltpu.make_async_copy(
            src.at[pl.ds((n // 3 + a * n_kt) * LANES * H, LANES * H)],
            raw.at[slot, a], sem_raw.at[slot]) for a in range(2)]

    def start_raw(n):
        for i, src in enumerate((wq_hbm, wk_hbm, wv_hbm)):
            @pl.when(n % 3 == i)
            def _():
                for cp in raw_copies(n, src):
                    cp.start()

    blocks = ((B11, 0, 0), (B12, 0, 1), (B21, 1, 0), (B22, 1, 1))

    def proj_copies(src, dst, sem):
        return [pltpu.make_async_copy(
            src.at[:, a, :, pl.ds((b * n_kt + j) * LANES, LANES)], dst.at[p, j], sem)
            for p, a, b in blocks for j in range(n_kt)]

    def ffn_slot(pair, up):
        return (pair // 2) * GROUP + 2 * up + pair % 2

    def ffn_copies(src, up, sem):
        return [pltpu.make_async_copy(
            src.at[pl.ds(a * half, half), pl.ds((2 * j + b) * LANES, LANES)],
            wgu.at[p, ffn_slot(j, up)], sem)
            for p, a, b in blocks for j in range(n_ff)]

    wo_copies = proj_copies(wo_hbm, wo, sem_w.at[0])
    wg_copies = ffn_copies(wg_hbm, 0, sem_w.at[1])
    wu_copies = ffn_copies(wu_hbm, 1, sem_w.at[1])
    wd_copies = proj_copies(wd_hbm, wd, sem_w.at[2])

    def start(copies):
        for cp in copies:
            cp.start()

    def wait(copies):
        for cp in copies:
            cp.wait()

    def form_operands(w):
        def body(j, carry):
            sums = _weight_sums(w[B11, j], w[B12, j], w[B21, j], w[B22, j])
            for p, s in sums.items():
                w[p, j] = s
            return carry
        lax.fori_loop(0, w.shape[1], body, 0)

    x_head.start()
    start(raw_copies(0, wq_hbm))

    r = lax.broadcasted_iota(jnp.int32, (2 * L, 2 * L), 0)
    c = lax.broadcasted_iota(jnp.int32, (2 * L, 2 * L), 1)
    visible = (r < M) | ((r >= L) & (r < L + M)) | (r >= c)
    bias[...] = jnp.where((r >= L) == (c >= L),
                          jnp.where(visible, 0.0, -1e9), -jnp.inf).astype(F32)

    pre[...] = jnp.zeros(pre.shape, F32)
    x_head.wait()
    start(raw_copies(1, wk_hbm))
    for n in range(PRE_STEPS):
        first = (LAG + n) * seg
        hs = _layernorm(x_v[first:first + PRE_ROWS, :].astype(F32)).astype(BF16)
        for j in range(n_kt):
            pre_in[j, n * PRE_ROWS:(n + 1) * PRE_ROWS, :] = jnp.concatenate(
                [_tile(hs, j), _tile(hs, j + n_kt)], axis=1)

    raw32 = raw.bitcast(jnp.uint32)

    def relayout(n, carry):
        slot, i, kt = n % RAW_SLOTS, n % 3, n // 3
        wait(raw_copies(n, wq_hbm))

        @pl.when(n + 2 < 3 * n_kt)
        def _():
            start_raw(n + 2)

        @pl.when(n + 2 == 3 * n_kt)
        def _():
            start(wo_copies)

        rows = pl.ds(pl.multiple_of(kt * LANES, LANES), LANES)
        for g in range(H // GROUP):
            tiles = []
            for j in range(g * GROUP // 2, (g + 1) * GROUP // 2):
                b = []
                for a in range(2):
                    even = raw32[slot, a, pl.ds(j, LANES // 2, stride=H), :]
                    odd = raw32[slot, a, pl.ds(H // 2 + j, LANES // 2, stride=H), :]
                    b.append(pltpu.bitcast((even & 0xFFFF) | (odd << 16), BF16))
                    b.append(pltpu.bitcast(
                        (even >> 16) | (odd & jnp.uint32(0xFFFF0000)), BF16))
                for p, s in {**_weight_sums(*b), B11: b[0], B22: b[3]}.items():
                    wqkv[i, p, j, rows, :] = s
                tiles += [jnp.concatenate([b[0], b[2]], axis=0),
                          jnp.concatenate([b[1], b[3]], axis=0)]
            pre[i, g] += _dot(pre_in[kt], jnp.concatenate(tiles, axis=1))
        return carry

    lax.fori_loop(0, 3 * n_kt, relayout, 0)

    mem0 = mem0_ref[...].astype(F32)

    def put(dst, rows, cols, top, bottom=None, products=None):
        sums = _row_sums(*top, *(bottom or ()))
        for p in products or sums:
            dst[p, rows, cols] = sums[p].astype(dst.dtype)

    def halves(x):
        return x[:, :half], x[:, half:]

    def feed_memory(*mems):
        put(lhs_h, slice(0, M), slice(None), *map(halves, mems))

    def feed_tokens(*hs):
        put(lhs_h, slice(M, M + hs[0].shape[0]), slice(None), *map(halves, hs))

    def feed_both(use_pre):
        h2 = _layernorm(xa[1])
        if use_pre:
            h1 = _layernorm(xa[0, PRE_ROWS:, :])
            cut = PRE_ROWS // 2
            feed_tokens(jnp.concatenate([h1, h2[:cut]], axis=0), h2[cut:])
        else:
            feed_tokens(_layernorm(xa[0]), h2)

    def feed_ffn(*xs):
        for n, x in enumerate(xs):
            xb[n] = x
        put(lhs_b, slice(None), slice(None), *(halves(_layernorm(x)) for x in xs))

    def attention(products, fillers=(None, None, None), pre_rows=None):
        n_rows = L if pre_rows is None else L - PRE_ROWS // 2
        total = L if products is ONE else 2 * L

        def project(g, i):
            m = {p: _dot(lhs_h[p, 0:n_rows, :], jnp.concatenate(
                [wqkv[i, p, g * GROUP + j] for j in range(GROUP)], axis=1))
                for p in products}
            heads = []
            for j in range(GROUP):
                for b, side in enumerate((_left(m), _right(m))):
                    parts = [_tile(y, j) for y in side]
                    if pre_rows is not None:
                        head = 2 * (g * GROUP + j) + b
                        col = head % GROUP * Dh
                        parts = [parts[0][:M], pre[i, head // GROUP, pre_rows, col:col + Dh],
                                 parts[0][M:L - PRE_ROWS], parts[1][:M],
                                 parts[0][L - PRE_ROWS:], parts[1][M:]]
                    heads.append(jnp.concatenate(parts, axis=0).astype(BF16))
            return heads

        def probabilities(q, k):
            s = lax.dot_general(q, k, (((1,), (1,)), ((), ())), preferred_element_type=F32)
            b = bias[0:total, 0:total]
            s = jnp.where(b == 0.0, s * scale, b)
            e = jnp.exp(s - jnp.max(s, axis=-1, keepdims=True))
            return (e * (1.0 / jnp.sum(e, axis=-1, keepdims=True))).astype(BF16)

        def mix(g, p, v):
            for j in range(GROUP):
                o = [_dot(p[2 * j + b], v[2 * j + b]) for b in range(2)]
                col = (g * GROUP + j) * Dh
                put(lhs_o, slice(None), slice(col, col + Dh),
                    *((o[0][at:at + L], o[1][at:at + L]) for at in range(0, total, L)))

        q, k = project(0, 0), project(0, 1)
        v = project(0, 2)
        for g in range(n_groups):
            last = g + 1 == n_groups
            p = [probabilities(a, b) for a, b in zip(q, k)]
            if not last:
                q = project(g + 1, 0)
            elif fillers[0]:
                fillers[0]()
            mix(g, p, v)
            if not last:
                k, v = project(g + 1, 1), project(g + 1, 2)
            elif fillers[1]:
                fillers[1]()

    def block_product(lhs, w, p, lo=0, hi=None):
        hi = w.shape[2] if hi is None else hi
        tiles = [w[p, j, lo:hi].reshape((hi - lo) * LANES, LANES) for j in range(n_kt)]
        return _dot(lhs[p, :, lo * LANES:hi * LANES], jnp.concatenate(tiles, axis=1))

    def assemble(m):
        return [jnp.concatenate(lr, axis=1) for lr in zip(_left(m), _right(m))]

    def out_proj(products):
        return assemble({p: block_product(lhs_o, wo, p) for p in products})

    def gate_up(products, keep=None):
        for g in range(n_ff // 2):
            m = {p: _dot(lhs_b[p], jnp.concatenate(
                [wgu[p, g * GROUP + j] for j in range(GROUP)], axis=1)) for p in products}
            act = [[jax.nn.sigmoid(y[:, :2 * LANES]) * y[:, 2 * LANES:] for y in side]
                   for side in (_left(m), _right(m))]
            rows = list(zip(*act))
            if keep and products is ONE:
                rows.append([jnp.zeros_like(a) for a in rows[0]])
            put(lhs_d, slice(None), slice(2 * g * LANES, (2 * g + 2) * LANES), *rows)

    def down(products):
        ys = assemble({p: block_product(lhs_d, wd, p) for p in products})
        return [xb[n] + y for n, y in enumerate(ys)]

    def out_copy(s):
        slot = s % OUT_SLOTS
        return pltpu.make_async_copy(out_v.at[slot], out_hbm.at[seg_rows(s)], sem_out.at[slot])

    def emit(s, x):
        out_v[s % OUT_SLOTS] = x.astype(out_v.dtype)

    feed_memory(mem0)

    def fill(t, carry):
        xs = x_v[seg_rows(t), :].astype(F32)
        feed_tokens(_layernorm(xs))
        attention(ONE)

        @pl.when(t == 0)
        def _():
            start(wg_copies)
            wait(wo_copies)
            start(wu_copies)
            form_operands(wo)

        @pl.when(t == LAG - 1)
        def _():
            start(wd_copies)

        o, = out_proj(ONE)
        ring[t] = xs + o[M:]
        feed_memory(o[:M])
        return o[:M]

    mem1 = lax.fori_loop(0, LAG, fill, mem0)
    feed_memory(mem1, mem0)
    feed_ffn(ring[0], ring[1])
    wait(wg_copies)
    wait(wu_copies)
    form_operands(wgu)
    gate_up(BOTH)
    wait(wd_copies)
    x_tail.start()
    form_operands(wd)
    ring[0], ring[1] = down(BOTH)
    feed_ffn(ring[2])
    gate_up(ONE, keep=True)
    xa[0] = x_v[seg_rows(LAG), :].astype(F32)
    xa[1] = ring[0]
    feed_both(True)

    def step(t, carry, *, use_pre):
        @pl.when(t >= LAG + 2)
        def _():
            out_copy(t - LAG - 2).start()

        @pl.when(t >= LAG + 1 + OUT_SLOTS)
        def _():
            out_copy(t - LAG - 1 - OUT_SLOTS).wait()

        def down_part(products):
            for p in products:
                dacc[p] = block_product(lhs_d, wd, p)

        pre_rows = None
        if use_pre:
            pre_rows = pl.ds(pl.multiple_of((t - LAG) * PRE_ROWS, PRE_ROWS), PRE_ROWS)
        attention(BOTH, (lambda: down_part((0, 1)), lambda: down_part((2,))), pre_rows)
        o1, o2 = out_proj(BOTH)
        m = {p: dacc[p] if p < 3 else block_product(lhs_d, wd, p) for p in BOTH}
        y1, y2 = assemble(m)
        x1, x2 = xb[0] + y1, xb[1] + y2
        feed_memory(o1[:M], o2[:M])
        feed_ffn(xa[0] + o1[M:], xa[1] + o2[M:])
        ring[(t - 1) % RING] = x1
        emit(jnp.maximum(t - LAG - 1, 0), x2)
        xa[0] = x_v[seg_rows(jnp.minimum(t + 1, n_seg - 1)), :].astype(F32)
        xa[1] = ring[(t + 1 - LAG) % RING]
        feed_both(use_pre)
        gate_up(BOTH)
        return o2[:M]

    lax.fori_loop(LAG, LAG + PRE_STEPS, functools.partial(step, use_pre=True), mem0)
    x_tail.wait()
    feed_both(False)
    mem2 = lax.fori_loop(LAG + PRE_STEPS, n_seg, functools.partial(step, use_pre=False), mem0)

    tail = n_seg - LAG
    out_copy(tail - 2).start()
    out_copy(tail - 1 - OUT_SLOTS).wait()
    ring[(n_seg - 1) % RING], x2 = down(BOTH)
    emit(tail - 1, x2)
    out_copy(tail - 1).start()
    feed_memory(mem2)

    def drain(s, carry):
        xs = ring[s % RING]
        feed_tokens(_layernorm(xs))
        attention(ONE)
        o, = out_proj(ONE)
        ring[s % RING] = xs + o[M:]
        feed_memory(o[:M])
        return carry

    lax.fori_loop(tail, n_seg, drain, 0)
    for s in range(tail, n_seg):
        out_copy(s - OUT_SLOTS).wait()
    feed_ffn(ring[tail % RING], ring[(tail + 1) % RING])
    gate_up(BOTH)
    for n, x in enumerate(down(BOTH)):
        emit(tail + n, x)
    start([out_copy(tail), out_copy(tail + 1)])
    feed_ffn(ring[(tail + 2) % RING])
    gate_up(ONE)
    emit(tail + 2, down(ONE)[0])
    out_copy(tail + 2).start()
    wait([out_copy(s) for s in range(n_seg - OUT_SLOTS, n_seg)])


@functools.partial(jax.jit, static_argnames=("A_seg_len",))
def pallas_interleave_layers__memory_aug_recurrent_mem_tr__glu_gated_glu__prompt_kernel(
    A_x, A_mem0, A_Wq, A_Wk, A_Wv, A_Wo, A_seg_len, B_x, B_w_gate, B_w_up, B_w_down,
):
    del B_x
    B, S, D = A_x.shape
    M = A_mem0.shape[1]
    _, H, Dh = A_Wq.shape
    F = B_w_gate.shape[1]
    seg = int(A_seg_len)
    assert B == 1 and S % seg == 0 and Dh == LANES and D == 2 * GROUP * LANES
    L, half, n_ff, n_pre = M + seg, D // 2, F // (2 * LANES), PRE_STEPS * PRE_ROWS
    hbm = pl.BlockSpec(memory_space=pl.ANY)
    out = pl.pallas_call(
        functools.partial(_kernel, seg=seg),
        out_shape=jax.ShapeDtypeStruct((S, D), A_x.dtype),
        in_specs=[hbm, pl.BlockSpec(memory_space=pltpu.VMEM)] + [hbm] * 7,
        out_specs=hbm,
        scratch_shapes=[
            pltpu.VMEM((S, D), BF16),
            pltpu.VMEM((OUT_SLOTS, seg, D), A_x.dtype),
            pltpu.VMEM((RAW_SLOTS, 2, LANES * H, Dh), BF16),
            pltpu.VMEM((3, 7, H // 2, half, LANES), BF16),
            pltpu.VMEM((7, GROUP, H // 2, Dh, LANES), BF16),
            pltpu.VMEM((7, 2 * n_ff, half, LANES), BF16),
            pltpu.VMEM((7, GROUP, n_ff, LANES, LANES), BF16),
            pltpu.VMEM((7, L, half), F32),
            pltpu.VMEM((7, L, H * Dh // 2), F32),
            pltpu.VMEM((7, seg, half), BF16),
            pltpu.VMEM((7, seg, F // 2), BF16),
            pltpu.VMEM((3, seg, half), F32),
            pltpu.VMEM((2, seg, D), F32),
            pltpu.VMEM((2, seg, D), F32),
            pltpu.VMEM((RING, seg, D), F32),
            pltpu.VMEM((2 * L, 2 * L), F32),
            pltpu.VMEM((GROUP, n_pre, 2 * LANES), BF16),
            pltpu.VMEM((3, H // GROUP, n_pre, GROUP * Dh), F32),
            pltpu.SemaphoreType.DMA((2,)),
            pltpu.SemaphoreType.DMA((RAW_SLOTS,)),
            pltpu.SemaphoreType.DMA((3,)),
            pltpu.SemaphoreType.DMA((OUT_SLOTS,)),
        ],
        compiler_params=pltpu.CompilerParams(vmem_limit_bytes=126 * 2**20),
    )(A_x.reshape(S, D), A_mem0.reshape(M, D), A_Wq.reshape(D * H, Dh),
      A_Wk.reshape(D * H, Dh), A_Wv.reshape(D * H, Dh),
      A_Wo.reshape(H // 2, 2, Dh, D), B_w_gate, B_w_up,
      B_w_down.reshape(n_ff, 2, LANES, D))
    return out.reshape(B, S, D)
```

```python
import functools
import itertools

import jax
import jax.numpy as jnp
from jax import lax
import jax.experimental.pallas as pl
import jax.experimental.pallas.tpu as pltpu

F32 = jnp.float32
BF16 = jnp.bfloat16
U32 = jnp.uint32
LANES = 128
LAG = 4
RING = 4
GROUP = 4
PRE_ROWS = 16
PRE_STEPS = 16
X_HEAD = LAG + PRE_STEPS + 1
OUT_SLOTS = 4
B11, B12, B21, B22 = 1, 2, 3, 4
SUMS_ONLY = (0, 5, 6)


def _layernorm(x):
    m = jnp.mean(x, axis=-1, keepdims=True)
    d = x - m
    v = jnp.mean(d * d, axis=-1, keepdims=True)
    return d * lax.rsqrt(v + 1e-5)


def _dot(a, b):
    return lax.dot_general(_from_words(a), _from_words(b), (((1,), (0,)), ((), ())),
                           preferred_element_type=F32)


def _to_words(x):
    return pltpu.bitcast(x.astype(BF16), U32)


def _from_words(x):
    return pltpu.bitcast(x, BF16) if x.dtype == U32 else x


def _weight_sums(*words):
    b11, b12, b21, b22 = (_from_words(b).astype(F32) for b in words)
    sums = {0: b11 + b22, 2: b12 - b22, 3: b21 - b11, 5: b11 + b12, 6: b21 + b22}
    return {p: s.astype(BF16) for p, s in sums.items()}


def _row_sums(a11, a12, a21=None, a22=None):
    if a21 is None:
        return {0: a11, 2: a11, 4: a11 + a12, 6: a12}
    return {0: a11 + a22, 1: a21 + a22, 2: a11, 3: a22,
            4: a11 + a12, 5: a21 - a11, 6: a12 - a22}


def _left(m):
    if 1 not in m:
        return [m[0] - m[4] + m[6]]
    return [m[0] + m[3] - m[4] + m[6], m[1] + m[3]]


def _right(m):
    if 1 not in m:
        return [m[2] + m[4]]
    return [m[2] + m[4], m[0] - m[1] + m[2] + m[5]]


def _run(main, filler=()):
    filler = iter(filler)
    for _ in main:
        next(filler, None)
    for _ in filler:
        pass


def _tile(x, j):
    return x[:, j * LANES:(j + 1) * LANES]


def _kernel(x_hbm, mem0_ref, wq_hbm, wk_hbm, wv_hbm, wo_hbm, wg_hbm, wu_hbm, wd_hbm,
            out_hbm,
            x_v, out_v, wqkv, wo_v, wgu_v, wd_v,
            lhs_h, lhs_o, lhs_b, lhs_d, mem, xa, xb, ring, bias, pre_in, pre,
            sem_x, sem_raw, sem_w, sem_out, *, seg):
    S, D = x_v.shape
    M = mem0_ref.shape[0]
    Dh = LANES
    H = 2 * wo_hbm.shape[0]
    n_seg = S // seg
    L = M + seg
    half = D // 2
    n_kt = half // LANES
    wo, wgu, wd = (ref.bitcast(U32) for ref in (wo_v, wgu_v, wd_v))
    n_ff = wd.shape[2]
    n_groups = H // (2 * GROUP)
    scale = Dh ** -0.5
    ONE, BOTH = (0, 2, 4, 6), (0, 1, 2, 3, 4, 5, 6)

    def seg_rows(s, n=1):
        start = s * seg
        return pl.ds(start if isinstance(start, int) else pl.multiple_of(start, seg), n * seg)

    x_head = pltpu.make_async_copy(
        x_hbm.at[seg_rows(0, X_HEAD)], x_v.at[seg_rows(0, X_HEAD)], sem_x.at[0])
    x_tail = pltpu.make_async_copy(
        x_hbm.at[seg_rows(X_HEAD, n_seg - X_HEAD)],
        x_v.at[seg_rows(X_HEAD, n_seg - X_HEAD)], sem_x.at[1])

    n_raw = LANES * H // half

    def raw_slot(n):
        k = n % len(SUMS_ONLY)
        return jnp.where(k == 0, SUMS_ONLY[0], SUMS_ONLY[1] + k - 1)

    def raw_copies(n, src):
        return [pltpu.make_async_copy(
            src.at[pl.ds((n // 3 + a * n_kt) * n_raw, n_raw)],
            wgu_v.at[raw_slot(n), pl.ds(a * n_raw, n_raw)],
            sem_raw.at[n % len(SUMS_ONLY)]) for a in range(2)]

    def start_raw(n):
        for i, src in enumerate((wq_hbm, wk_hbm, wv_hbm)):
            @pl.when(n % 3 == i)
            def _():
                for cp in raw_copies(n, src):
                    cp.start()

    blocks = ((B11, 0, 0), (B12, 0, 1), (B21, 1, 0), (B22, 1, 1))

    def proj_copies(src, dst, sem):
        return [pltpu.make_async_copy(
            src.at[:, a, :, pl.ds((b * n_kt + j) * LANES, LANES)], dst.at[p, j], sem)
            for p, a, b in blocks for j in range(n_kt)]

    def ffn_slot(pair, up):
        return (pair // 2) * GROUP + 2 * up + pair % 2

    def ffn_copies(src, up, sem):
        return [pltpu.make_async_copy(
            src.at[pl.ds(a * half, half), pl.ds((2 * j + b) * LANES, LANES)],
            wgu_v.at[p, ffn_slot(j, up)], sem)
            for p, a, b in blocks for j in range(n_ff)]

    wo_copies = proj_copies(wo_hbm, wo_v, sem_w.at[0])
    wg_copies = ffn_copies(wg_hbm, 0, sem_w.at[1])
    wu_copies = ffn_copies(wu_hbm, 1, sem_w.at[2])
    wd_copies = proj_copies(wd_hbm, wd_v, sem_w.at[3])

    def start(copies):
        for cp in copies:
            cp.start()

    def wait(copies):
        for cp in copies:
            cp.wait()

    def form_operands(w, w_v):
        def body(j, carry):
            blocks = range(w.shape[2] if w.ndim == 5 else n_kt)
            src = [k if w.ndim == 5 else pl.ds(k * LANES // 2, LANES // 2) for k in blocks]
            raw = [[w[p, j, k] for p in (B11, B12, B21, B22)] for k in src]
            for k in blocks:
                for p, s in _weight_sums(*raw[k]).items():
                    w_v[p, j, k if w.ndim == 5 else pl.ds(k * LANES, LANES)] = s
            return carry
        lax.fori_loop(0, w.shape[1], body, 0)

    x_head.start()
    start(raw_copies(0, wq_hbm))

    r = lax.broadcasted_iota(jnp.int32, (2 * L, 2 * L), 0)
    c = lax.broadcasted_iota(jnp.int32, (2 * L, 2 * L), 1)
    visible = (r < M) | ((r >= L) & (r < L + M)) | (r >= c)
    bias[...] = jnp.where((r >= L) == (c >= L),
                          jnp.where(visible, 0.0, -1e9), -jnp.inf).astype(F32)

    pre[...] = jnp.zeros(pre.shape, F32)
    x_head.wait()
    start(raw_copies(1, wk_hbm))
    for n in range(PRE_STEPS):
        first = (LAG + n) * seg
        hs = _to_words(_layernorm(x_v[first:first + PRE_ROWS, :].astype(F32)))
        for j in range(n_kt):
            pre_in[j, n * PRE_ROWS // 2:(n + 1) * PRE_ROWS // 2, :] = jnp.concatenate(
                [_tile(hs, j), _tile(hs, j + n_kt)], axis=1)

    def relayout(n, carry):
        slot, i, kt = raw_slot(n), n % 3, n // 3
        wait(raw_copies(n, wq_hbm))

        @pl.when(n + 2 < 3 * n_kt)
        def _():
            start_raw(n + 2)

        @pl.when(n + 2 == 3 * n_kt)
        def _():
            start(wo_copies)

        rows = pl.ds(pl.multiple_of(kt * (LANES // 2), LANES // 2), LANES // 2)
        for g in range(H // GROUP):
            tiles = []
            for j in range(g * GROUP // 2, (g + 1) * GROUP // 2):
                b = []
                for a in range(2):
                    even, odd = (jnp.concatenate(
                        [wgu[slot, a * n_raw + piece, pl.ds(row, half // (2 * H), stride=H), :]
                         for piece in range(n_raw)], axis=0) for row in (j, H // 2 + j))
                    b.append((even & 0xFFFF) | (odd << 16))
                    b.append((even >> 16) | (odd & jnp.uint32(0xFFFF0000)))
                wqkv[i, B11, j, rows, :] = b[0]
                wqkv[i, B22, j, rows, :] = b[3]
                for p, s in _weight_sums(*b).items():
                    wqkv[i, p, j, rows, :] = _to_words(s)
                tiles += [jnp.concatenate([b[0], b[2]], axis=0),
                          jnp.concatenate([b[1], b[3]], axis=0)]
            pre[i, g] += _dot(pre_in[kt], jnp.concatenate(tiles, axis=1))
        return carry

    lax.fori_loop(0, 3 * n_kt, relayout, 0)

    mem0 = mem0_ref[...].astype(F32)

    def put(dst, rows, cols, top, bottom=None):
        sums = _row_sums(*top, *(bottom or ()))
        for p in sums:
            dst[p, rows, cols] = _to_words(sums[p]) if dst.dtype == U32 else sums[p]

    def halves(x):
        return x[:, :half], x[:, half:]

    def feed_memory(*mems):
        put(lhs_h, slice(0, M), slice(None), *map(halves, mems))

    def feed_tokens(*hs):
        put(lhs_h, slice(M, M + hs[0].shape[0]), slice(None), *map(halves, hs))

    def feed_both(use_pre):
        h2 = _layernorm(xa[1])
        if use_pre:
            h1 = _layernorm(xa[0, PRE_ROWS:, :])
            cut = PRE_ROWS // 2
            feed_tokens(jnp.concatenate([h1, h2[:cut]], axis=0), h2[cut:])
        else:
            feed_tokens(_layernorm(xa[0]), h2)

    def feed_ffn(*xs):
        for n, x in enumerate(xs):
            xb[n] = x
        put(lhs_b, slice(None), slice(None), *(halves(_layernorm(x)) for x in xs))

    def attention(products, pre_rows=None, filler=()):
        filler = iter(filler)
        n_rows = L if pre_rows is None else L - PRE_ROWS // 2
        total = L if products is ONE else 2 * L

        def project(g, i):
            if g == n_groups:
                return next(filler, None)
            m = {}
            for p in products:
                m[p] = _dot(lhs_h[p, 0:n_rows, :], jnp.concatenate(
                    [wqkv[i, p, g * GROUP + j] for j in range(GROUP)], axis=1))
                yield
            heads = []
            for j in range(GROUP):
                for b, side in enumerate((_left(m), _right(m))):
                    parts = [_tile(y, j) for y in side]
                    if pre_rows is not None:
                        head = 2 * (g * GROUP + j) + b
                        col = head % GROUP * Dh
                        parts = [parts[0][:M], pre[i, head // GROUP, pre_rows, col:col + Dh],
                                 parts[0][M:L - PRE_ROWS], parts[1][:M],
                                 parts[0][L - PRE_ROWS:], parts[1][M:]]
                    heads.append(jnp.concatenate(parts, axis=0).astype(BF16))
            return heads

        def probabilities(q, k):
            s = lax.dot_general(q, k, (((1,), (1,)), ((), ())), preferred_element_type=F32)
            b = bias[0:total, 0:total]
            s = jnp.where(b == 0.0, s * scale, b)
            e = jnp.exp(s - jnp.max(s, axis=-1, keepdims=True))
            return (e * (1.0 / jnp.sum(e, axis=-1, keepdims=True))).astype(BF16)

        def mix(g, probs, v, pairs):
            for j in pairs:
                o = [_dot(probs[2 * j + b], v[2 * j + b]) for b in range(2)]
                col = (g * GROUP + j) * Dh
                put(lhs_o, slice(None), slice(col, col + Dh),
                    *((o[0][at:at + L], o[1][at:at + L]) for at in range(0, total, L)))

        q = yield from project(0, 0)
        k = yield from project(0, 1)
        v = yield from project(0, 2)
        for g in range(n_groups):
            probs = [probabilities(a, b) for a, b in zip(q[:GROUP], k[:GROUP])]
            q_next = yield from project(g + 1, 0)
            mix(g, probs, v, range(GROUP // 2))
            probs += [probabilities(a, b) for a, b in zip(q[GROUP:], k[GROUP:])]
            k_next = yield from project(g + 1, 1)
            mix(g, probs, v, range(GROUP // 2, GROUP))
            q, k = q_next, k_next
            v = yield from project(g + 1, 2)
        yield

    def block_product(lhs, w, p, lo=0, hi=None):
        hi = w.shape[2] if hi is None else hi
        tiles = [w[p, j, lo:hi].reshape((hi - lo) * LANES // 2, LANES) for j in range(n_kt)]
        return _dot(lhs[p, :, lo * LANES:hi * LANES], jnp.concatenate(tiles, axis=1))

    def assemble(m):
        return [jnp.concatenate(lr, axis=1) for lr in zip(_left(m), _right(m))]

    def project_out(lhs, w, products, done):
        m = {}
        for p in products:
            m[p] = block_product(lhs, w, p)
            yield
        done(*assemble(m))

    def gate_up():
        for g in range(n_ff // 2):
            m = {}
            for p in BOTH:
                m[p] = _dot(lhs_b[p], jnp.concatenate(
                    [wgu[p, g * GROUP + j] for j in range(GROUP)], axis=1))
                yield
            act = [[jax.nn.sigmoid(y[:, :2 * LANES]) * y[:, 2 * LANES:] for y in side]
                   for side in (_left(m), _right(m))]
            put(lhs_d, slice(None), slice(2 * g * LANES, (2 * g + 2) * LANES), *zip(*act))

    def down(done):
        x = xb[0], xb[1]
        return project_out(lhs_d, wd, BOTH, lambda *y: done(x[0] + y[0], x[1] + y[1]))

    def single(s, xs):
        def done(o):
            ring[s % RING] = xs + o[M:]
            mem[0] = o[:M]
            feed_memory(o[:M])

        feed_tokens(_layernorm(xs))
        yield from attention(ONE)
        yield from project_out(lhs_o, wo, ONE, done)

    def out_copy(s):
        slot = s % OUT_SLOTS
        return pltpu.make_async_copy(out_v.at[slot], out_hbm.at[seg_rows(s)], sem_out.at[slot])

    def emit(s, x):
        out_v[s % OUT_SLOTS] = x.astype(out_v.dtype)

    def first(s):
        return single(s, x_v[seg_rows(s), :].astype(F32))

    def keep(*slots):
        def done(*xs):
            for s, x in zip(slots, xs):
                ring[s] = x
        return done

    def fill(s, carry):
        stages = first(s)
        _run(itertools.islice(stages, 3 * n_groups * len(ONE) + 1))

        @pl.when(s == 0)
        def _():
            wait(wo_copies)
            form_operands(wo, wo_v)

        @pl.when(s == 1)
        def _():
            start(wu_copies)

        @pl.when(s == 2)
        def _():
            start(wd_copies)

        _run(stages)
        return carry

    feed_memory(mem0)
    start(wg_copies)
    lax.fori_loop(0, LAG, fill, 0)
    feed_memory(mem[0], mem0)
    feed_ffn(ring[0], ring[1])
    wait(wg_copies)
    wait(wu_copies)
    form_operands(wgu, wgu_v)
    wait(wd_copies)
    x_tail.start()
    form_operands(wd, wd_v)
    _run(gate_up())
    projected = down(keep(0, 1))
    feed_ffn(ring[3], ring[2])
    _run(projected)
    xa[0] = x_v[seg_rows(LAG), :].astype(F32)
    xa[1] = ring[0]
    feed_both(True)
    _run(gate_up())

    def step(t, carry, *, use_pre):
        @pl.when(t >= LAG + 2)
        def _():
            out_copy(t - LAG - 2).start()

        @pl.when(t >= LAG + 1 + OUT_SLOTS)
        def _():
            out_copy(t - LAG - 1 - OUT_SLOTS).wait()

        def attended(o1, o2):
            mem[0] = o2[:M]
            feed_memory(o1[:M], o2[:M])
            feed_ffn(xa[0] + o1[M:], xa[1] + o2[M:])
            xa[0] = x_v[seg_rows(jnp.minimum(t + 1, n_seg - 1)), :].astype(F32)
            xa[1] = ring[(t + 1 - LAG) % RING]
            feed_both(use_pre)

        def gated(x1, x2):
            ring[(t - 1) % RING] = x1
            ring[jnp.where(t == LAG, LAG - 2, RING)] = x2
            emit(jnp.maximum(t - LAG - 1, 0), x2)

        pre_rows = None
        if use_pre:
            pre_rows = pl.ds(pl.multiple_of((t - LAG) * PRE_ROWS, PRE_ROWS), PRE_ROWS)
        projected = down(gated)
        _run(attention(BOTH, pre_rows, projected))
        _run(project_out(lhs_o, wo, BOTH, attended))
        _run(projected)
        _run(gate_up())
        return carry

    lax.fori_loop(LAG, LAG + PRE_STEPS, functools.partial(step, use_pre=True), 0)
    x_tail.wait()
    feed_both(False)
    lax.fori_loop(LAG + PRE_STEPS, n_seg, functools.partial(step, use_pre=False), 0)

    tail = n_seg - LAG

    def finish(x1, x2):
        ring[(n_seg - 1) % RING] = x1
        emit(tail - 1, x2)

    def drain(s, carry):
        _run(single(s, ring[s % RING]))
        return carry

    def drain_ffn(n, carry):
        def done(*xs):
            for k, x in enumerate(xs):
                emit(s + k, x)

        s = tail + 2 * n
        feed_ffn(ring[s % RING], ring[(s + 1) % RING])
        _run(gate_up())
        _run(down(done))
        start([out_copy(s), out_copy(s + 1)])
        return carry

    out_copy(tail - 2).start()
    out_copy(tail - 1 - OUT_SLOTS).wait()
    _run(down(finish))
    out_copy(tail - 1).start()
    feed_memory(mem[0])
    lax.fori_loop(tail, n_seg, drain, 0)
    wait([out_copy(s) for s in range(tail - OUT_SLOTS, tail)])
    lax.fori_loop(0, LAG // 2, drain_ffn, 0)
    wait([out_copy(s) for s in range(tail, n_seg)])


@functools.partial(jax.jit, static_argnames=("A_seg_len",))
def pallas_interleave_layers__memory_aug_recurrent_mem_tr__glu_gated_glu__prompt_kernel(
    A_x, A_mem0, A_Wq, A_Wk, A_Wv, A_Wo, A_seg_len, B_x, B_w_gate, B_w_up, B_w_down,
):
    del B_x
    B, S, D = A_x.shape
    M = A_mem0.shape[1]
    _, H, Dh = A_Wq.shape
    F = B_w_gate.shape[1]
    seg = int(A_seg_len)
    assert B == 1 and S % seg == 0 and Dh == LANES and D == 2 * GROUP * LANES
    L, half, n_ff, n_pre = M + seg, D // 2, F // (2 * LANES), PRE_STEPS * PRE_ROWS
    hbm = pl.BlockSpec(memory_space=pl.ANY)
    out = pl.pallas_call(
        functools.partial(_kernel, seg=seg),
        out_shape=jax.ShapeDtypeStruct((S, D), A_x.dtype),
        in_specs=[hbm, pl.BlockSpec(memory_space=pltpu.VMEM)] + [hbm] * 7,
        out_specs=hbm,
        scratch_shapes=[
            pltpu.VMEM((S, D), BF16),
            pltpu.VMEM((OUT_SLOTS, seg, D), A_x.dtype),
            pltpu.VMEM((3, 7, H // 2, half // 2, LANES), U32),
            pltpu.VMEM((7, GROUP, H // 2, Dh, LANES), BF16),
            pltpu.VMEM((7, 2 * n_ff, half, LANES), BF16),
            pltpu.VMEM((7, GROUP, n_ff, LANES, LANES), BF16),
            pltpu.VMEM((7, L, half), F32),
            pltpu.VMEM((7, L, H * Dh // 2), F32),
            pltpu.VMEM((7, seg // 2, half), U32),
            pltpu.VMEM((7, seg // 2, F // 2), U32),
            pltpu.VMEM((1, M, D), F32),
            pltpu.VMEM((2, seg, D), F32),
            pltpu.VMEM((2, seg, D), F32),
            pltpu.VMEM((RING + 1, seg, D), F32),
            pltpu.VMEM((2 * L, 2 * L), F32),
            pltpu.VMEM((GROUP, n_pre // 2, 2 * LANES), U32),
            pltpu.VMEM((3, H // GROUP, n_pre, GROUP * Dh), F32),
            pltpu.SemaphoreType.DMA((2,)),
            pltpu.SemaphoreType.DMA((len(SUMS_ONLY),)),
            pltpu.SemaphoreType.DMA((4,)),
            pltpu.SemaphoreType.DMA((OUT_SLOTS,)),
        ],
        compiler_params=pltpu.CompilerParams(vmem_limit_bytes=127 * 2**20),
    )(A_x.reshape(S, D), A_mem0.reshape(M, D), A_Wq.reshape(-1, half, Dh),
      A_Wk.reshape(-1, half, Dh), A_Wv.reshape(-1, half, Dh),
      A_Wo.reshape(H // 2, 2, Dh, D), B_w_gate, B_w_up,
      B_w_down.reshape(n_ff, 2, LANES, D))
    return out.reshape(B, S, D)
```

```python
import functools
import itertools

import jax
import jax.numpy as jnp
from jax import lax
import jax.experimental.pallas as pl
import jax.experimental.pallas.tpu as pltpu

F32 = jnp.float32
BF16 = jnp.bfloat16
U32 = jnp.uint32
LANES = 128
LAG = 4
RING = 4
GROUP = 4
HEAD_QUADS = 2
PRE_ROWS = 16
PRE_STEPS = 16
X_HEAD = LAG + PRE_STEPS + 1
OUT_SLOTS = 4
UNROLL = 1
B11, B12, B21, B22 = 1, 2, 3, 4
SUMS_ONLY = (0, 5, 6)


def _layernorm(x):
    m = jnp.mean(x, axis=-1, keepdims=True)
    d = x - m
    v = jnp.mean(d * d, axis=-1, keepdims=True)
    return d * lax.rsqrt(v + 1e-5)


def _dot(a, b):
    return lax.dot_general(_from_words(a), _from_words(b), (((1,), (0,)), ((), ())),
                           preferred_element_type=F32)


def _to_words(x):
    return pltpu.bitcast(x.astype(BF16), U32)


def _from_words(x):
    return pltpu.bitcast(x, BF16) if x.dtype == U32 else x


def _weight_sums(*words):
    b11, b12, b21, b22 = (_from_words(b).astype(F32) for b in words)
    sums = {0: b11 + b22, 2: b12 - b22, 3: b21 - b11, 5: b11 + b12, 6: b21 + b22}
    return {p: s.astype(BF16) for p, s in sums.items()}


def _row_sums(a11, a12, a21, a22):
    return (a11 + a22, a21 + a22, a11, a22, a11 + a12, a21 - a11, a12 - a22)


def _left(m):
    return m[0] + m[3] - m[4] + m[6], m[1] + m[3]


def _right(m):
    return m[2] + m[4], m[0] - m[1] + m[2] + m[5]


QUAD = 4
C = (-1.5, -0.5, 0.5, 1.5)
PAIRS = tuple(itertools.combinations(range(QUAD), 2))
N_QUAD = QUAD * QUAD + QUAD + len(PAIRS)


def _quad_weight_sums(w):
    w = [[_from_words(b).astype(F32) for b in row] for row in w]
    sums = {}
    for i in range(QUAD):
        others = [j for j in range(QUAD) if j != i]
        sums[QUAD * i + i] = functools.reduce(jnp.add, [w[i][j] for j in others], w[i][i])
        sums[QUAD * QUAD + i] = functools.reduce(
            jnp.subtract, [w[j][i] for j in others], w[i][i])
    for n, (i, j) in enumerate(PAIRS):
        sums[QUAD * QUAD + QUAD + n] = w[i][j] + w[j][i]
    return {p: s.astype(BF16) for p, s in sums.items()}


def _times(c, x):
    return x if c == 1 else c * x


def _quad_row_sums(*rows):
    p = rows[-1]
    sums = {QUAD * i + i: p[i] for i in range(QUAD)}
    if len(rows) == 2:
        q = [rows[0][i] - C[i] * p[i] for i in range(QUAD)]
        sums.update({QUAD * QUAD + i: q[i] for i in range(QUAD)})
        for n, (i, j) in enumerate(PAIRS):
            both = q[i] + q[j]
            sums[QUAD * QUAD + QUAD + n] = both
            sums[QUAD * i + j] = both - _times(C[j] - C[i], p[i])
            sums[QUAD * j + i] = both + _times(C[j] - C[i], p[j])
    return sums


def _quad_product(product, n_layers):
    u = [product(QUAD * i + i, QUAD * i + i) for i in range(QUAD)]
    if n_layers == 1:
        for i, j in PAIRS:
            t = product(QUAD * j + j, QUAD * j + i) - product(QUAD * i + i, QUAD * i + j)
            u[i], u[j] = u[i] + t, u[j] - t
        return [u]
    v = [product(QUAD * QUAD + i, QUAD * QUAD + i) for i in range(QUAD)]
    for n, (i, j) in enumerate(PAIRS):
        m_ji, m_ij, m0 = (product(s, s) for s in (
            QUAD * j + i, QUAD * i + j, QUAD * QUAD + QUAD + n))
        t = _times(1 / (C[j] - C[i]), m_ji + m_ij - m0)
        u[i], u[j] = u[i] + t, u[j] - t
        v[i], v[j] = v[i] + m_ji, v[j] + m_ij
    return [[v[i] + C[i] * u[i] for i in range(QUAD)], u]


def _run(stages, n=None):
    for _ in itertools.islice(stages, n):
        pass


def _tile(x, j):
    return x[:, j * LANES:(j + 1) * LANES]


def _kernel(x_hbm, mem0_ref, wq_hbm, wk_hbm, wv_hbm, wo_hbm, wg_hbm, wu_hbm, wd_hbm,
            out_hbm,
            x_v, out_v, wqkv, wo_v, wgu_v, wd_v,
            lhs_h, lhs_o, lhs_b, lhs_d, early, mem, xa, xb, ring, bias, pre_in, pre,
            sem_x, sem_raw, sem_w, sem_out, *, seg):
    S, D = x_v.shape
    M = mem0_ref.shape[0]
    Dh = LANES
    H = QUAD * wo_hbm.shape[0]
    quarter = D // QUAD
    n_seg = S // seg
    L = M + seg
    half = D // 2
    n_kt = half // LANES
    wo, wgu, wd = (ref.bitcast(U32) for ref in (wo_v, wgu_v, wd_v))
    n_ff = wd.shape[2]
    n_groups = H // (QUAD * HEAD_QUADS)
    scale = Dh ** -0.5

    def seg_rows(s, n=1):
        start = s * seg
        return pl.ds(start if isinstance(start, int) else pl.multiple_of(start, seg), n * seg)

    x_head = pltpu.make_async_copy(
        x_hbm.at[seg_rows(0, X_HEAD)], x_v.at[seg_rows(0, X_HEAD)], sem_x.at[0])
    x_tail = pltpu.make_async_copy(
        x_hbm.at[seg_rows(X_HEAD, n_seg - X_HEAD)],
        x_v.at[seg_rows(X_HEAD, n_seg - X_HEAD)], sem_x.at[1])

    raw_rows = quarter // n_kt
    n_raw = raw_rows * H // half

    def raw_slot(n):
        k = n % len(SUMS_ONLY)
        return jnp.where(k == 0, SUMS_ONLY[0], SUMS_ONLY[1] + k - 1)

    def raw_copies(n, src):
        return [pltpu.make_async_copy(
            src.at[pl.ds((n // 3 + a * n_kt) * n_raw, n_raw)],
            wgu_v.at[raw_slot(n), pl.ds(a * n_raw, n_raw)],
            sem_raw.at[n % len(SUMS_ONLY)]) for a in range(QUAD)]

    def start_raw(n):
        for i, src in enumerate((wq_hbm, wk_hbm, wv_hbm)):
            @pl.when(n % 3 == i)
            def _():
                for cp in raw_copies(n, src):
                    cp.start()

    blocks = ((B11, 0, 0), (B12, 0, 1), (B21, 1, 0), (B22, 1, 1))

    def proj_copies(src, dst, sem):
        return [pltpu.make_async_copy(
            src.at[:, a, :, pl.ds((b * n_kt + j) * LANES, LANES)], dst.at[p, j], sem)
            for p, a, b in blocks for j in range(n_kt)]

    def ffn_slot(pair, up):
        return (pair // 2) * GROUP + 2 * up + pair % 2

    def ffn_copies(src, up, sem):
        return [pltpu.make_async_copy(
            src.at[pl.ds(a * half, half), pl.ds((2 * j + b) * LANES, LANES)],
            wgu_v.at[p, ffn_slot(j, up)], sem)
            for p, a, b in blocks for j in range(n_ff)]

    wo_copies = [pltpu.make_async_copy(
        wo_hbm.at[:, a, :, pl.ds(b * quarter + j * LANES, LANES)],
        wo_v.at[QUAD * a + b, j], sem_w.at[0])
        for a in range(QUAD) for b in range(QUAD) for j in range(quarter // LANES)]
    wg_copies = ffn_copies(wg_hbm, 0, sem_w.at[1])
    wu_copies = ffn_copies(wu_hbm, 1, sem_w.at[2])
    wd_copies = proj_copies(wd_hbm, wd_v, sem_w.at[3])

    def start(copies):
        for cp in copies:
            cp.start()

    def wait(copies):
        for cp in copies:
            cp.wait()

    def form_operands(w, w_v):
        def body(j, carry):
            blocks = range(w.shape[2] if w.ndim == 5 else n_kt)
            src = [k if w.ndim == 5 else pl.ds(k * LANES // 2, LANES // 2) for k in blocks]
            raw = [[w[p, j, k] for p in (B11, B12, B21, B22)] for k in src]
            for k in blocks:
                for p, s in _weight_sums(*raw[k]).items():
                    w_v[p, j, k if w.ndim == 5 else pl.ds(k * LANES, LANES)] = s
            return carry
        lax.fori_loop(0, w.shape[1], body, 0)

    x_head.start()
    start(raw_copies(0, wq_hbm))

    r = lax.broadcasted_iota(jnp.int32, (2 * L, 2 * L), 0)
    c = lax.broadcasted_iota(jnp.int32, (2 * L, 2 * L), 1)
    visible = (r < M) | ((r >= L) & (r < L + M)) | (r >= c)
    bias[...] = jnp.where((r >= L) == (c >= L),
                          jnp.where(visible, 0.0, -1e9), -jnp.inf).astype(F32)

    pre[...] = jnp.zeros(pre.shape, F32)
    x_head.wait()
    start(raw_copies(1, wk_hbm))
    for n in range(PRE_STEPS):
        first = (LAG + n) * seg
        hs = (_layernorm(x_v[first:first + PRE_ROWS, :].astype(F32)))
        for j in range(n_kt):
            pre_in[j, n * PRE_ROWS // 2:(n + 1) * PRE_ROWS // 2, :] = _to_words(
                jnp.concatenate([hs[:, a * quarter + j * raw_rows:][:, :raw_rows]
                                 for a in range(QUAD)], axis=1))

    def relayout(n, carry):
        slot, i, kt = raw_slot(n), n % 3, n // 3
        wait(raw_copies(n, wq_hbm))

        @pl.when(n + 2 < 3 * n_kt)
        def _():
            start_raw(n + 2)

        @pl.when(n + 2 == 3 * n_kt)
        def _():
            start(wo_copies)

        rows = pl.ds(pl.multiple_of(kt * (raw_rows // 2), raw_rows // 2), raw_rows // 2)
        for g in range(H // QUAD):
            w = []
            for a in range(QUAD):
                w.append([])
                for j in range(g * QUAD // 2, (g + 1) * QUAD // 2):
                    even, odd = (jnp.concatenate(
                        [wgu[slot, a * n_raw + piece, pl.ds(row, half // (2 * H), stride=H), :]
                         for piece in range(n_raw)], axis=0) for row in (j, H // 2 + j))
                    w[a].append((even & 0xFFFF) | (odd << 16))
                    w[a].append((even >> 16) | (odd & jnp.uint32(0xFFFF0000)))
            for a, b in itertools.permutations(range(QUAD), 2):
                wqkv[i, QUAD * a + b, g, rows, :] = w[a][b]
            for p, s in _quad_weight_sums(w).items():
                wqkv[i, p, g, rows, :] = _to_words(s)
            pre[i, g] += _dot(pre_in[kt], jnp.concatenate(
                [jnp.concatenate(row, axis=1) for row in w], axis=0))
        return carry

    lax.fori_loop(0, 3 * n_kt, relayout, 0)

    mem0 = mem0_ref[...].astype(F32)

    def put(dst, cols, top, bottom):
        for p, s in enumerate(_row_sums(*top, *bottom)):
            dst[p, :, cols] = _to_words(s)

    def halves(x):
        return x[:, :half], x[:, half:]

    def feed(rows, *hs):
        sums = _quad_row_sums(
            *([h[:, a * quarter:(a + 1) * quarter] for a in range(QUAD)] for h in hs))
        for p, s in sums.items():
            lhs_h[p, rows, :] = s

    def feed_memory(*mems):
        feed(slice(0, M), *mems)

    def feed_tokens(*hs):
        feed(slice(M, M + hs[0].shape[0]), *hs)

    def feed_both(use_pre):
        h2 = _layernorm(xa[1])
        if use_pre:
            h1 = _layernorm(xa[0, PRE_ROWS:, :])
            cut = PRE_ROWS // 2
            feed_tokens(jnp.concatenate([h1, h2[:cut]], axis=0), h2[cut:])
        else:
            feed_tokens(_layernorm(xa[0]), h2)

    def feed_ffn():
        put(lhs_b, slice(None), *(halves(_layernorm(xb[n])) for n in range(2)))

    def attention(n_layers, filler, pre_rows=None, midway=()):
        n_rows = L if pre_rows is None else L - PRE_ROWS // 2
        total = n_layers * L

        def project(g, i):
            if g == n_groups:
                return _run(filler, 1)
            quads = range(g * HEAD_QUADS, (g + 1) * HEAD_QUADS)
            ys = _quad_product(lambda a, w: _dot(lhs_h[a, 0:n_rows, :], jnp.concatenate(
                [wqkv[i, w, quad] for quad in quads], axis=1)), n_layers)
            heads = []
            for j, quad in enumerate(quads):
                for b in range(QUAD):
                    parts = [_tile(y[b], j) for y in ys]
                    if pre_rows is not None:
                        parts = [parts[0][:M], pre[i, quad, pre_rows, b * Dh:(b + 1) * Dh],
                                 parts[0][M:L - PRE_ROWS], parts[1][:M],
                                 parts[0][L - PRE_ROWS:], parts[1][M:]]
                    heads.append(jnp.concatenate(parts, axis=0).astype(BF16))
            if i == 2:
                heads = [jnp.concatenate([y, jnp.zeros((LANES - total, Dh), BF16)], axis=0)
                         for y in heads]
            return heads

        def probabilities(q, k):
            s = lax.dot_general(q, k, (((1,), (1,)), ((), ())), preferred_element_type=F32)
            b = bias[0:total, 0:total]
            s = jnp.where(b == 0.0, s * scale, b)
            e = jnp.exp(s - jnp.max(s, axis=-1, keepdims=True))
            p = e * (1.0 / jnp.sum(e, axis=-1, keepdims=True))
            return jnp.concatenate([p, jnp.zeros((total, LANES - total), F32)], axis=1).astype(BF16)

        def mix(quad, probs, v):
            o = [_dot(a, b) for a, b in zip(probs, v)]
            sums = _quad_row_sums(*([y[at:at + L] for y in o] for at in range(0, total, L)))
            for p, s in sums.items():
                lhs_o[p, :, quad * Dh:(quad + 1) * Dh] = s

        q = project(0, 0)
        k = project(0, 1)
        v = project(0, 2)
        _run(midway, 1)
        for g in range(n_groups):
            cut = QUAD * ((HEAD_QUADS + 1) // 2)
            probs = [probabilities(a, b) for a, b in zip(q[:cut], k[:cut])]
            q_next = project(g + 1, 0)
            for j in range(cut // QUAD):
                mix(g * HEAD_QUADS + j, probs[QUAD * j:], v[QUAD * j:][:QUAD])
            probs += [probabilities(a, b) for a, b in zip(q[cut:], k[cut:])]
            k_next = project(g + 1, 1)
            _run(midway, 1)
            for j in range(cut // QUAD, HEAD_QUADS):
                mix(g * HEAD_QUADS + j, probs[QUAD * j:], v[QUAD * j:][:QUAD])
            q, k = q_next, k_next
            v = project(g + 1, 2)

    def out_product(a, w, lo, hi):
        tiles = [wo[w, j, lo:hi].reshape((hi - lo) * Dh // 2, LANES)
                 for j in range(quarter // LANES)]
        return _dot(lhs_o[a, :, lo * Dh:hi * Dh], jnp.concatenate(tiles, axis=1))

    split = H // QUAD - HEAD_QUADS

    def out_early(n_layers):
        slots = range(QUAD * QUAD if n_layers == 1 else N_QUAD)
        for w in slots:
            a = w // QUAD * (QUAD + 1) if n_layers == 1 else w
            early[w] = out_product(a, w, 0, split)
            if w % 4 == 3:
                yield

    def out_proj(n_layers, lo=split):
        def product(a, w):
            y = out_product(a, w, lo, H // QUAD)
            return early[w] + y if lo else y
        return [jnp.concatenate(y, axis=1) for y in _quad_product(product, n_layers)]

    def down():
        m = [_dot(lhs_d[p], jnp.concatenate(
            [wd[p, j].reshape(n_ff * LANES // 2, LANES) for j in range(n_kt)], axis=1))
            for p in range(7)]
        return [xb[n] + jnp.concatenate(y, axis=1)
                for n, y in enumerate(zip(_left(m), _right(m)))]

    def gate_up():
        for g in range(n_ff // 2):
            m = {}
            for p in range(7):
                m[p] = _dot(lhs_b[p], jnp.concatenate(
                    [wgu[p, g * GROUP + j] for j in range(GROUP)], axis=1))
            act = [[jax.nn.sigmoid(y[:, :2 * LANES]) * y[:, 2 * LANES:] for y in side]
                   for side in (_left(m), _right(m))]
            put(lhs_d, slice(2 * g * LANES, (2 * g + 2) * LANES), *zip(*act))

    def ffn():
        feed_ffn()
        gate_up()
        return down()

    def single(s, xs, xs_next, before_out=None):
        filler = () if before_out else out_early(1)
        attention(1, filler)
        _run(filler)
        feed_tokens(_layernorm(xs_next))
        if before_out:
            before_out()
        o, = out_proj(1, 0 if before_out else split)
        ring[s % RING] = xs + o[M:]
        mem[0] = o[:M]
        feed_memory(o[:M])

    def out_copy(s):
        slot = s % OUT_SLOTS
        return pltpu.make_async_copy(out_v.at[slot], out_hbm.at[seg_rows(s)], sem_out.at[slot])

    def emit(s, x):
        out_v[s % OUT_SLOTS] = x.astype(out_v.dtype)

    def tokens(s):
        return x_v[seg_rows(s), :].astype(F32)

    def fill(s, carry):
        @pl.when(s == 1)
        def _():
            start(wu_copies)

        @pl.when(s == 2)
        def _():
            start(wd_copies)

        single(s, tokens(s), tokens(s + 1))
        return carry

    def prepare_wo():
        wait(wo_copies)

        def body(quad, carry):
            for j in range(quarter // LANES):
                w = [[wo[QUAD * a + b, j, quad] for b in range(QUAD)] for a in range(QUAD)]
                for p, s in _quad_weight_sums(w).items():
                    wo_v[p, j, quad] = s
            return carry

        lax.fori_loop(0, H // QUAD, body, 0)

    feed_memory(mem0)
    feed_tokens(_layernorm(tokens(0)))
    start(wg_copies)
    single(0, tokens(0), tokens(1), prepare_wo)
    lax.fori_loop(1, LAG, fill, 0)
    feed_memory(mem[0], mem0)
    xb[0], xb[1] = ring[0], ring[1]
    wait(wg_copies)
    wait(wu_copies)
    form_operands(wgu, wgu_v)
    wait(wd_copies)
    x_tail.start()
    form_operands(wd, wd_v)
    ring[0], ring[1] = ffn()
    xb[0], xb[1] = ring[3], ring[2]
    xa[0] = tokens(LAG)
    xa[1] = ring[0]
    feed_both(True)

    def step(t, use_pre):
        pre_rows = None
        if use_pre:
            pre_rows = pl.ds(pl.multiple_of((t - LAG) * PRE_ROWS, PRE_ROWS), PRE_ROWS)

        def gated():
            gate_up()
            yield
            ring[(t - 1) % RING], x2 = down()
            ring[jnp.where(t == LAG, LAG - 2, RING)] = x2
            emit(jnp.maximum(t - LAG - 1, 0), x2)

        feed_ffn()
        filler = out_early(2)
        attention(2, filler, pre_rows, gated())
        _run(filler)
        a1, a2 = xa[0], xa[1]
        xa[0] = tokens(jnp.minimum(t + 1, n_seg - 1))
        xa[1] = ring[(t + 1 - LAG) % RING]
        feed_both(use_pre)
        o1, o2 = out_proj(2)
        mem[0] = o2[:M]
        feed_memory(o1[:M], o2[:M])
        xb[0], xb[1] = a1 + o1[M:], a2 + o2[M:]

    def steps(first, last, use_pre):
        def body(n, carry):
            t = first + UNROLL * n
            for k in range(UNROLL):
                s = t + k - LAG - 1

                @pl.when(s >= UNROLL)
                def _():
                    out_copy(s - UNROLL).start()

                @pl.when(s >= OUT_SLOTS)
                def _():
                    out_copy(s - OUT_SLOTS).wait()

            for k in range(UNROLL):
                step(t + k, use_pre)
            return carry

        lax.fori_loop(0, (last - first) // UNROLL, body, 0)

    steps(LAG, LAG + PRE_STEPS, True)
    x_tail.wait()
    feed_both(False)
    steps(LAG + PRE_STEPS, n_seg, False)

    tail = n_seg - LAG

    def drain(s, carry):
        single(s, ring[s % RING], ring[(s + 1) % RING])
        return carry

    def drain_ffn(n, carry):
        s = tail + 2 * n
        xb[0], xb[1] = ring[s % RING], ring[(s + 1) % RING]
        for k, x in enumerate(ffn()):
            emit(s + k, x)
        start([out_copy(s), out_copy(s + 1)])
        return carry

    start([out_copy(s) for s in range(tail - 1 - UNROLL, tail - 1)])
    out_copy(tail - 1 - OUT_SLOTS).wait()
    ring[(n_seg - 1) % RING], x2 = ffn()
    emit(tail - 1, x2)
    feed_memory(mem[0])
    feed_tokens(_layernorm(ring[tail % RING]))
    out_copy(tail - 1).start()
    lax.fori_loop(tail, n_seg, drain, 0)
    wait([out_copy(s) for s in range(tail - OUT_SLOTS, tail)])
    lax.fori_loop(0, LAG // 2, drain_ffn, 0)
    wait([out_copy(s) for s in range(tail, n_seg)])


@functools.partial(jax.jit, static_argnames=("A_seg_len",))
def pallas_interleave_layers__memory_aug_recurrent_mem_tr__glu_gated_glu__prompt_kernel(
    A_x, A_mem0, A_Wq, A_Wk, A_Wv, A_Wo, A_seg_len, B_x, B_w_gate, B_w_up, B_w_down,
):
    del B_x
    B, S, D = A_x.shape
    M = A_mem0.shape[1]
    _, H, Dh = A_Wq.shape
    F = B_w_gate.shape[1]
    seg = int(A_seg_len)
    assert B == 1 and S % seg == 0 and Dh == LANES and D == 2 * GROUP * LANES
    L, half, n_ff, n_pre = M + seg, D // 2, F // (2 * LANES), PRE_STEPS * PRE_ROWS
    quarter = D // QUAD
    hbm = pl.BlockSpec(memory_space=pl.ANY)
    out = pl.pallas_call(
        functools.partial(_kernel, seg=seg),
        out_shape=jax.ShapeDtypeStruct((S, D), A_x.dtype),
        in_specs=[hbm, pl.BlockSpec(memory_space=pltpu.VMEM)] + [hbm] * 7,
        out_specs=hbm,
        scratch_shapes=[
            pltpu.VMEM((S, D), BF16),
            pltpu.VMEM((OUT_SLOTS, seg, D), A_x.dtype),
            pltpu.VMEM((3, N_QUAD, H // QUAD, quarter // 2, Dh), U32),
            pltpu.VMEM((N_QUAD, quarter // LANES, H // QUAD, Dh, LANES), BF16),
            pltpu.VMEM((7, 2 * n_ff, half, LANES), BF16),
            pltpu.VMEM((7, GROUP, n_ff, LANES, LANES), BF16),
            pltpu.VMEM((N_QUAD, L, quarter), F32),
            pltpu.VMEM((N_QUAD, L, H * Dh // QUAD), F32),
            pltpu.VMEM((7, seg // 2, half), U32),
            pltpu.VMEM((7, seg // 2, F // 2), U32),
            pltpu.VMEM((N_QUAD, L, quarter), F32),
            pltpu.VMEM((1, M, D), F32),
            pltpu.VMEM((2, seg, D), F32),
            pltpu.VMEM((2, seg, D), F32),
            pltpu.VMEM((RING + 1, seg, D), F32),
            pltpu.VMEM((2 * L, 2 * L), F32),
            pltpu.VMEM((GROUP, n_pre // 2, 2 * LANES), U32),
            pltpu.VMEM((3, H // GROUP, n_pre, GROUP * Dh), F32),
            pltpu.SemaphoreType.DMA((2,)),
            pltpu.SemaphoreType.DMA((len(SUMS_ONLY),)),
            pltpu.SemaphoreType.DMA((4,)),
            pltpu.SemaphoreType.DMA((OUT_SLOTS,)),
        ],
        compiler_params=pltpu.CompilerParams(vmem_limit_bytes=127 * 2**20),
    )(A_x.reshape(S, D), A_mem0.reshape(M, D), A_Wq.reshape(-1, half, Dh),
      A_Wk.reshape(-1, half, Dh), A_Wv.reshape(-1, half, Dh),
      A_Wo.reshape(H // QUAD, QUAD, Dh, D), B_w_gate, B_w_up,
      B_w_down.reshape(n_ff, 2, LANES, D))
    return out.reshape(B, S, D)
```

```python
import functools
import itertools

import jax
import jax.numpy as jnp
from jax import lax
import jax.experimental.pallas as pl
import jax.experimental.pallas.tpu as pltpu

F32 = jnp.float32
BF16 = jnp.bfloat16
U32 = jnp.uint32
LANES = 128
LAG = 4
RING = 4
HEAD_QUADS = 2
RAW_ROWS = 64
RAW_SLOTS = 3
PRE_ROWS = 16
PRE_STEPS = 16
X_HEAD = LAG + PRE_STEPS + 1
OUT_SLOTS = 4
UNROLL = 1

QUAD = 4
C = (-1.5, -0.5, 0.5, 1.5)
PAIRS = tuple(itertools.combinations(range(QUAD), 2))
V_SLOT, PAIR_SLOT = QUAD * QUAD, QUAD * QUAD + QUAD
N_SLOTS = PAIR_SLOT + len(PAIRS)


def _slot(i, j):
    return QUAD * j + i


def _to_words(x):
    return pltpu.bitcast(x.astype(BF16), U32)


def _from_words(x):
    return pltpu.bitcast(x, BF16) if x.dtype == U32 else x


def _weight_sums(w):
    w = [[_from_words(b).astype(F32) for b in row] for row in w]
    sums = {}
    for i in range(QUAD):
        others = [j for j in range(QUAD) if j != i]
        sums[_slot(i, i)] = functools.reduce(jnp.add, [w[i][j] for j in others], w[i][i])
        sums[V_SLOT + i] = functools.reduce(jnp.subtract, [w[j][i] for j in others], w[i][i])
    for n, (i, j) in enumerate(PAIRS):
        sums[PAIR_SLOT + n] = w[i][j] + w[j][i]
    return {p: s.astype(BF16) for p, s in sums.items()}


def _times(c, x):
    return x if c == 1 else c * x


def _put_rows(dst, rows, cols, *layers):
    for i in range(QUAD):
        dst[0, i, rows, cols] = layers[-1][i]
        if len(layers) == 2:
            dst[1, i, rows, cols] = layers[0][i] - C[i] * layers[1][i]


def _block_matmul(rows, weights, n_layers):
    u = [_dot(rows(0, i), weights(_slot(i, i))) for i in range(QUAD)]
    if n_layers == 1:
        for i, j in PAIRS:
            t = _dot(rows(0, j), weights(_slot(j, i))) - _dot(rows(0, i), weights(_slot(i, j)))
            u[i], u[j] = u[i] + t, u[j] - t
        return [u]
    v = [_dot(rows(1, i), weights(V_SLOT + i)) for i in range(QUAD)]
    for n, (i, j) in enumerate(PAIRS):
        both, gap = rows(1, i) + rows(1, j), C[j] - C[i]
        m_ji = _dot(both + _times(gap, rows(0, j)), weights(_slot(j, i)))
        m_ij = _dot(both - _times(gap, rows(0, i)), weights(_slot(i, j)))
        m = _dot(both, weights(PAIR_SLOT + n))
        t = _times(1 / gap, m_ji + m_ij - m)
        u[i], u[j] = u[i] + t, u[j] - t
        v[i], v[j] = v[i] + m_ji, v[j] + m_ij
    return [[v[i] + C[i] * u[i] for i in range(QUAD)], u]


def _dot(a, b):
    return lax.dot_general(_from_words(a), _from_words(b), (((1,), (0,)), ((), ())),
                           preferred_element_type=F32)


def _layernorm(x):
    m = jnp.mean(x, axis=-1, keepdims=True)
    d = x - m
    v = jnp.mean(d * d, axis=-1, keepdims=True)
    return d * lax.rsqrt(v + 1e-5)


def _run(stages, n=None):
    for _ in itertools.islice(stages, n):
        pass


def _tile(x, j):
    return x[:, j * LANES:(j + 1) * LANES]


def _kernel(x_hbm, mem0_ref, wq_hbm, wk_hbm, wv_hbm, wo_hbm, wg_hbm, wu_hbm, wd_hbm,
            out_hbm,
            x_v, out_v, raw_v, wqkv, wo_v, wgu_v, wd_v,
            h_attn, attn, h_ffn, act, early, mem, xa, xb, ring, bias, pre_in, pre,
            sem_x, sem_raw, sem_w, sem_out, *, seg):
    S, D = x_v.shape
    M = mem0_ref.shape[0]
    Dh = LANES
    n_hq, n_fq = wo_hbm.shape[0], wd_hbm.shape[0]
    H = QUAD * n_hq
    n_seg = S // seg
    L = M + seg
    quarter = D // QUAD
    n_chunks = quarter // RAW_ROWS
    n_groups = n_hq // HEAD_QUADS
    scale = Dh ** -0.5
    raw, wo, wgu, wd = (ref.bitcast(U32) for ref in (raw_v, wo_v, wgu_v, wd_v))

    def seg_rows(s, n=1):
        start = s * seg
        return pl.ds(start if isinstance(start, int) else pl.multiple_of(start, seg), n * seg)

    x_head = pltpu.make_async_copy(
        x_hbm.at[seg_rows(0, X_HEAD)], x_v.at[seg_rows(0, X_HEAD)], sem_x.at[0])
    x_tail = pltpu.make_async_copy(
        x_hbm.at[seg_rows(X_HEAD, n_seg - X_HEAD)],
        x_v.at[seg_rows(X_HEAD, n_seg - X_HEAD)], sem_x.at[1])

    def raw_copy(n, src):
        return pltpu.make_async_copy(
            src.at[:, n // 3], raw_v.at[n % RAW_SLOTS], sem_raw.at[n % RAW_SLOTS])

    def start_raw(n):
        for i, src in enumerate((wq_hbm, wk_hbm, wv_hbm)):
            pl.when(n % 3 == i)(raw_copy(n, src).start)

    def out_copies(src, dst, sem):
        return [pltpu.make_async_copy(
            src.at[:, i, :, pl.ds(j * quarter + k * LANES, LANES)], dst.at[_slot(i, j), k], sem)
            for i in range(QUAD) for j in range(QUAD) for k in range(quarter // LANES)]

    def in_copies(src, k, sem):
        return [pltpu.make_async_copy(
            src.at[:, :, pl.ds((QUAD * g + j) * LANES, LANES)],
            wgu_v.at[pl.ds(_slot(0, j), QUAD), k, g], sem)
            for g in range(n_fq) for j in range(QUAD)]

    wo_copies = out_copies(wo_hbm, wo_v, sem_w.at[0])
    wg_copies = in_copies(wg_hbm, 0, sem_w.at[1])
    wu_copies = in_copies(wu_hbm, 1, sem_w.at[2])
    wd_copies = out_copies(wd_hbm, wd_v, sem_w.at[3])

    def start(copies):
        for cp in copies:
            cp.start()

    def wait(copies):
        for cp in copies:
            cp.wait()

    def form_operands(w, w_v):
        def body(g, carry):
            at = [(k, r) for k in range(w.shape[1]) for r in range(0, w_v.shape[3], LANES)]
            blocks = [[[w[_slot(i, j), k, g, r // 2:(r + LANES) // 2] for j in range(QUAD)]
                       for i in range(QUAD)] for k, r in at]
            for (k, r), b in zip(at, blocks):
                for p, s in _weight_sums(b).items():
                    w_v[p, k, g, r:r + LANES] = s
            return carry
        lax.fori_loop(0, w.shape[2], body, 0)

    x_head.start()
    raw_copy(0, wq_hbm).start()

    r = lax.broadcasted_iota(jnp.int32, (2 * L, 2 * L), 0)
    c = lax.broadcasted_iota(jnp.int32, (2 * L, 2 * L), 1)
    visible = (r < M) | ((r >= L) & (r < L + M)) | (r >= c)
    bias[...] = jnp.where((r >= L) == (c >= L),
                          jnp.where(visible, 0.0, -1e9), -jnp.inf).astype(F32)

    pre[...] = jnp.zeros(pre.shape, F32)
    x_head.wait()
    raw_copy(1, wk_hbm).start()
    for n in range(PRE_STEPS):
        first = (LAG + n) * seg
        hs = _layernorm(x_v[first:first + PRE_ROWS, :].astype(F32))
        for k in range(n_chunks):
            pre_in[k, n * PRE_ROWS // 2:(n + 1) * PRE_ROWS // 2, :] = _to_words(
                jnp.concatenate([hs[:, i * quarter + k * RAW_ROWS:][:, :RAW_ROWS]
                                 for i in range(QUAD)], axis=1))

    def relayout(n, carry):
        slot, which, chunk = n % RAW_SLOTS, n % 3, n // 3
        raw_copy(n, wq_hbm).wait()

        @pl.when(n + 2 < 3 * n_chunks)
        def _():
            start_raw(n + 2)

        @pl.when(n + 2 == 3 * n_chunks)
        def _():
            start(wo_copies)

        rows = pl.ds(pl.multiple_of(chunk * (RAW_ROWS // 2), RAW_ROWS // 2), RAW_ROWS // 2)
        for g in range(n_hq):
            w = [[] for _ in range(QUAD)]
            for i, pair in itertools.product(range(QUAD), (2 * g, 2 * g + 1)):
                even, odd = (raw[slot, i, pl.ds(row, RAW_ROWS // 2, stride=H), :]
                             for row in (pair, H // 2 + pair))
                w[i].append((even & 0xFFFF) | (odd << 16))
                w[i].append((even >> 16) | (odd & jnp.uint32(0xFFFF0000)))
            for i, j in itertools.permutations(range(QUAD), 2):
                wqkv[which, _slot(i, j), g, rows, :] = w[i][j]
            for p, s in _weight_sums(w).items():
                wqkv[which, p, g, rows, :] = _to_words(s)
            pre[which, g] += _dot(pre_in[chunk], jnp.concatenate(
                [jnp.concatenate(row, axis=1) for row in w], axis=0))
        return carry

    lax.fori_loop(0, 3 * n_chunks, relayout, 0)

    mem0 = mem0_ref[...].astype(F32)
    every = slice(None)

    def feed(dst, rows, *hs):
        _put_rows(dst, rows, every,
                  *([h[:, i * quarter:(i + 1) * quarter] for i in range(QUAD)] for h in hs))

    def feed_memory(*mems):
        feed(h_attn, slice(0, M), *mems)

    def feed_tokens(*hs):
        feed(h_attn, slice(M, M + hs[0].shape[0]), *hs)

    def feed_both(use_pre):
        h2 = _layernorm(xa[1])
        if use_pre:
            h1 = _layernorm(xa[0, PRE_ROWS:, :])
            cut = PRE_ROWS // 2
            feed_tokens(jnp.concatenate([h1, h2[:cut]], axis=0), h2[cut:])
        else:
            feed_tokens(_layernorm(xa[0]), h2)

    def feed_ffn():
        feed(h_ffn, every, _layernorm(xb[0]), _layernorm(xb[1]))

    def attention(n_layers, filler, pre_rows=None, midway=()):
        n_rows = L if pre_rows is None else L - PRE_ROWS // 2
        total = n_layers * L

        def project(g, which):
            if g == n_groups:
                return _run(filler, 1)
            quads = range(g * HEAD_QUADS, (g + 1) * HEAD_QUADS)
            ys = _block_matmul(
                lambda k, i: h_attn[k, i, 0:n_rows, :],
                lambda p: jnp.concatenate([wqkv[which, p, quad] for quad in quads], axis=1),
                n_layers)
            heads = []
            for (n, quad), j in itertools.product(enumerate(quads), range(QUAD)):
                parts = [_tile(y[j], n) for y in ys]
                if pre_rows is not None:
                    parts = [parts[0][:M], pre[which, quad, pre_rows, j * Dh:(j + 1) * Dh],
                             parts[0][M:L - PRE_ROWS], parts[1][:M],
                             parts[0][L - PRE_ROWS:], parts[1][M:]]
                if which == 2:
                    parts.append(jnp.zeros((LANES - total, Dh), F32))
                heads.append(jnp.concatenate(parts, axis=0).astype(BF16))
            return heads

        def probabilities(q, k):
            s = lax.dot_general(q, k, (((1,), (1,)), ((), ())), preferred_element_type=F32)
            b = bias[0:total, 0:total]
            s = jnp.where(b == 0.0, s * scale, b)
            e = jnp.exp(s - jnp.max(s, axis=-1, keepdims=True))
            p = e * (1.0 / jnp.sum(e, axis=-1, keepdims=True))
            return jnp.concatenate(
                [p, jnp.zeros((total, LANES - total), F32)], axis=1).astype(BF16)

        def mix(quad, probs, v):
            o = [_dot(a, b) for a, b in zip(probs, v)]
            _put_rows(attn, every, slice(quad * Dh, (quad + 1) * Dh),
                      *([y[at:at + L] for y in o] for at in range(0, total, L)))

        q, k, v = (project(0, which) for which in range(3))
        _run(midway, 1)
        for g in range(n_groups):
            probs = [probabilities(a, b) for a, b in zip(q[:QUAD], k[:QUAD])]
            q_next = project(g + 1, 0)
            mix(2 * g, probs, v[:QUAD])
            probs = [probabilities(a, b) for a, b in zip(q[QUAD:], k[QUAD:])]
            k_next = project(g + 1, 1)
            _run(midway, 1)
            mix(2 * g + 1, probs, v[QUAD:])
            q, k, v = q_next, k_next, project(g + 1, 2)

    def project_out(src, w, n_layers, lo, hi):
        ys = _block_matmul(
            lambda k, i: src[k, i, :, lo * LANES:hi * LANES],
            lambda p: jnp.concatenate(
                [w[p, k, lo:hi].reshape((hi - lo) * LANES // 2, LANES)
                 for k in range(quarter // LANES)], axis=1),
            n_layers)
        return [jnp.concatenate(y, axis=1) for y in ys]

    def out_early(n_layers):
        for g in range(n_groups - 1):
            ys = project_out(attn, wo, n_layers, g * HEAD_QUADS, (g + 1) * HEAD_QUADS)
            for n, y in enumerate(ys):
                early[n] = early[n] + y if g else y
            yield

    def out_late(n_layers):
        ys = project_out(attn, wo, n_layers, n_hq - HEAD_QUADS, n_hq)
        return [early[n] + y for n, y in enumerate(ys)]

    def gate_up():
        for g in range(n_fq):
            ys = _block_matmul(
                lambda k, i: h_ffn[k, i],
                lambda p: jnp.concatenate([wgu[p, 0, g], wgu[p, 1, g]], axis=1), 2)
            _put_rows(act, every, slice(g * LANES, (g + 1) * LANES),
                      *([jax.nn.sigmoid(_tile(b, 0)) * _tile(b, 1) for b in y] for y in ys))

    def down():
        return [xb[n] + y for n, y in enumerate(project_out(act, wd, 2, 0, n_fq))]

    def ffn():
        feed_ffn()
        gate_up()
        return down()

    def single(s, xs, xs_next, before_out=None):
        attention(1, () if before_out else out_early(1))
        feed_tokens(_layernorm(xs_next))
        if before_out:
            before_out()
        o, = project_out(attn, wo, 1, 0, n_hq) if before_out else out_late(1)
        ring[s % RING] = xs + o[M:]
        mem[...] = o[:M]
        feed_memory(o[:M])

    def out_copy(s):
        slot = s % OUT_SLOTS
        return pltpu.make_async_copy(out_v.at[slot], out_hbm.at[seg_rows(s)], sem_out.at[slot])

    def emit(s, x):
        out_v[s % OUT_SLOTS] = x.astype(out_v.dtype)

    def tokens(s):
        return x_v[seg_rows(s), :].astype(F32)

    def fill(s, carry):
        pl.when(s == 1)(lambda: start(wu_copies))
        pl.when(s == 2)(lambda: start(wd_copies))
        single(s, tokens(s), tokens(s + 1))
        return carry

    def prepare_wo():
        wait(wo_copies)
        form_operands(wo, wo_v)

    feed_memory(mem0)
    feed_tokens(_layernorm(tokens(0)))
    start(wg_copies)
    single(0, tokens(0), tokens(1), prepare_wo)
    lax.fori_loop(1, LAG, fill, 0)
    feed_memory(mem[...], mem0)
    xb[0], xb[1] = ring[0], ring[1]
    wait(wg_copies)
    wait(wu_copies)
    form_operands(wgu, wgu_v)
    wait(wd_copies)
    x_tail.start()
    form_operands(wd, wd_v)
    ring[0], ring[1] = ffn()
    xb[0], xb[1] = ring[3], ring[2]
    xa[0], xa[1] = tokens(LAG), ring[0]
    feed_both(True)

    def step(t, use_pre):
        def gated():
            gate_up()
            yield
            ring[(t - 1) % RING], x2 = down()
            ring[jnp.where(t == LAG, LAG - 2, RING)] = x2
            emit(jnp.maximum(t - LAG - 1, 0), x2)

        pre_rows = None
        if use_pre:
            pre_rows = pl.ds(pl.multiple_of((t - LAG) * PRE_ROWS, PRE_ROWS), PRE_ROWS)
        feed_ffn()
        attention(2, out_early(2), pre_rows, gated())
        a1, a2 = xa[0], xa[1]
        xa[0], xa[1] = tokens(jnp.minimum(t + 1, n_seg - 1)), ring[(t + 1 - LAG) % RING]
        feed_both(use_pre)
        o1, o2 = out_late(2)
        mem[...] = o2[:M]
        feed_memory(o1[:M], o2[:M])
        xb[0], xb[1] = a1 + o1[M:], a2 + o2[M:]

    def steps(first, last, use_pre):
        def body(n, carry):
            t = first + UNROLL * n
            for k in range(UNROLL):
                s = t + k - LAG - 1
                pl.when(s >= UNROLL)(lambda: out_copy(s - UNROLL).start())
                pl.when(s >= OUT_SLOTS)(lambda: out_copy(s - OUT_SLOTS).wait())
            for k in range(UNROLL):
                step(t + k, use_pre)
            return carry

        lax.fori_loop(0, (last - first) // UNROLL, body, 0)

    steps(LAG, LAG + PRE_STEPS, True)
    x_tail.wait()
    feed_both(False)
    steps(LAG + PRE_STEPS, n_seg, False)

    tail = n_seg - LAG

    def drain(s, carry):
        single(s, ring[s % RING], ring[(s + 1) % RING])
        return carry

    def drain_ffn(n, carry):
        s = tail + 2 * n
        xb[0], xb[1] = ring[s % RING], ring[(s + 1) % RING]
        for k, x in enumerate(ffn()):
            emit(s + k, x)
        start([out_copy(s), out_copy(s + 1)])
        return carry

    start([out_copy(s) for s in range(tail - 1 - UNROLL, tail - 1)])
    out_copy(tail - 1 - OUT_SLOTS).wait()
    ring[(n_seg - 1) % RING], x2 = ffn()
    emit(tail - 1, x2)
    feed_memory(mem[...])
    feed_tokens(_layernorm(ring[tail % RING]))
    out_copy(tail - 1).start()
    lax.fori_loop(tail, n_seg, drain, 0)
    wait([out_copy(s) for s in range(tail - OUT_SLOTS, tail)])
    lax.fori_loop(0, LAG // 2, drain_ffn, 0)
    wait([out_copy(s) for s in range(tail, n_seg)])


@functools.partial(jax.jit, static_argnames=("A_seg_len",))
def pallas_interleave_layers__memory_aug_recurrent_mem_tr__glu_gated_glu__prompt_kernel(
    A_x, A_mem0, A_Wq, A_Wk, A_Wv, A_Wo, A_seg_len, B_x, B_w_gate, B_w_up, B_w_down,
):
    del B_x
    B, S, D = A_x.shape
    M = A_mem0.shape[1]
    _, H, Dh = A_Wq.shape
    F = B_w_gate.shape[1]
    seg = int(A_seg_len)
    assert B == 1 and S % seg == 0 and Dh == LANES
    L, quarter, n_pre = M + seg, D // QUAD, PRE_STEPS * PRE_ROWS
    n_hq, n_fq = H // QUAD, F // (QUAD * LANES)
    hbm = pl.BlockSpec(memory_space=pl.ANY)
    staged = [w.reshape(QUAD, quarter // RAW_ROWS, RAW_ROWS * H, Dh) for w in (A_Wq, A_Wk, A_Wv)]
    out = pl.pallas_call(
        functools.partial(_kernel, seg=seg),
        out_shape=jax.ShapeDtypeStruct((S, D), A_x.dtype),
        in_specs=[hbm, pl.BlockSpec(memory_space=pltpu.VMEM)] + [hbm] * 7,
        out_specs=hbm,
        scratch_shapes=[
            pltpu.VMEM((S, D), BF16),
            pltpu.VMEM((OUT_SLOTS, seg, D), A_x.dtype),
            pltpu.VMEM((RAW_SLOTS, QUAD, RAW_ROWS * H, Dh), BF16),
            pltpu.VMEM((3, N_SLOTS, n_hq, quarter // 2, Dh), U32),
            pltpu.VMEM((N_SLOTS, quarter // LANES, n_hq, Dh, LANES), BF16),
            pltpu.VMEM((N_SLOTS, 2, n_fq, quarter, LANES), BF16),
            pltpu.VMEM((N_SLOTS, quarter // LANES, n_fq, LANES, LANES), BF16),
            pltpu.VMEM((2, QUAD, L, quarter), F32),
            pltpu.VMEM((2, QUAD, L, n_hq * Dh), F32),
            pltpu.VMEM((2, QUAD, seg, quarter), F32),
            pltpu.VMEM((2, QUAD, seg, n_fq * LANES), F32),
            pltpu.VMEM((2, L, D), F32),
            pltpu.VMEM((M, D), F32),
            pltpu.VMEM((2, seg, D), F32),
            pltpu.VMEM((2, seg, D), F32),
            pltpu.VMEM((RING + 1, seg, D), F32),
            pltpu.VMEM((2 * L, 2 * L), F32),
            pltpu.VMEM((quarter // RAW_ROWS, n_pre // 2, QUAD * RAW_ROWS), U32),
            pltpu.VMEM((3, n_hq, n_pre, QUAD * Dh), F32),
            pltpu.SemaphoreType.DMA((2,)),
            pltpu.SemaphoreType.DMA((RAW_SLOTS,)),
            pltpu.SemaphoreType.DMA((4,)),
            pltpu.SemaphoreType.DMA((OUT_SLOTS,)),
        ],
        compiler_params=pltpu.CompilerParams(vmem_limit_bytes=127 * 2**20),
    )(A_x.reshape(S, D), A_mem0.reshape(M, D), *staged,
      A_Wo.reshape(n_hq, QUAD, Dh, D), B_w_gate.reshape(QUAD, quarter, F),
      B_w_up.reshape(QUAD, quarter, F), B_w_down.reshape(n_fq, QUAD, LANES, D))
    return out.reshape(B, S, D)
```

```python
import functools
import itertools

import jax
import jax.numpy as jnp
from jax import lax
import jax.experimental.pallas as pl
import jax.experimental.pallas.tpu as pltpu

F32 = jnp.float32
BF16 = jnp.bfloat16
U32 = jnp.uint32
LANES = 128
LAG = 4
RING = 4
HEAD_QUADS = 2
RAW_ROWS = 64
RAW_SLOTS = 3
RAW_PAD = 16
PRE_ROWS = 16
PRE_STEPS = 16
X_HEAD = LAG + PRE_STEPS + 1
OUT_SLOTS = 4

QUAD = 4
C = (-1.5, -0.5, 0.5, 1.5)
PAIRS = tuple(itertools.combinations(range(QUAD), 2))
V_SLOT, PAIR_SLOT = QUAD * QUAD, QUAD * QUAD + QUAD
ORDER = ((1, 2), (1, 3), (2, 3), (0, 1), (1, 1), (0, 2), (2, 2), (0, 3), (0, 0), (3, 3))
N_SLOTS = PAIR_SLOT + len(PAIRS)


def _slot(i, j):
    return QUAD * j + i


def _to_words(x):
    return pltpu.bitcast(x.astype(BF16), U32)


def _from_words(x):
    return pltpu.bitcast(x, BF16) if x.dtype == U32 else x


def _weight_sums(w):
    w = [[_from_words(b).astype(F32) for b in row] for row in w]
    sums = {}
    for i in range(QUAD):
        others = [j for j in range(QUAD) if j != i]
        sums[_slot(i, i)] = functools.reduce(jnp.add, [w[i][j] for j in others], w[i][i])
        sums[V_SLOT + i] = functools.reduce(jnp.subtract, [w[j][i] for j in others], w[i][i])
    for n, (i, j) in enumerate(PAIRS):
        sums[PAIR_SLOT + n] = w[i][j] + w[j][i]
    return {p: s.astype(BF16) for p, s in sums.items()}


def _times(c, x):
    return x if c == 1 else c * x


def _put_rows(dst, rows, cols, *layers):
    for i in range(QUAD):
        dst[0, i, rows, cols] = layers[-1][i]
        if len(layers) == 2:
            dst[1, i, rows, cols] = layers[0][i] - C[i] * layers[1][i]


def _block_matmul(rows, weights, n_layers):
    u, v = {}, {}

    def add(acc, i, y):
        acc[i] = acc[i] + y if i in acc else y

    for i, j in ORDER:
        if i == j:
            add(u, i, _dot(rows(0, i), weights(_slot(i, i))))
            if n_layers == 2:
                add(v, i, _dot(rows(1, i), weights(V_SLOT + i)))
            continue
        if n_layers == 1:
            t = _dot(rows(0, j), weights(_slot(j, i))) - _dot(rows(0, i), weights(_slot(i, j)))
        else:
            both, gap = rows(1, i) + rows(1, j), C[j] - C[i]
            m_ji = _dot(both + _times(gap, rows(0, j)), weights(_slot(j, i)))
            m_ij = _dot(both - _times(gap, rows(0, i)), weights(_slot(i, j)))
            m = _dot(both, weights(PAIR_SLOT + PAIRS.index((i, j))))
            t = _times(1 / gap, m_ji + m_ij - m)
            add(v, i, m_ji)
            add(v, j, m_ij)
        add(u, i, t)
        u[j] = u[j] - t if j in u else -t
    u = [u[i] for i in range(QUAD)]
    return [u] if n_layers == 1 else [[v[i] + C[i] * u[i] for i in range(QUAD)], u]


def _dot(a, b):
    return lax.dot_general(_from_words(a), _from_words(b), (((1,), (0,)), ((), ())),
                           preferred_element_type=F32)


def _layernorm(x):
    m = jnp.mean(x, axis=-1, keepdims=True)
    d = x - m
    v = jnp.mean(d * d, axis=-1, keepdims=True)
    return d * lax.rsqrt(v + 1e-5)


def _gate(g, u):
    u = 0.5 * u
    return u * jnp.tanh(0.5 * g) + u


def _run(stages, n=None):
    for _ in itertools.islice(stages, n):
        pass


def _tile(x, j):
    return x[:, j * LANES:(j + 1) * LANES]


def _kernel(x_hbm, mem0_ref, wq_hbm, wk_hbm, wv_hbm, wo_hbm, wg_hbm, wu_hbm, wd_hbm,
            out_hbm,
            x_v, out_v, raw_v, wqkv, wo_v, wgu_v, wd_v,
            h_attn, attn, h_ffn, act, early, mem, xa, xb, ring, bias, pre_in, pre,
            sem_x, sem_raw, sem_w, sem_out, *, seg):
    S, D = x_v.shape
    M = mem0_ref.shape[0]
    Dh = LANES
    n_hq, n_fq = wo_hbm.shape[0], wd_hbm.shape[0]
    H = QUAD * n_hq
    n_seg = S // seg
    L = M + seg
    quarter = D // QUAD
    n_chunks = quarter // RAW_ROWS
    n_groups = n_hq // HEAD_QUADS
    scale = Dh ** -0.5
    raw, wo, wgu, wd = (ref.bitcast(U32) for ref in (raw_v, wo_v, wgu_v, wd_v))

    def seg_rows(s, n=1):
        start = s * seg
        return pl.ds(start if isinstance(start, int) else pl.multiple_of(start, seg), n * seg)

    x_head = pltpu.make_async_copy(
        x_hbm.at[seg_rows(0, X_HEAD)], x_v.at[seg_rows(0, X_HEAD)], sem_x.at[0])
    x_tail = pltpu.make_async_copy(
        x_hbm.at[seg_rows(X_HEAD, n_seg - X_HEAD)],
        x_v.at[seg_rows(X_HEAD, n_seg - X_HEAD)], sem_x.at[1])

    def raw_copy(n, src):
        return pltpu.make_async_copy(
            src.at[:, n // 3], raw_v.at[n % RAW_SLOTS, :, pl.ds(RAW_PAD, RAW_ROWS * H)],
            sem_raw.at[n % RAW_SLOTS])

    def start_raw(n):
        for i, src in enumerate((wq_hbm, wk_hbm, wv_hbm)):
            pl.when(n % 3 == i)(raw_copy(n, src).start)

    def out_copies(src, dst, sem):
        return [pltpu.make_async_copy(
            src.at[:, i, :, pl.ds(j * quarter + k * LANES, LANES)], dst.at[_slot(i, j), k], sem)
            for i in range(QUAD) for j in range(QUAD) for k in range(quarter // LANES)]

    def in_copies(src, k, sem):
        return [pltpu.make_async_copy(
            src.at[:, :, pl.ds((QUAD * g + j) * LANES, LANES)],
            wgu_v.at[pl.ds(_slot(0, j), QUAD), k, g], sem)
            for g in range(n_fq) for j in range(QUAD)]

    wo_copies = out_copies(wo_hbm, wo_v, sem_w.at[0])
    wg_copies = in_copies(wg_hbm, 0, sem_w.at[1])
    wu_copies = in_copies(wu_hbm, 1, sem_w.at[2])
    wd_copies = out_copies(wd_hbm, wd_v, sem_w.at[3])

    def start(copies):
        for cp in copies:
            cp.start()

    def wait(copies):
        for cp in copies:
            cp.wait()

    def form_operands(w, w_v):
        def body(g, carry):
            at = [(k, r) for k in range(w.shape[1]) for r in range(0, w_v.shape[3], 32)]
            blocks = [[[w[_slot(i, j), k, g, r // 2:r // 2 + 16] for j in range(QUAD)]
                       for i in range(QUAD)] for k, r in at]
            for (k, r), b in zip(at, blocks):
                for p, s in _weight_sums(b).items():
                    w_v[p, k, g, r:r + 32] = s
            return carry
        lax.fori_loop(0, w.shape[2], body, 0)

    x_head.start()

    r = lax.broadcasted_iota(jnp.int32, (2 * L, 2 * L), 0)
    c = lax.broadcasted_iota(jnp.int32, (2 * L, 2 * L), 1)
    visible = (r < M) | ((r >= L) & (r < L + M)) | (r >= c)
    bias[...] = jnp.where((r >= L) == (c >= L),
                          jnp.where(visible, 0.0, -1e9), -jnp.inf).astype(F32)

    for at in (0, RAW_PAD + RAW_ROWS * H):
        raw_v[:, :, at:at + RAW_PAD, :] = jnp.zeros((RAW_SLOTS, QUAD, RAW_PAD, Dh), BF16)
    x_head.wait()
    raw_copy(0, wq_hbm).start()
    for n in range(PRE_STEPS):
        first = (LAG + n) * seg
        hs = _layernorm(x_v[first:first + PRE_ROWS, :].astype(F32))
        for k in range(n_chunks):
            pre_in[k, n * PRE_ROWS // 2:(n + 1) * PRE_ROWS // 2, :] = _to_words(
                jnp.concatenate([hs[:, i * quarter + k * RAW_ROWS:][:, :RAW_ROWS]
                                 for i in range(QUAD)], axis=1))

    raw_copy(1, wk_hbm).start()

    def columns(slot, i):
        sub = lax.broadcasted_iota(jnp.int32, (8, Dh), 0)
        out = []
        for at in range(RAW_PAD // 2, (RAW_PAD + RAW_ROWS * H) // 2, 8 * H):
            x = {c: raw[slot, i, pl.ds(at + c, 8, stride=H + 1), :] for c in range(-7, H)}
            for bit in (1, 2, 4):
                x = {c: jnp.where(sub & bit != 0, x[c - bit], x[c]) for c in x if c - bit in x}
            out.append(x)
        return [jnp.concatenate([x[c] for x in out], axis=0) for c in range(H)]

    def relayout(n, carry):
        slot, which, chunk = n % RAW_SLOTS, n % 3, n // 3
        raw_copy(n, wq_hbm).wait()

        @pl.when(n + 2 < 3 * n_chunks)
        def _():
            start_raw(n + 2)

        @pl.when(n + 2 == 3 * n_chunks)
        def _():
            start(wo_copies)

        rows = pl.ds(pl.multiple_of(chunk * (RAW_ROWS // 2), RAW_ROWS // 2), RAW_ROWS // 2)
        words = [columns(slot, i) for i in range(QUAD)]
        for g in range(n_hq):
            w = [[] for _ in range(QUAD)]
            for i, pair in itertools.product(range(QUAD), (2 * g, 2 * g + 1)):
                even, odd = words[i][pair], words[i][H // 2 + pair]
                w[i].append((even & 0xFFFF) | (odd << 16))
                w[i].append((even >> 16) | (odd & jnp.uint32(0xFFFF0000)))
            for i, j in itertools.permutations(range(QUAD), 2):
                wqkv[which, _slot(i, j), g, rows, :] = w[i][j]
            for p, s in _weight_sums(w).items():
                wqkv[which, p, g, rows, :] = _to_words(s)
            pre[which, g] = jnp.where(chunk == 0, 0.0, pre[which, g]) + _dot(pre_in[chunk], jnp.concatenate(
                [jnp.concatenate(row, axis=1) for row in w], axis=0))
        return carry

    lax.fori_loop(0, 3 * n_chunks, relayout, 0)

    mem0 = mem0_ref[...].astype(F32)
    every = slice(None)

    def feed(dst, rows, *hs):
        _put_rows(dst, rows, every,
                  *([h[:, i * quarter:(i + 1) * quarter] for i in range(QUAD)] for h in hs))

    def feed_memory(*mems):
        feed(h_attn, slice(0, M), *mems)

    def feed_tokens(*hs):
        feed(h_attn, slice(M, M + hs[0].shape[0]), *hs)

    def feed_both(use_pre):
        h2 = _layernorm(xa[1])
        if use_pre:
            h1 = _layernorm(xa[0, PRE_ROWS:, :])
            cut = PRE_ROWS // 2
            feed_tokens(jnp.concatenate([h1, h2[:cut]], axis=0), h2[cut:])
        else:
            feed_tokens(_layernorm(xa[0]), h2)

    def feed_ffn():
        feed(h_ffn, every, _layernorm(xb[0]), _layernorm(xb[1]))

    def attention(n_layers, filler, pre_rows=None, midway=()):
        n_rows = L if pre_rows is None else L - PRE_ROWS // 2
        total = n_layers * L

        def project(g, which):
            if g == n_groups:
                return _run(filler, 1)
            quads = range(g * HEAD_QUADS, (g + 1) * HEAD_QUADS)
            ys = _block_matmul(
                lambda k, i: h_attn[k, i, 0:n_rows, :],
                lambda p: jnp.concatenate([wqkv[which, p, quad] for quad in quads], axis=1),
                n_layers)
            heads = []
            for (n, quad), j in itertools.product(enumerate(quads), range(QUAD)):
                parts = [_tile(y[j], n) for y in ys]
                if pre_rows is not None:
                    parts = [parts[0][:M], pre[which, quad, pre_rows, j * Dh:(j + 1) * Dh],
                             parts[0][M:L - PRE_ROWS], parts[1][:M],
                             parts[0][L - PRE_ROWS:], parts[1][M:]]
                if which == 2:
                    parts.append(jnp.zeros((LANES - total, Dh), F32))
                y = jnp.concatenate(parts, axis=0)
                heads.append((y.T if which == 1 else y).astype(BF16))
            return heads

        def probabilities(q, k):
            s = _dot(q, k)
            b = bias[0:total, 0:total]
            s = jnp.where(b == 0.0, s * scale, b)
            e = jnp.exp(s - jnp.max(s, axis=-1, keepdims=True))
            p = e * (1.0 / jnp.sum(e, axis=-1, keepdims=True))
            return jnp.concatenate(
                [p, jnp.zeros((total, LANES - total), F32)], axis=1).astype(BF16)

        def mix(quad, probs, v):
            o = [_dot(a, b) for a, b in zip(probs, v)]
            _put_rows(attn, every, slice(quad * Dh, (quad + 1) * Dh),
                      *([y[at:at + L] for y in o] for at in range(0, total, L)))

        q, k, v = (project(0, which) for which in range(3))
        _run(midway, 1)
        for g in range(n_groups):
            probs = [probabilities(a, b) for a, b in zip(q[:QUAD], k[:QUAD])]
            q_next = project(g + 1, 0)
            mix(2 * g, probs, v[:QUAD])
            probs = [probabilities(a, b) for a, b in zip(q[QUAD:], k[QUAD:])]
            k_next = project(g + 1, 1)
            _run(midway, 1)
            mix(2 * g + 1, probs, v[QUAD:])
            q, k, v = q_next, k_next, project(g + 1, 2)

    def project_out(src, w, n_layers, lo, hi):
        ys = _block_matmul(
            lambda k, i: src[k, i, :, lo * LANES:hi * LANES],
            lambda p: jnp.concatenate(
                [w[p, k, lo:hi].reshape((hi - lo) * LANES // 2, LANES)
                 for k in range(quarter // LANES)], axis=1),
            n_layers)
        return [jnp.concatenate(y, axis=1) for y in ys]

    def out_early(n_layers):
        for g in range(n_groups - 1):
            ys = project_out(attn, wo, n_layers, g * HEAD_QUADS, (g + 1) * HEAD_QUADS)
            for n, y in enumerate(ys):
                early[n] = early[n] + y if g else y
            yield

    def out_late(n_layers):
        ys = project_out(attn, wo, n_layers, n_hq - HEAD_QUADS, n_hq)
        return [early[n] + y for n, y in enumerate(ys)]

    def gate_up():
        for g in range(n_fq):
            ys = _block_matmul(
                lambda k, i: h_ffn[k, i],
                lambda p: jnp.concatenate([wgu[p, 0, g], wgu[p, 1, g]], axis=1), 2)
            _put_rows(act, every, slice(g * LANES, (g + 1) * LANES),
                      *([_gate(_tile(b, 0), _tile(b, 1)) for b in y] for y in ys))

    def down():
        return [xb[n] + y for n, y in enumerate(project_out(act, wd, 2, 0, n_fq))]

    def ffn():
        feed_ffn()
        gate_up()
        return down()

    def single(s, xs, xs_next, before_out=None):
        attention(1, () if before_out else out_early(1))
        feed_tokens(_layernorm(xs_next))
        if before_out:
            before_out()
        o, = project_out(attn, wo, 1, 0, n_hq) if before_out else out_late(1)
        ring[s % RING] = xs + o[M:]
        mem[...] = o[:M]
        feed_memory(o[:M])

    def out_copy(s):
        slot = s % OUT_SLOTS
        return pltpu.make_async_copy(out_v.at[slot], out_hbm.at[seg_rows(s)], sem_out.at[slot])

    def emit(s, x):
        out_v[s % OUT_SLOTS] = x.astype(out_v.dtype)

    def tokens(s):
        return x_v[seg_rows(s), :].astype(F32)

    def fill(s, carry):
        pl.when(s == 1)(lambda: start(wu_copies))
        pl.when(s == 2)(lambda: start(wd_copies))
        single(s, tokens(s), tokens(s + 1))
        return carry

    def prepare_wo():
        wait(wo_copies)
        form_operands(wo, wo_v)

    feed_memory(mem0)
    feed_tokens(_layernorm(tokens(0)))
    start(wg_copies)
    single(0, tokens(0), tokens(1), prepare_wo)
    lax.fori_loop(1, LAG, fill, 0)
    feed_memory(mem[...], mem0)
    xb[0], xb[1] = ring[0], ring[1]
    wait(wg_copies)
    wait(wu_copies)
    form_operands(wgu, wgu_v)
    wait(wd_copies)
    x_tail.start()
    form_operands(wd, wd_v)
    ring[0], ring[1] = ffn()
    xb[0], xb[1] = ring[3], ring[2]
    xa[0], xa[1] = tokens(LAG), ring[0]
    feed_both(True)

    def step(t, carry, *, use_pre):
        s = t - LAG - 1
        pl.when(s >= 1)(lambda: out_copy(s - 1).start())
        pl.when(s >= OUT_SLOTS)(lambda: out_copy(s - OUT_SLOTS).wait())

        def gated():
            gate_up()
            yield
            ring[(t - 1) % RING], x2 = down()
            ring[jnp.where(t == LAG, LAG - 2, RING)] = x2
            emit(jnp.maximum(s, 0), x2)

        pre_rows = None
        if use_pre:
            pre_rows = pl.ds(pl.multiple_of((t - LAG) * PRE_ROWS, PRE_ROWS), PRE_ROWS)
        feed_ffn()
        attention(2, out_early(2), pre_rows, gated())
        a1, a2 = xa[0], xa[1]
        xa[0], xa[1] = tokens(jnp.minimum(t + 1, n_seg - 1)), ring[(t + 1 - LAG) % RING]
        feed_both(use_pre)
        o1, o2 = out_late(2)
        mem[...] = o2[:M]
        feed_memory(o1[:M], o2[:M])
        xb[0], xb[1] = a1 + o1[M:], a2 + o2[M:]
        return carry

    lax.fori_loop(LAG, LAG + PRE_STEPS, functools.partial(step, use_pre=True), 0)
    x_tail.wait()
    feed_both(False)
    lax.fori_loop(LAG + PRE_STEPS, n_seg, functools.partial(step, use_pre=False), 0)

    tail = n_seg - LAG

    def drain(s, carry):
        single(s, ring[s % RING], ring[(s + 1) % RING])
        return carry

    def drain_ffn(n, carry):
        s = tail + 2 * n
        xb[0], xb[1] = ring[s % RING], ring[(s + 1) % RING]
        for k, x in enumerate(ffn()):
            emit(s + k, x)
        start([out_copy(s), out_copy(s + 1)])
        return carry

    out_copy(tail - 2).start()
    out_copy(tail - 1 - OUT_SLOTS).wait()
    ring[(n_seg - 1) % RING], x2 = ffn()
    emit(tail - 1, x2)
    feed_memory(mem[...])
    feed_tokens(_layernorm(ring[tail % RING]))
    out_copy(tail - 1).start()
    lax.fori_loop(tail, n_seg, drain, 0)
    wait([out_copy(s) for s in range(tail - OUT_SLOTS, tail)])
    lax.fori_loop(0, LAG // 2, drain_ffn, 0)
    wait([out_copy(s) for s in range(tail, n_seg)])


@functools.partial(jax.jit, static_argnames=("A_seg_len",))
def pallas_interleave_layers__memory_aug_recurrent_mem_tr__glu_gated_glu__prompt_kernel(
    A_x, A_mem0, A_Wq, A_Wk, A_Wv, A_Wo, A_seg_len, B_x, B_w_gate, B_w_up, B_w_down,
):
    del B_x
    B, S, D = A_x.shape
    M = A_mem0.shape[1]
    _, H, Dh = A_Wq.shape
    F = B_w_gate.shape[1]
    seg = int(A_seg_len)
    assert B == 1 and S % seg == 0 and Dh == LANES
    L, quarter, n_pre = M + seg, D // QUAD, PRE_STEPS * PRE_ROWS
    n_hq, n_fq = H // QUAD, F // (QUAD * LANES)
    hbm = pl.BlockSpec(memory_space=pl.ANY)
    staged = [w.reshape(QUAD, quarter // RAW_ROWS, RAW_ROWS * H, Dh) for w in (A_Wq, A_Wk, A_Wv)]
    out = pl.pallas_call(
        functools.partial(_kernel, seg=seg),
        out_shape=jax.ShapeDtypeStruct((S, D), A_x.dtype),
        in_specs=[hbm, pl.BlockSpec(memory_space=pltpu.VMEM)] + [hbm] * 7,
        out_specs=hbm,
        scratch_shapes=[
            pltpu.VMEM((S, D), BF16),
            pltpu.VMEM((OUT_SLOTS, seg, D), A_x.dtype),
            pltpu.VMEM((RAW_SLOTS, QUAD, RAW_ROWS * H + 2 * RAW_PAD, Dh), BF16),
            pltpu.VMEM((3, N_SLOTS, n_hq, quarter // 2, Dh), U32),
            pltpu.VMEM((N_SLOTS, quarter // LANES, n_hq, Dh, LANES), BF16),
            pltpu.VMEM((N_SLOTS, 2, n_fq, quarter, LANES), BF16),
            pltpu.VMEM((N_SLOTS, quarter // LANES, n_fq, LANES, LANES), BF16),
            pltpu.VMEM((2, QUAD, L, quarter), F32),
            pltpu.VMEM((2, QUAD, L, n_hq * Dh), F32),
            pltpu.VMEM((2, QUAD, seg, quarter), F32),
            pltpu.VMEM((2, QUAD, seg, n_fq * LANES), F32),
            pltpu.VMEM((2, L, D), F32),
            pltpu.VMEM((M, D), F32),
            pltpu.VMEM((2, seg, D), F32),
            pltpu.VMEM((2, seg, D), F32),
            pltpu.VMEM((RING + 1, seg, D), F32),
            pltpu.VMEM((2 * L, 2 * L), F32),
            pltpu.VMEM((quarter // RAW_ROWS, n_pre // 2, QUAD * RAW_ROWS), U32),
            pltpu.VMEM((3, n_hq, n_pre, QUAD * Dh), F32),
            pltpu.SemaphoreType.DMA((2,)),
            pltpu.SemaphoreType.DMA((RAW_SLOTS,)),
            pltpu.SemaphoreType.DMA((4,)),
            pltpu.SemaphoreType.DMA((OUT_SLOTS,)),
        ],
        compiler_params=pltpu.CompilerParams(vmem_limit_bytes=127 * 2**20),
    )(A_x.reshape(S, D), A_mem0.reshape(M, D), *staged,
      A_Wo.reshape(n_hq, QUAD, Dh, D), B_w_gate.reshape(QUAD, quarter, F),
      B_w_up.reshape(QUAD, quarter, F), B_w_down.reshape(n_fq, QUAD, LANES, D))
    return out.reshape(B, S, D)
```

```python
import functools
import itertools

import jax
import jax.numpy as jnp
from jax import lax
import jax.experimental.pallas as pl
import jax.experimental.pallas.tpu as pltpu

F32 = jnp.float32
BF16 = jnp.bfloat16
U32 = jnp.uint32
LANES = 128
LAG = 4
RING = 4
HEAD_QUADS = 2
RAW_ROWS = 64
RAW_SLOTS = 3
RAW_PAD = 16
PRE_ROWS = 16
PRE_STEPS = 16
X_HEAD = LAG + PRE_STEPS + 1
OUT_SLOTS = 4

QUAD = 4
C = (-1.5, -0.5, 0.5, 1.5)
PAIRS = tuple(itertools.combinations(range(QUAD), 2))
V_SLOT, PAIR_SLOT = QUAD * QUAD, QUAD * QUAD + QUAD
ORDER = ((1, 2), (1, 3), (2, 3), (0, 1), (1, 1), (0, 2), (2, 2), (0, 3), (0, 0), (3, 3))
N_SLOTS = PAIR_SLOT + len(PAIRS)


def _slot(i, j):
    return QUAD * j + i


def _to_words(x):
    return pltpu.bitcast(x.astype(BF16), U32)


def _from_words(x):
    return pltpu.bitcast(x, BF16) if x.dtype == U32 else x


def _weight_sums(w):
    w = [[_from_words(b).astype(F32) for b in row] for row in w]
    sums = {}
    for i in range(QUAD):
        others = [j for j in range(QUAD) if j != i]
        sums[_slot(i, i)] = functools.reduce(jnp.add, [w[i][j] for j in others], w[i][i])
        sums[V_SLOT + i] = functools.reduce(jnp.subtract, [w[j][i] for j in others], w[i][i])
    for n, (i, j) in enumerate(PAIRS):
        sums[PAIR_SLOT + n] = w[i][j] + w[j][i]
    return {p: s.astype(BF16) for p, s in sums.items()}


def _times(c, x):
    return x if c == 1 else c * x


def _put_rows(dst, rows, cols, *layers):
    for i in range(QUAD):
        dst[0, i, rows, cols] = layers[-1][i]
        if len(layers) == 2:
            dst[1, i, rows, cols] = layers[0][i] - C[i] * layers[1][i]


def _block_matmul(rows, weights, n_layers):
    u, v = {}, {}

    def add(acc, i, y):
        acc[i] = acc[i] + y if i in acc else y

    for i, j in ORDER:
        if i == j:
            add(u, i, _dot(rows(0, i), weights(_slot(i, i))))
            if n_layers == 2:
                add(v, i, _dot(rows(1, i), weights(V_SLOT + i)))
            continue
        if n_layers == 1:
            t = _dot(rows(0, j), weights(_slot(j, i))) - _dot(rows(0, i), weights(_slot(i, j)))
        else:
            both, gap = rows(1, i) + rows(1, j), C[j] - C[i]
            m_ji = _dot(both + _times(gap, rows(0, j)), weights(_slot(j, i)))
            m_ij = _dot(both - _times(gap, rows(0, i)), weights(_slot(i, j)))
            m = _dot(both, weights(PAIR_SLOT + PAIRS.index((i, j))))
            t = _times(1 / gap, m_ji + m_ij - m)
            add(v, i, m_ji)
            add(v, j, m_ij)
        add(u, i, t)
        u[j] = u[j] - t if j in u else -t
    u = [u[i] for i in range(QUAD)]
    return [u] if n_layers == 1 else [[v[i] + C[i] * u[i] for i in range(QUAD)], u]


def _dot(a, b):
    return lax.dot_general(_from_words(a), _from_words(b), (((1,), (0,)), ((), ())),
                           preferred_element_type=F32)


def _layernorm(x):
    m = jnp.mean(x, axis=-1, keepdims=True)
    d = x - m
    v = jnp.mean(d * d, axis=-1, keepdims=True)
    return d * lax.rsqrt(v + 1e-5)


def _gate(g, u):
    u = 0.5 * u
    return u * jnp.tanh(0.5 * g) + u


def _run(stages, n=None):
    for _ in itertools.islice(stages, n):
        pass


def _tile(x, j):
    return x[:, j * LANES:(j + 1) * LANES]


def _kernel(x_hbm, mem0_ref, wq_hbm, wk_hbm, wv_hbm, wo_hbm, wg_hbm, wu_hbm, wd_hbm,
            out_hbm,
            x_v, x_pre, out_v, raw_v, wqkv, wo_v, wgu_v, wd_v,
            h_attn, attn, h_ffn, act, early, mem, xa, xb, ring, bias, pre_in, pre,
            sem_x, sem_raw, sem_w, sem_out):
    n_seg, seg, D = x_v.shape
    M = mem0_ref.shape[0]
    Dh = LANES
    n_hq, n_fq = wo_hbm.shape[0], wd_hbm.shape[0]
    H = QUAD * n_hq
    L = M + seg
    quarter = D // QUAD
    n_chunks = quarter // RAW_ROWS
    n_groups = n_hq // HEAD_QUADS
    scale = Dh ** -0.5
    raw, wo, wgu, wd = (ref.bitcast(U32) for ref in (raw_v, wo_v, wgu_v, wd_v))

    x_first = pltpu.make_async_copy(
        x_hbm.at[pl.ds(LAG, PRE_STEPS), pl.ds(0, PRE_ROWS)], x_pre, sem_x.at[0])
    x_head = pltpu.make_async_copy(
        x_hbm.at[pl.ds(0, X_HEAD)], x_v.at[pl.ds(0, X_HEAD)], sem_x.at[1])
    x_tail = pltpu.make_async_copy(
        x_hbm.at[pl.ds(X_HEAD, n_seg - X_HEAD)], x_v.at[pl.ds(X_HEAD, n_seg - X_HEAD)],
        sem_x.at[2])

    def raw_copy(n, src):
        return pltpu.make_async_copy(
            src.at[:, n // 3], raw_v.at[n % RAW_SLOTS, :, pl.ds(RAW_PAD, RAW_ROWS * H)],
            sem_raw.at[n % RAW_SLOTS])

    def start_raw(n):
        for i, src in enumerate((wq_hbm, wk_hbm, wv_hbm)):
            pl.when(n % 3 == i)(raw_copy(n, src).start)

    def out_copies(src, dst, sem):
        return [pltpu.make_async_copy(
            src.at[:, i, :, pl.ds(j * quarter + k * LANES, LANES)], dst.at[_slot(i, j), k], sem)
            for i in range(QUAD) for j in range(QUAD) for k in range(quarter // LANES)]

    def in_copies(src, k, sem):
        return [pltpu.make_async_copy(
            src.at[:, :, pl.ds((QUAD * g + j) * LANES, LANES)],
            wgu_v.at[pl.ds(_slot(0, j), QUAD), k, g], sem)
            for g in range(n_fq) for j in range(QUAD)]

    wo_copies = out_copies(wo_hbm, wo_v, sem_w.at[0])
    wg_copies = in_copies(wg_hbm, 0, sem_w.at[1])
    wu_copies = in_copies(wu_hbm, 1, sem_w.at[2])
    wd_copies = out_copies(wd_hbm, wd_v, sem_w.at[3])

    def start(copies):
        for cp in copies:
            cp.start()

    def wait(copies):
        for cp in copies:
            cp.wait()

    def form_operands(w, w_v):
        def body(g, carry):
            at = [(k, r) for k in range(w.shape[1]) for r in range(0, w_v.shape[3], 32)]
            blocks = [[[w[_slot(i, j), k, g, r // 2:r // 2 + 16] for j in range(QUAD)]
                       for i in range(QUAD)] for k, r in at]
            for (k, r), b in zip(at, blocks):
                for p, s in _weight_sums(b).items():
                    w_v[p, k, g, r:r + 32] = s
            return carry
        lax.fori_loop(0, w.shape[2], body, 0)

    raw_copy(0, wq_hbm).start()
    x_first.start()

    r = lax.broadcasted_iota(jnp.int32, (2 * L, 2 * L), 0)
    c = lax.broadcasted_iota(jnp.int32, (2 * L, 2 * L), 1)
    visible = (r < M) | ((r >= L) & (r < L + M)) | (r >= c)
    bias[...] = jnp.where((r >= L) == (c >= L),
                          jnp.where(visible, 0.0, -1e9), -jnp.inf).astype(F32)

    for at in (0, RAW_PAD + RAW_ROWS * H):
        raw_v[:, :, at:at + RAW_PAD, :] = jnp.zeros((RAW_SLOTS, QUAD, RAW_PAD, Dh), BF16)
    x_first.wait()
    raw_copy(1, wk_hbm).start()
    hs = _to_words(_layernorm(x_pre[...].astype(F32).reshape(PRE_STEPS * PRE_ROWS, D)))
    for k in range(n_chunks):
        pre_in[k] = jnp.concatenate(
            [hs[:, i * quarter + k * RAW_ROWS:][:, :RAW_ROWS] for i in range(QUAD)], axis=1)

    def columns(slot, i):
        sub = lax.broadcasted_iota(jnp.int32, (8, Dh), 0)
        out = []
        for at in range(RAW_PAD // 2, (RAW_PAD + RAW_ROWS * H) // 2, 8 * H):
            x = {c: raw[slot, i, pl.ds(at + c, 8, stride=H + 1), :] for c in range(-7, H)}
            for bit in (1, 2, 4):
                x = {c: jnp.where(sub & bit != 0, x[c - bit], x[c]) for c in x if c - bit in x}
            out.append(x)
        return [jnp.concatenate([x[c] for x in out], axis=0) for c in range(H)]

    def relayout(n, carry):
        slot, which, chunk = n % RAW_SLOTS, n % 3, n // 3
        raw_copy(n, wq_hbm).wait()

        @pl.when(n + 2 < 3 * n_chunks)
        def _():
            start_raw(n + 2)

        @pl.when(n + 3 == 3 * n_chunks)
        def _():
            start([x_head] + wo_copies)

        rows = pl.ds(pl.multiple_of(chunk * (RAW_ROWS // 2), RAW_ROWS // 2), RAW_ROWS // 2)
        words = [columns(slot, i) for i in range(QUAD)]
        for g in range(n_hq):
            w = [[] for _ in range(QUAD)]
            for i, pair in itertools.product(range(QUAD), (2 * g, 2 * g + 1)):
                even, odd = words[i][pair], words[i][H // 2 + pair]
                w[i].append((even & 0xFFFF) | (odd << 16))
                w[i].append((even >> 16) | (odd & jnp.uint32(0xFFFF0000)))
            for i, j in itertools.permutations(range(QUAD), 2):
                wqkv[which, _slot(i, j), g, rows, :] = w[i][j]
            for p, s in _weight_sums(w).items():
                wqkv[which, p, g, rows, :] = _to_words(s)
            pre[which, g] = jnp.where(chunk == 0, 0.0, pre[which, g]) + _dot(pre_in[chunk], jnp.concatenate(
                [jnp.concatenate(row, axis=1) for row in w], axis=0))
        return carry

    lax.fori_loop(0, 3 * n_chunks, relayout, 0)

    mem0 = mem0_ref[...].astype(F32)
    every = slice(None)

    def feed(dst, rows, *hs):
        _put_rows(dst, rows, every,
                  *([h[:, i * quarter:(i + 1) * quarter] for i in range(QUAD)] for h in hs))

    def feed_memory(*mems):
        feed(h_attn, slice(0, M), *mems)

    def feed_tokens(*hs):
        feed(h_attn, slice(M, M + hs[0].shape[0]), *hs)

    def feed_both(use_pre):
        h2 = _layernorm(xa[1])
        if use_pre:
            h1 = _layernorm(xa[0, PRE_ROWS:, :])
            cut = PRE_ROWS // 2
            feed_tokens(jnp.concatenate([h1, h2[:cut]], axis=0), h2[cut:])
        else:
            feed_tokens(_layernorm(xa[0]), h2)

    def feed_ffn():
        feed(h_ffn, every, _layernorm(xb[0]), _layernorm(xb[1]))

    def attention(n_layers, filler, pre_rows=None, midway=()):
        n_rows = L if pre_rows is None else L - PRE_ROWS // 2
        total = n_layers * L

        def project(g, which):
            if g == n_groups:
                return _run(filler, 1)
            quads = range(g * HEAD_QUADS, (g + 1) * HEAD_QUADS)
            ys = _block_matmul(
                lambda k, i: h_attn[k, i, 0:n_rows, :],
                lambda p: jnp.concatenate([wqkv[which, p, quad] for quad in quads], axis=1),
                n_layers)
            heads = []
            for (n, quad), j in itertools.product(enumerate(quads), range(QUAD)):
                parts = [_tile(y[j], n) for y in ys]
                if pre_rows is not None:
                    parts = [parts[0][:M], pre[which, quad, pre_rows, j * Dh:(j + 1) * Dh],
                             parts[0][M:L - PRE_ROWS], parts[1][:M],
                             parts[0][L - PRE_ROWS:], parts[1][M:]]
                if which == 2:
                    parts.append(jnp.zeros((LANES - total, Dh), F32))
                y = jnp.concatenate(parts, axis=0)
                heads.append((y.T if which == 1 else y).astype(BF16))
            return heads

        def probabilities(q, k):
            s = _dot(q, k)
            b = bias[0:total, 0:total]
            s = jnp.where(b == 0.0, s * scale, b)
            e = jnp.exp(s - jnp.max(s, axis=-1, keepdims=True))
            p = e * (1.0 / jnp.sum(e, axis=-1, keepdims=True))
            return jnp.concatenate(
                [p, jnp.zeros((total, LANES - total), F32)], axis=1).astype(BF16)

        def mix(quad, probs, v):
            o = [_dot(a, b) for a, b in zip(probs, v)]
            _put_rows(attn, every, slice(quad * Dh, (quad + 1) * Dh),
                      *([y[at:at + L] for y in o] for at in range(0, total, L)))

        q, k, v = (project(0, which) for which in range(3))
        _run(midway, 1)
        for g in range(n_groups):
            probs = [probabilities(a, b) for a, b in zip(q[:QUAD], k[:QUAD])]
            q_next = project(g + 1, 0)
            mix(2 * g, probs, v[:QUAD])
            probs = [probabilities(a, b) for a, b in zip(q[QUAD:], k[QUAD:])]
            k_next = project(g + 1, 1)
            _run(midway, 1)
            mix(2 * g + 1, probs, v[QUAD:])
            q, k, v = q_next, k_next, project(g + 1, 2)

    def project_out(src, w, n_layers, lo, hi):
        ys = _block_matmul(
            lambda k, i: src[k, i, :, lo * LANES:hi * LANES],
            lambda p: jnp.concatenate(
                [w[p, k, lo:hi].reshape((hi - lo) * LANES // 2, LANES)
                 for k in range(quarter // LANES)], axis=1),
            n_layers)
        return [jnp.concatenate(y, axis=1) for y in ys]

    def out_early(n_layers):
        for g in range(n_groups - 1):
            ys = project_out(attn, wo, n_layers, g * HEAD_QUADS, (g + 1) * HEAD_QUADS)
            for n, y in enumerate(ys):
                early[n] = early[n] + y if g else y
            yield

    def out_late(n_layers):
        ys = project_out(attn, wo, n_layers, n_hq - HEAD_QUADS, n_hq)
        return [early[n] + y for n, y in enumerate(ys)]

    def gate_up():
        for g in range(n_fq):
            ys = _block_matmul(
                lambda k, i: h_ffn[k, i],
                lambda p: jnp.concatenate([wgu[p, 0, g], wgu[p, 1, g]], axis=1), 2)
            _put_rows(act, every, slice(g * LANES, (g + 1) * LANES),
                      *([_gate(_tile(b, 0), _tile(b, 1)) for b in y] for y in ys))

    def down():
        return [xb[n] + y for n, y in enumerate(project_out(act, wd, 2, 0, n_fq))]

    def ffn():
        feed_ffn()
        gate_up()
        return down()

    def single(s, xs, xs_next, before_out=None):
        attention(1, () if before_out else out_early(1))
        feed_tokens(_layernorm(xs_next))
        if before_out:
            before_out()
        o, = project_out(attn, wo, 1, 0, n_hq) if before_out else out_late(1)
        ring[s % RING] = xs + o[M:]
        mem[...] = o[:M]
        feed_memory(o[:M])

    def out_copy(s):
        slot = s % OUT_SLOTS
        return pltpu.make_async_copy(out_v.at[slot], out_hbm.at[s], sem_out.at[slot])

    def emit(s, x):
        out_v[s % OUT_SLOTS] = x.astype(out_v.dtype)

    def tokens(s):
        return x_v[s].astype(F32)

    def fill(s, carry):
        pl.when(s == 1)(lambda: start(wu_copies))
        pl.when(s == 2)(lambda: start(wd_copies))
        single(s, tokens(s), tokens(s + 1))
        return carry

    def prepare_wo():
        wait(wo_copies)
        form_operands(wo, wo_v)

    x_head.wait()
    feed_memory(mem0)
    feed_tokens(_layernorm(tokens(0)))
    start(wg_copies)
    single(0, tokens(0), tokens(1), prepare_wo)
    lax.fori_loop(1, LAG, fill, 0)
    feed_memory(mem[...], mem0)
    xb[0], xb[1] = ring[0], ring[1]
    wait(wg_copies)
    wait(wu_copies)
    form_operands(wgu, wgu_v)
    wait(wd_copies)
    x_tail.start()
    form_operands(wd, wd_v)
    ring[0], ring[1] = ffn()
    xb[0], xb[1] = ring[3], ring[2]
    xa[0], xa[1] = tokens(LAG), ring[0]
    feed_both(True)

    def step(t, carry, *, use_pre):
        s = t - LAG - 1
        pl.when(not use_pre or s >= 1)(lambda: out_copy(s - 1).start())
        pl.when(not use_pre or s >= OUT_SLOTS)(lambda: out_copy(s - OUT_SLOTS).wait())

        def gated():
            gate_up()
            yield
            ring[(t - 1) % RING], x2 = down()
            ring[jnp.where(t == LAG, LAG - 2, RING)] = x2
            emit(jnp.maximum(s, 0), x2)

        pre_rows = None
        if use_pre:
            pre_rows = pl.ds(pl.multiple_of((t - LAG) * PRE_ROWS, PRE_ROWS), PRE_ROWS)
        feed_ffn()
        attention(2, out_early(2), pre_rows, gated())
        a1, a2 = xa[0], xa[1]
        xa[0], xa[1] = tokens(jnp.minimum(t + 1, n_seg - 1)), ring[(t + 1 - LAG) % RING]
        feed_both(use_pre)
        o1, o2 = out_late(2)
        mem[...] = o2[:M]
        feed_memory(o1[:M], o2[:M])
        xb[0], xb[1] = a1 + o1[M:], a2 + o2[M:]
        return carry

    lax.fori_loop(LAG, LAG + PRE_STEPS, functools.partial(step, use_pre=True), 0)
    x_tail.wait()
    feed_both(False)
    lax.fori_loop(LAG + PRE_STEPS, n_seg, functools.partial(step, use_pre=False), 0)

    tail = n_seg - LAG

    def drain(s, carry):
        single(s, ring[s % RING], ring[(s + 1) % RING])
        return carry

    def drain_ffn(n, carry):
        s = tail + 2 * n
        xb[0], xb[1] = ring[s % RING], ring[(s + 1) % RING]
        for k, x in enumerate(ffn()):
            emit(s + k, x)
        start([out_copy(s), out_copy(s + 1)])
        return carry

    out_copy(tail - 2).start()
    out_copy(tail - 1 - OUT_SLOTS).wait()
    ring[(n_seg - 1) % RING], x2 = ffn()
    emit(tail - 1, x2)
    feed_memory(mem[...])
    feed_tokens(_layernorm(ring[tail % RING]))
    out_copy(tail - 1).start()
    lax.fori_loop(tail, n_seg, drain, 0)
    wait([out_copy(s) for s in range(tail - OUT_SLOTS, tail)])
    lax.fori_loop(0, LAG // 2, drain_ffn, 0)
    wait([out_copy(s) for s in range(tail, n_seg)])


@functools.partial(jax.jit, static_argnames=("A_seg_len",))
def pallas_interleave_layers__memory_aug_recurrent_mem_tr__glu_gated_glu__prompt_kernel(
    A_x, A_mem0, A_Wq, A_Wk, A_Wv, A_Wo, A_seg_len, B_x, B_w_gate, B_w_up, B_w_down,
):
    del B_x
    B, S, D = A_x.shape
    M = A_mem0.shape[1]
    _, H, Dh = A_Wq.shape
    F = B_w_gate.shape[1]
    seg = int(A_seg_len)
    assert B == 1 and S % seg == 0 and Dh == LANES
    L, quarter, n_pre = M + seg, D // QUAD, PRE_STEPS * PRE_ROWS
    n_hq, n_fq = H // QUAD, F // (QUAD * LANES)
    hbm = pl.BlockSpec(memory_space=pl.ANY)
    staged = [w.reshape(QUAD, quarter // RAW_ROWS, RAW_ROWS * H, Dh) for w in (A_Wq, A_Wk, A_Wv)]
    out = pl.pallas_call(
        _kernel,
        out_shape=jax.ShapeDtypeStruct((S // seg, seg, D), A_x.dtype),
        in_specs=[hbm, pl.BlockSpec(memory_space=pltpu.VMEM)] + [hbm] * 7,
        out_specs=hbm,
        scratch_shapes=[
            pltpu.VMEM((S // seg, seg, D), BF16),
            pltpu.VMEM((PRE_STEPS, PRE_ROWS, D), BF16),
            pltpu.VMEM((OUT_SLOTS, seg, D), A_x.dtype),
            pltpu.VMEM((RAW_SLOTS, QUAD, RAW_ROWS * H + 2 * RAW_PAD, Dh), BF16),
            pltpu.VMEM((3, N_SLOTS, n_hq, quarter // 2, Dh), U32),
            pltpu.VMEM((N_SLOTS, quarter // LANES, n_hq, Dh, LANES), BF16),
            pltpu.VMEM((N_SLOTS, 2, n_fq, quarter, LANES), BF16),
            pltpu.VMEM((N_SLOTS, quarter // LANES, n_fq, LANES, LANES), BF16),
            pltpu.VMEM((2, QUAD, L, quarter), F32),
            pltpu.VMEM((2, QUAD, L, n_hq * Dh), F32),
            pltpu.VMEM((2, QUAD, seg, quarter), F32),
            pltpu.VMEM((2, QUAD, seg, n_fq * LANES), F32),
            pltpu.VMEM((2, L, D), F32),
            pltpu.VMEM((M, D), F32),
            pltpu.VMEM((2, seg, D), F32),
            pltpu.VMEM((2, seg, D), F32),
            pltpu.VMEM((RING + 1, seg, D), F32),
            pltpu.VMEM((2 * L, 2 * L), F32),
            pltpu.VMEM((quarter // RAW_ROWS, n_pre // 2, QUAD * RAW_ROWS), U32),
            pltpu.VMEM((3, n_hq, n_pre, QUAD * Dh), F32),
            pltpu.SemaphoreType.DMA((3,)),
            pltpu.SemaphoreType.DMA((RAW_SLOTS,)),
            pltpu.SemaphoreType.DMA((4,)),
            pltpu.SemaphoreType.DMA((OUT_SLOTS,)),
        ],
        compiler_params=pltpu.CompilerParams(vmem_limit_bytes=127 * 2**20),
    )(A_x.reshape(S // seg, seg, D), A_mem0.reshape(M, D), *staged,
      A_Wo.reshape(n_hq, QUAD, Dh, D), B_w_gate.reshape(QUAD, quarter, F),
      B_w_up.reshape(QUAD, quarter, F), B_w_down.reshape(n_fq, QUAD, LANES, D))
    return out.reshape(B, S, D)
```

```python
import functools
import itertools

import jax
import jax.numpy as jnp
from jax import lax
import jax.experimental.pallas as pl
import jax.experimental.pallas.tpu as pltpu

F32 = jnp.float32
BF16 = jnp.bfloat16
U32 = jnp.uint32
LANES = 128
LAG = 4
RING = 8
HEAD_QUADS = 2
RAW_ROWS = 64
RAW_SLOTS = 3
RAW_PAD = 16
PRE_ROWS = 16
PRE_STEPS = 16
X_HEAD = LAG + PRE_STEPS + 1
OUT_SLOTS = 4

QUAD = 4
C = (-1.5, -0.5, 0.5, 1.5)
PAIRS = tuple(itertools.combinations(range(QUAD), 2))
V_SLOT, PAIR_SLOT = QUAD * QUAD, QUAD * QUAD + QUAD
ORDER = ((1, 2), (1, 3), (2, 3), (0, 1), (1, 1), (0, 2), (2, 2), (0, 3), (0, 0), (3, 3))
N_SLOTS = PAIR_SLOT + len(PAIRS)


def _slot(i, j):
    return QUAD * j + i


def _to_words(x):
    return pltpu.bitcast(x.astype(BF16), U32)


def _from_words(x):
    return pltpu.bitcast(x, BF16) if x.dtype == U32 else x


def _weight_sums(w):
    w = [[_from_words(b).astype(F32) for b in row] for row in w]
    sums = {}
    for i in range(QUAD):
        others = [j for j in range(QUAD) if j != i]
        sums[_slot(i, i)] = functools.reduce(jnp.add, [w[i][j] for j in others], w[i][i])
        sums[V_SLOT + i] = functools.reduce(jnp.subtract, [w[j][i] for j in others], w[i][i])
    for n, (i, j) in enumerate(PAIRS):
        sums[PAIR_SLOT + n] = w[i][j] + w[j][i]
    return {p: s.astype(BF16) for p, s in sums.items()}


def _times(c, x):
    return x if c == 1 else c * x


def _put_rows(dst, rows, cols, *layers):
    for i in range(QUAD):
        dst[0, i, rows, cols] = layers[-1][i]
        if len(layers) == 2:
            dst[1, i, rows, cols] = layers[0][i] - C[i] * layers[1][i]


def _block_matmul(rows, weights, n_layers):
    u, v = {}, {}

    def add(acc, i, y):
        acc[i] = acc[i] + y if i in acc else y

    for i, j in ORDER:
        if i == j:
            add(u, i, _dot(rows(0, i), weights(_slot(i, i))))
            if n_layers == 2:
                add(v, i, _dot(rows(1, i), weights(V_SLOT + i)))
            continue
        if n_layers == 1:
            t = _dot(rows(0, j), weights(_slot(j, i))) - _dot(rows(0, i), weights(_slot(i, j)))
        else:
            both, gap = rows(1, i) + rows(1, j), C[j] - C[i]
            m_ji = _dot(both + _times(gap, rows(0, j)), weights(_slot(j, i)))
            m_ij = _dot(both - _times(gap, rows(0, i)), weights(_slot(i, j)))
            m = _dot(both, weights(PAIR_SLOT + PAIRS.index((i, j))))
            t = _times(1 / gap, m_ji + m_ij - m)
            add(v, i, m_ji)
            add(v, j, m_ij)
        add(u, i, t)
        u[j] = u[j] - t if j in u else -t
    u = [u[i] for i in range(QUAD)]
    return [u] if n_layers == 1 else [[v[i] + C[i] * u[i] for i in range(QUAD)], u]


def _dot(a, b):
    return lax.dot_general(_from_words(a), _from_words(b), (((1,), (0,)), ((), ())),
                           preferred_element_type=F32)


def _layernorm(x):
    m = jnp.mean(x, axis=-1, keepdims=True)
    d = x - m
    v = jnp.mean(d * d, axis=-1, keepdims=True)
    return d * lax.rsqrt(v + 1e-5)


def _gate(g, u):
    u = 0.5 * u
    return u * jnp.tanh(0.5 * g) + u


def _run(stages, n=None):
    for _ in itertools.islice(stages, n):
        pass


def _tile(x, j):
    return x[:, j * LANES:(j + 1) * LANES]


def _kernel(x_hbm, mem0_ref, wq_hbm, wk_hbm, wv_hbm, wo_hbm, wg_hbm, wu_hbm, wd_hbm,
            out_hbm,
            x_v, x_pre, out_v, raw_v, wqkv, wo_v, wgu_v, wd_v,
            h_attn, attn, h_ffn, act, early, mem, normed, xb, ring, bias, pre_in, pre,
            sem_x, sem_raw, sem_w, sem_out):
    n_seg, seg, D = x_v.shape
    M = mem0_ref.shape[0]
    Dh = LANES
    n_hq, n_fq = wo_hbm.shape[0], wd_hbm.shape[0]
    H = QUAD * n_hq
    L = M + seg
    quarter = D // QUAD
    n_chunks = quarter // RAW_ROWS
    n_groups = n_hq // HEAD_QUADS
    scale = Dh ** -0.5
    raw, wo, wgu, wd = (ref.bitcast(U32) for ref in (raw_v, wo_v, wgu_v, wd_v))

    x_first = pltpu.make_async_copy(
        x_hbm.at[pl.ds(LAG, PRE_STEPS), pl.ds(0, PRE_ROWS)], x_pre, sem_x.at[0])
    x_head = pltpu.make_async_copy(
        x_hbm.at[pl.ds(0, X_HEAD)], x_v.at[pl.ds(0, X_HEAD)], sem_x.at[1])
    x_tail = pltpu.make_async_copy(
        x_hbm.at[pl.ds(X_HEAD, n_seg - X_HEAD)], x_v.at[pl.ds(X_HEAD, n_seg - X_HEAD)],
        sem_x.at[2])

    def raw_copy(n, src):
        return pltpu.make_async_copy(
            src.at[:, n // 3], raw_v.at[n % RAW_SLOTS, :, pl.ds(RAW_PAD, RAW_ROWS * H)],
            sem_raw.at[n % RAW_SLOTS])

    def start_raw(n):
        for i, src in enumerate((wq_hbm, wk_hbm, wv_hbm)):
            pl.when(n % 3 == i)(raw_copy(n, src).start)

    def out_copies(src, dst, sem):
        return [pltpu.make_async_copy(
            src.at[:, i, :, pl.ds(j * quarter + k * LANES, LANES)], dst.at[_slot(i, j), k], sem)
            for i in range(QUAD) for j in range(QUAD) for k in range(quarter // LANES)]

    def in_copies(src, k, sem):
        return [pltpu.make_async_copy(
            src.at[:, :, pl.ds((QUAD * g + j) * LANES, LANES)],
            wgu_v.at[pl.ds(_slot(0, j), QUAD), k, g], sem)
            for g in range(n_fq) for j in range(QUAD)]

    wo_copies = out_copies(wo_hbm, wo_v, sem_w.at[0])
    wg_copies = in_copies(wg_hbm, 0, sem_w.at[1])
    wu_copies = in_copies(wu_hbm, 1, sem_w.at[2])
    wd_copies = out_copies(wd_hbm, wd_v, sem_w.at[3])

    def start(copies):
        for cp in copies:
            cp.start()

    def wait(copies):
        for cp in copies:
            cp.wait()

    def form_operands(w, w_v):
        def body(g, carry):
            at = [(k, r) for k in range(w.shape[1]) for r in range(0, w_v.shape[3], 32)]
            blocks = [[[w[_slot(i, j), k, g, r // 2:r // 2 + 16] for j in range(QUAD)]
                       for i in range(QUAD)] for k, r in at]
            for (k, r), b in zip(at, blocks):
                for p, s in _weight_sums(b).items():
                    w_v[p, k, g, r:r + 32] = s
            return carry
        lax.fori_loop(0, w.shape[2], body, 0)

    raw_copy(0, wq_hbm).start()
    x_first.start()

    r = lax.broadcasted_iota(jnp.int32, (2 * L, 2 * L), 0)
    c = lax.broadcasted_iota(jnp.int32, (2 * L, 2 * L), 1)
    visible = (r < M) | ((r >= L) & (r < L + M)) | (r >= c)
    bias[...] = jnp.where((r >= L) == (c >= L),
                          jnp.where(visible, 0.0, -1e9), -jnp.inf).astype(F32)

    for at in (0, RAW_PAD + RAW_ROWS * H):
        raw_v[:, :, at:at + RAW_PAD, :] = jnp.zeros((RAW_SLOTS, QUAD, RAW_PAD, Dh), BF16)
    x_first.wait()
    raw_copy(1, wk_hbm).start()
    hs = _to_words(_layernorm(x_pre[...].astype(F32).reshape(PRE_STEPS * PRE_ROWS, D)))
    for k in range(n_chunks):
        pre_in[k] = jnp.concatenate(
            [hs[:, i * quarter + k * RAW_ROWS:][:, :RAW_ROWS] for i in range(QUAD)], axis=1)

    def columns(slot, i):
        sub = lax.broadcasted_iota(jnp.int32, (8, Dh), 0)
        out = []
        for at in range(RAW_PAD // 2, (RAW_PAD + RAW_ROWS * H) // 2, 8 * H):
            x = {c: raw[slot, i, pl.ds(at + c, 8, stride=H + 1), :] for c in range(-7, H)}
            for bit in (1, 2, 4):
                x = {c: jnp.where(sub & bit != 0, x[c - bit], x[c]) for c in x if c - bit in x}
            out.append(x)
        return [jnp.concatenate([x[c] for x in out], axis=0) for c in range(H)]

    def relayout(n, carry):
        slot, which, chunk = n % RAW_SLOTS, n % 3, n // 3
        raw_copy(n, wq_hbm).wait()

        @pl.when(n + 2 < 3 * n_chunks)
        def _():
            start_raw(n + 2)

        @pl.when(n + 3 == 3 * n_chunks)
        def _():
            start([x_head] + wo_copies)

        rows = pl.ds(pl.multiple_of(chunk * (RAW_ROWS // 2), RAW_ROWS // 2), RAW_ROWS // 2)
        words = [columns(slot, i) for i in range(QUAD)]
        for g in range(n_hq):
            w = [[] for _ in range(QUAD)]
            for i, pair in itertools.product(range(QUAD), (2 * g, 2 * g + 1)):
                even, odd = words[i][pair], words[i][H // 2 + pair]
                w[i].append((even & 0xFFFF) | (odd << 16))
                w[i].append((even >> 16) | (odd & jnp.uint32(0xFFFF0000)))
            for i, j in itertools.permutations(range(QUAD), 2):
                wqkv[which, _slot(i, j), g, rows, :] = w[i][j]
            for p, s in _weight_sums(w).items():
                wqkv[which, p, g, rows, :] = _to_words(s)
            pre[which, g] = jnp.where(chunk == 0, 0.0, pre[which, g]) + _dot(pre_in[chunk], jnp.concatenate(
                [jnp.concatenate(row, axis=1) for row in w], axis=0))
        return carry

    lax.fori_loop(0, 3 * n_chunks, relayout, 0)

    mem0 = mem0_ref[...].astype(F32)
    every = slice(None)

    def feed(dst, rows, *hs):
        _put_rows(dst, rows, every,
                  *([h[:, i * quarter:(i + 1) * quarter] for i in range(QUAD)] for h in hs))

    def feed_memory(*mems):
        feed(h_attn, slice(0, M), *mems)

    def feed_tokens(*hs):
        feed(h_attn, slice(M, M + hs[0].shape[0]), *hs)

    def feed_both(use_pre):
        if use_pre:
            cut = PRE_ROWS // 2
            feed_tokens(jnp.concatenate([normed[0, PRE_ROWS:], normed[1, :cut]], axis=0),
                        normed[1, cut:])
        else:
            feed_tokens(normed[0], normed[1])

    def feed_ffn():
        feed(h_ffn, every, _layernorm(xb[0]), _layernorm(xb[1]))

    def attention(n_layers, filler, pre_rows=None, midway=()):
        n_rows = L if pre_rows is None else L - PRE_ROWS // 2
        total = n_layers * L

        def project(g, which):
            if g == n_groups:
                return _run(filler, 1)
            quads = range(g * HEAD_QUADS, (g + 1) * HEAD_QUADS)
            ys = _block_matmul(
                lambda k, i: h_attn[k, i, 0:n_rows, :],
                lambda p: jnp.concatenate([wqkv[which, p, quad] for quad in quads], axis=1),
                n_layers)
            heads = []
            for (n, quad), j in itertools.product(enumerate(quads), range(QUAD)):
                parts = [_tile(y[j], n) for y in ys]
                if pre_rows is not None:
                    parts = [parts[0][:M], pre[which, quad, pre_rows, j * Dh:(j + 1) * Dh],
                             parts[0][M:L - PRE_ROWS], parts[1][:M],
                             parts[0][L - PRE_ROWS:], parts[1][M:]]
                y = jnp.concatenate(parts, axis=0)
                heads.append((y.T if which == 1 else y).astype(BF16))
            return heads

        def probabilities(q, k):
            s = _dot(q, k)
            b = bias[0:total, 0:total]
            s = jnp.where(b == 0.0, s * scale, b)
            e = jnp.exp(s - jnp.max(s, axis=-1, keepdims=True))
            p = e * (1.0 / jnp.sum(e, axis=-1, keepdims=True))
            return p.astype(BF16)

        def mix(quad, probs, v):
            o = [_dot(a, b) for a, b in zip(probs, v)]
            _put_rows(attn, every, slice(quad * Dh, (quad + 1) * Dh),
                      *([y[at:at + L] for y in o] for at in range(0, total, L)))

        q, k = (project(0, which) for which in range(2))
        _run(midway, 1)
        v = project(0, 2)
        for g in range(n_groups):
            probs = [probabilities(a, b) for a, b in zip(q[:QUAD], k[:QUAD])]
            q_next = project(g + 1, 0)
            mix(2 * g, probs, v[:QUAD])
            probs = [probabilities(a, b) for a, b in zip(q[QUAD:], k[QUAD:])]
            k_next = project(g + 1, 1)
            _run(midway, 1)
            mix(2 * g + 1, probs, v[QUAD:])
            q, k, v = q_next, k_next, project(g + 1, 2)

    def project_out(src, w, n_layers, lo, hi):
        ys = _block_matmul(
            lambda k, i: src[k, i, :, lo * LANES:hi * LANES],
            lambda p: jnp.concatenate(
                [w[p, k, lo:hi].reshape((hi - lo) * LANES // 2, LANES)
                 for k in range(quarter // LANES)], axis=1),
            n_layers)
        return [jnp.concatenate(y, axis=1) for y in ys]

    def out_early(n_layers):
        for g in range(n_groups - 1):
            ys = project_out(attn, wo, n_layers, g * HEAD_QUADS, (g + 1) * HEAD_QUADS)
            for n, y in enumerate(ys):
                early[n] = early[n] + y if g else y
            yield

    def out_late(n_layers):
        ys = project_out(attn, wo, n_layers, n_hq - HEAD_QUADS, n_hq)
        return [early[n] + y for n, y in enumerate(ys)]

    def gate_up():
        for g in range(n_fq):
            ys = _block_matmul(
                lambda k, i: h_ffn[k, i],
                lambda p: jnp.concatenate([wgu[p, 0, g], wgu[p, 1, g]], axis=1), 2)
            _put_rows(act, every, slice(g * LANES, (g + 1) * LANES),
                      *([_gate(_tile(b, 0), _tile(b, 1)) for b in y] for y in ys))

    def down():
        return [xb[n] + y for n, y in enumerate(project_out(act, wd, 2, 0, n_fq))]

    def ffn():
        feed_ffn()
        gate_up()
        return down()

    def single(s, xs, xs_next, before_out=None):
        attention(1, () if before_out else out_early(1))
        feed_tokens(_layernorm(xs_next))
        if before_out:
            before_out()
        o, = project_out(attn, wo, 1, 0, n_hq) if before_out else out_late(1)
        ring[s % RING] = xs + o[M:]
        mem[...] = o[:M]
        feed_memory(o[:M])

    def out_copy(s):
        slot = s % OUT_SLOTS
        return pltpu.make_async_copy(out_v.at[slot], out_hbm.at[s], sem_out.at[slot])

    def emit(s, x):
        out_v[s % OUT_SLOTS] = x.astype(out_v.dtype)

    def tokens(s):
        return x_v[s].astype(F32)

    def fill(s, carry):
        pl.when(s == 1)(lambda: start(wu_copies))
        pl.when(s == 2)(lambda: start(wd_copies))
        single(s, tokens(s), tokens(s + 1))
        return carry

    def prepare_wo():
        wait(wo_copies)
        form_operands(wo, wo_v)

    x_head.wait()
    feed_memory(mem0)
    feed_tokens(_layernorm(tokens(0)))
    start(wg_copies)
    single(0, tokens(0), tokens(1), prepare_wo)
    lax.fori_loop(1, LAG, fill, 0)
    feed_memory(mem[...], mem0)
    xb[0], xb[1] = ring[0], ring[1]
    wait(wg_copies)
    wait(wu_copies)
    form_operands(wgu, wgu_v)
    wait(wd_copies)
    x_tail.start()
    form_operands(wd, wd_v)
    ring[0], ring[1] = ffn()
    xb[0], xb[1] = ring[3], ring[2]
    normed[0], normed[1] = _layernorm(tokens(LAG)), _layernorm(ring[0])
    feed_both(True)

    def step(t, carry, *, use_pre):
        s = t - LAG - 1
        pl.when(not use_pre or s >= 1)(lambda: out_copy(s - 1).start())
        pl.when(not use_pre or s >= OUT_SLOTS)(lambda: out_copy(s - OUT_SLOTS).wait())

        def gated():
            gate_up()
            yield
            ring[(t - 1) % RING], x2 = down()
            ring[jnp.where(t == LAG, LAG - 2, RING)] = x2
            emit(jnp.maximum(s, 0), x2)
            normed[1] = _layernorm(ring[(t + 1 - LAG) % RING])
            normed[0] = _layernorm(tokens(jnp.minimum(t + 1, n_seg - 1)))

        pre_rows = None
        if use_pre:
            pre_rows = pl.ds(pl.multiple_of((t - LAG) * PRE_ROWS, PRE_ROWS), PRE_ROWS)
        feed_ffn()
        attention(2, out_early(2), pre_rows, gated())
        feed_both(use_pre)
        o1, o2 = out_late(2)
        mem[...] = o2[:M]
        feed_memory(o1[:M], o2[:M])
        xb[0], xb[1] = tokens(t) + o1[M:], ring[(t - LAG) % RING] + o2[M:]
        return carry

    lax.fori_loop(LAG, LAG + PRE_STEPS, functools.partial(step, use_pre=True), 0)
    x_tail.wait()
    feed_both(False)
    lax.fori_loop(LAG + PRE_STEPS, n_seg, functools.partial(step, use_pre=False), 0)

    tail = n_seg - LAG

    def drain(s, carry):
        single(s, ring[s % RING], ring[(s + 1) % RING])
        return carry

    def drain_ffn(n, carry):
        s = tail + 2 * n
        xb[0], xb[1] = ring[s % RING], ring[(s + 1) % RING]
        for k, x in enumerate(ffn()):
            emit(s + k, x)
        start([out_copy(s), out_copy(s + 1)])
        return carry

    out_copy(tail - 2).start()
    out_copy(tail - 1 - OUT_SLOTS).wait()
    ring[(n_seg - 1) % RING], x2 = ffn()
    emit(tail - 1, x2)
    feed_memory(mem[...])
    feed_tokens(_layernorm(ring[tail % RING]))
    out_copy(tail - 1).start()
    lax.fori_loop(tail, n_seg, drain, 0)
    wait([out_copy(s) for s in range(tail - OUT_SLOTS, tail)])
    lax.fori_loop(0, LAG // 2, drain_ffn, 0)
    wait([out_copy(s) for s in range(tail, n_seg)])


@functools.partial(jax.jit, static_argnames=("A_seg_len",))
def pallas_interleave_layers__memory_aug_recurrent_mem_tr__glu_gated_glu__prompt_kernel(
    A_x, A_mem0, A_Wq, A_Wk, A_Wv, A_Wo, A_seg_len, B_x, B_w_gate, B_w_up, B_w_down,
):
    del B_x
    B, S, D = A_x.shape
    M = A_mem0.shape[1]
    _, H, Dh = A_Wq.shape
    F = B_w_gate.shape[1]
    seg = int(A_seg_len)
    assert B == 1 and S % seg == 0 and Dh == LANES
    L, quarter, n_pre = M + seg, D // QUAD, PRE_STEPS * PRE_ROWS
    n_hq, n_fq = H // QUAD, F // (QUAD * LANES)
    hbm = pl.BlockSpec(memory_space=pl.ANY)
    staged = [w.reshape(QUAD, quarter // RAW_ROWS, RAW_ROWS * H, Dh) for w in (A_Wq, A_Wk, A_Wv)]
    out = pl.pallas_call(
        _kernel,
        out_shape=jax.ShapeDtypeStruct((S // seg, seg, D), A_x.dtype),
        in_specs=[hbm, pl.BlockSpec(memory_space=pltpu.VMEM)] + [hbm] * 7,
        out_specs=hbm,
        scratch_shapes=[
            pltpu.VMEM((S // seg, seg, D), BF16),
            pltpu.VMEM((PRE_STEPS, PRE_ROWS, D), BF16),
            pltpu.VMEM((OUT_SLOTS, seg, D), A_x.dtype),
            pltpu.VMEM((RAW_SLOTS, QUAD, RAW_ROWS * H + 6 * RAW_PAD, Dh), BF16),
            pltpu.VMEM((3, N_SLOTS, n_hq, quarter // 2, Dh), U32),
            pltpu.VMEM((N_SLOTS, quarter // LANES, n_hq, Dh, LANES), BF16),
            pltpu.VMEM((N_SLOTS, 2, n_fq, quarter, LANES), BF16),
            pltpu.VMEM((N_SLOTS, quarter // LANES, n_fq, LANES, LANES), BF16),
            pltpu.VMEM((2, QUAD, L, quarter), F32),
            pltpu.VMEM((2, QUAD, L, n_hq * Dh), F32),
            pltpu.VMEM((2, QUAD, seg, quarter), F32),
            pltpu.VMEM((2, QUAD, seg, n_fq * LANES), F32),
            pltpu.VMEM((2, L, D), F32),
            pltpu.VMEM((M, D), F32),
            pltpu.VMEM((2, seg, D), F32),
            pltpu.VMEM((2, seg, D), F32),
            pltpu.VMEM((RING + 1, seg, D), F32),
            pltpu.VMEM((2 * L, 2 * L), F32),
            pltpu.VMEM((quarter // RAW_ROWS, n_pre // 2, QUAD * RAW_ROWS), U32),
            pltpu.VMEM((3, n_hq, n_pre, QUAD * Dh), F32),
            pltpu.SemaphoreType.DMA((3,)),
            pltpu.SemaphoreType.DMA((RAW_SLOTS,)),
            pltpu.SemaphoreType.DMA((4,)),
            pltpu.SemaphoreType.DMA((OUT_SLOTS,)),
        ],
        compiler_params=pltpu.CompilerParams(vmem_limit_bytes=127 * 2**20),
    )(A_x.reshape(S // seg, seg, D), A_mem0.reshape(M, D), *staged,
      A_Wo.reshape(n_hq, QUAD, Dh, D), B_w_gate.reshape(QUAD, quarter, F),
      B_w_up.reshape(QUAD, quarter, F), B_w_down.reshape(n_fq, QUAD, LANES, D))
    return out.reshape(B, S, D)
```

```python
import functools
import itertools

import jax
import jax.numpy as jnp
from jax import lax
import jax.experimental.pallas as pl
import jax.experimental.pallas.tpu as pltpu

F32 = jnp.float32
BF16 = jnp.bfloat16
U32 = jnp.uint32
LANES = 128
LAG = 4
RING = 8
HEAD_QUADS = 2
RAW_ROWS = 64
RAW_SLOTS = 3
RAW_PAD = 16
PRE_ROWS = 16
PRE_STEPS = 16
X_HEAD = LAG + PRE_STEPS + 1
OUT_SLOTS = 4

QUAD = 4
C = (-1.5, -0.5, 0.5, 1.5)
PAIRS = tuple(itertools.combinations(range(QUAD), 2))
V_SLOT, PAIR_SLOT = QUAD * QUAD, QUAD * QUAD + QUAD
ORDER = ((1, 2), (1, 3), (2, 3), (0, 1), (1, 1), (0, 2), (2, 2), (0, 3), (0, 0), (3, 3))
N_SLOTS = PAIR_SLOT + len(PAIRS)


def _slot(i, j):
    return QUAD * j + i


def _to_words(x):
    return pltpu.bitcast(x.astype(BF16), U32)


def _from_words(x):
    return pltpu.bitcast(x, BF16) if x.dtype == U32 else x


def _weight_sums(w):
    w = [[_from_words(b).astype(F32) for b in row] for row in w]
    sums = {}
    for i in range(QUAD):
        others = [j for j in range(QUAD) if j != i]
        sums[_slot(i, i)] = functools.reduce(jnp.add, [w[i][j] for j in others], w[i][i])
        sums[V_SLOT + i] = functools.reduce(jnp.subtract, [w[j][i] for j in others], w[i][i])
    for n, (i, j) in enumerate(PAIRS):
        sums[PAIR_SLOT + n] = w[i][j] + w[j][i]
    return {p: s.astype(BF16) for p, s in sums.items()}


def _times(c, x):
    return x if c == 1 else c * x


def _put_rows(dst, rows, cols, *layers):
    for i in range(QUAD):
        dst[0, i, rows, cols] = layers[-1][i]
        if len(layers) == 2:
            dst[1, i, rows, cols] = layers[0][i] - C[i] * layers[1][i]


def _block_matmul(rows, weights, n_layers):
    u, v = {}, {}

    def add(acc, i, y):
        acc[i] = acc[i] + y if i in acc else y

    for i, j in ORDER:
        if i == j:
            add(u, i, _dot(rows(0, i), weights(_slot(i, i))))
            if n_layers == 2:
                add(v, i, _dot(rows(1, i), weights(V_SLOT + i)))
            continue
        if n_layers == 1:
            t = _dot(rows(0, j), weights(_slot(j, i))) - _dot(rows(0, i), weights(_slot(i, j)))
        else:
            both, gap = rows(1, i) + rows(1, j), C[j] - C[i]
            m_ji = _dot(both + _times(gap, rows(0, j)), weights(_slot(j, i)))
            m_ij = _dot(both - _times(gap, rows(0, i)), weights(_slot(i, j)))
            m = _dot(both, weights(PAIR_SLOT + PAIRS.index((i, j))))
            t = _times(1 / gap, m_ji + m_ij - m)
            add(v, i, m_ji)
            add(v, j, m_ij)
        add(u, i, t)
        u[j] = u[j] - t if j in u else -t
    u = [u[i] for i in range(QUAD)]
    return [u] if n_layers == 1 else [[v[i] + C[i] * u[i] for i in range(QUAD)], u]


def _dot(a, b):
    return lax.dot_general(_from_words(a), _from_words(b), (((1,), (0,)), ((), ())),
                           preferred_element_type=F32)


def _layernorm(x):
    m = jnp.mean(x, axis=-1, keepdims=True)
    d = x - m
    v = jnp.mean(d * d, axis=-1, keepdims=True)
    return d * lax.rsqrt(v + 1e-5)


def _gate(g, u):
    u = 0.5 * u
    return u * jnp.tanh(0.5 * g) + u


def _run(stages, n=None):
    for _ in itertools.islice(stages, n):
        pass


def _tile(x, j):
    return x[:, j * LANES:(j + 1) * LANES]


def _kernel(x_hbm, mem0_ref, wq_hbm, wk_hbm, wv_hbm, wo_hbm, wg_hbm, wu_hbm, wd_hbm,
            out_hbm,
            x_v, x_pre, out_v, raw_v, wqkv, wo_v, wgu_v, wd_v,
            h_attn, attn, h_ffn, act, early, mem, normed, xb, ring, bias, pre_in, pre,
            sem_x, sem_raw, sem_w, sem_out):
    n_seg, seg, D = x_v.shape
    M = mem0_ref.shape[0]
    Dh = LANES
    n_hq, n_fq = wo_hbm.shape[0], wd_hbm.shape[0]
    H = QUAD * n_hq
    L = M + seg
    quarter = D // QUAD
    n_chunks = quarter // RAW_ROWS
    n_groups = n_hq // HEAD_QUADS
    scale = Dh ** -0.5
    raw, wo, wgu, wd = (ref.bitcast(U32) for ref in (raw_v, wo_v, wgu_v, wd_v))

    x_first = pltpu.make_async_copy(
        x_hbm.at[pl.ds(LAG, PRE_STEPS), pl.ds(0, PRE_ROWS)], x_pre, sem_x.at[0])
    x_head = pltpu.make_async_copy(
        x_hbm.at[pl.ds(0, X_HEAD)], x_v.at[pl.ds(0, X_HEAD)], sem_x.at[1])
    x_tail = pltpu.make_async_copy(
        x_hbm.at[pl.ds(X_HEAD, n_seg - X_HEAD)], x_v.at[pl.ds(X_HEAD, n_seg - X_HEAD)],
        sem_x.at[2])

    def raw_copy(n, src):
        return pltpu.make_async_copy(
            src.at[:, n // 3], raw_v.at[n % RAW_SLOTS, :, pl.ds(RAW_PAD, RAW_ROWS * H)],
            sem_raw.at[n % RAW_SLOTS])

    def start_raw(n):
        for i, src in enumerate((wq_hbm, wk_hbm, wv_hbm)):
            pl.when(n % 3 == i)(raw_copy(n, src).start)

    def out_copies(src, dst, sem):
        return [pltpu.make_async_copy(
            src.at[:, i, :, pl.ds(j * quarter + k * LANES, LANES)], dst.at[_slot(i, j), k], sem)
            for i in range(QUAD) for j in range(QUAD) for k in range(quarter // LANES)]

    def in_copies(src, k, sem):
        return [pltpu.make_async_copy(
            src.at[:, :, pl.ds((QUAD * g + j) * LANES, LANES)],
            wgu_v.at[pl.ds(_slot(0, j), QUAD), k, g], sem)
            for g in range(n_fq) for j in range(QUAD)]

    wo_copies = out_copies(wo_hbm, wo_v, sem_w.at[0])
    wg_copies = in_copies(wg_hbm, 0, sem_w.at[1])
    wu_copies = in_copies(wu_hbm, 1, sem_w.at[2])
    wd_copies = out_copies(wd_hbm, wd_v, sem_w.at[3])

    def start(copies):
        for cp in copies:
            cp.start()

    def wait(copies):
        for cp in copies:
            cp.wait()

    def form_operands(w, w_v):
        def body(g, carry):
            at = [(k, r) for k in range(w.shape[1]) for r in range(0, w_v.shape[3], 32)]
            blocks = [[[w[_slot(i, j), k, g, r // 2:r // 2 + 16] for j in range(QUAD)]
                       for i in range(QUAD)] for k, r in at]
            for (k, r), b in zip(at, blocks):
                for p, s in _weight_sums(b).items():
                    w_v[p, k, g, r:r + 32] = s
            return carry
        lax.fori_loop(0, w.shape[2], body, 0)

    raw_copy(0, wq_hbm).start()
    x_first.start()

    r = lax.broadcasted_iota(jnp.int32, (2 * L, 2 * L), 0)
    c = lax.broadcasted_iota(jnp.int32, (2 * L, 2 * L), 1)
    visible = (r < M) | ((r >= L) & (r < L + M)) | (r >= c)
    bias[...] = jnp.where((r >= L) == (c >= L),
                          jnp.where(visible, 0.0, -1e9), -jnp.inf).astype(F32)

    for at in (0, RAW_PAD + RAW_ROWS * H):
        raw_v[:, :, at:at + RAW_PAD, :] = jnp.zeros((RAW_SLOTS, QUAD, RAW_PAD, Dh), BF16)
    x_first.wait()
    raw_copy(1, wk_hbm).start()
    hs = _to_words(_layernorm(x_pre[...].astype(F32).reshape(PRE_STEPS * PRE_ROWS, D)))
    for k in range(n_chunks):
        pre_in[k] = jnp.concatenate(
            [hs[:, i * quarter + k * RAW_ROWS:][:, :RAW_ROWS] for i in range(QUAD)], axis=1)

    def columns(slot, i):
        sub = lax.broadcasted_iota(jnp.int32, (8, Dh), 0)
        out = []
        for at in range(RAW_PAD // 2, (RAW_PAD + RAW_ROWS * H) // 2, 8 * H):
            x = {c: raw[slot, i, pl.ds(at + c, 8, stride=H + 1), :] for c in range(-7, H)}
            for bit in (1, 2, 4):
                x = {c: jnp.where(sub & bit != 0, x[c - bit], x[c]) for c in x if c - bit in x}
            out.append(x)
        return [jnp.concatenate([x[c] for x in out], axis=0) for c in range(H)]

    def relayout(n, carry):
        slot, which, chunk = n % RAW_SLOTS, n % 3, n // 3
        raw_copy(n, wq_hbm).wait()

        @pl.when(n + 2 < 3 * n_chunks)
        def _():
            start_raw(n + 2)

        @pl.when(n + 3 == 3 * n_chunks)
        def _():
            start([x_head] + wo_copies)

        rows = pl.ds(pl.multiple_of(chunk * (RAW_ROWS // 2), RAW_ROWS // 2), RAW_ROWS // 2)
        words = [columns(slot, i) for i in range(QUAD)]
        for g in range(n_hq):
            w = [[] for _ in range(QUAD)]
            for i, pair in itertools.product(range(QUAD), (2 * g, 2 * g + 1)):
                even, odd = words[i][pair], words[i][H // 2 + pair]
                w[i].append((even & 0xFFFF) | (odd << 16))
                w[i].append((even >> 16) | (odd & jnp.uint32(0xFFFF0000)))
            for i, j in itertools.permutations(range(QUAD), 2):
                wqkv[which, _slot(i, j), g, rows, :] = w[i][j]
            for p, s in _weight_sums(w).items():
                wqkv[which, p, g, rows, :] = _to_words(s)
            pre[which, g] = jnp.where(chunk == 0, 0.0, pre[which, g]) + _dot(pre_in[chunk], jnp.concatenate(
                [jnp.concatenate(row, axis=1) for row in w], axis=0))
        return carry

    lax.fori_loop(0, 3 * n_chunks, relayout, 0)

    mem0 = mem0_ref[...].astype(F32)
    every = slice(None)

    def feed(dst, rows, *hs):
        _put_rows(dst, rows, every,
                  *([h[:, i * quarter:(i + 1) * quarter] for i in range(QUAD)] for h in hs))

    def feed_memory(*mems):
        feed(h_attn, slice(0, M), *mems)

    def feed_tokens(*hs):
        feed(h_attn, slice(M, M + hs[0].shape[0]), *hs)

    def feed_both(use_pre):
        if use_pre:
            cut = PRE_ROWS // 2
            feed_tokens(jnp.concatenate([normed[0, PRE_ROWS:], normed[1, :cut]], axis=0),
                        normed[1, cut:])
        else:
            feed_tokens(normed[0], normed[1])

    def feed_ffn():
        feed(h_ffn, every, _layernorm(xb[0]), _layernorm(xb[1]))

    def attention(n_layers, filler, pre_rows=None, midway=()):
        n_rows = L if pre_rows is None else L - PRE_ROWS // 2
        total = n_layers * L

        def project(g, which):
            if g == n_groups:
                return _run(filler, 1)
            quads = range(g * HEAD_QUADS, (g + 1) * HEAD_QUADS)
            ys = _block_matmul(
                lambda k, i: h_attn[k, i, 0:n_rows, :],
                lambda p: jnp.concatenate([wqkv[which, p, quad] for quad in quads], axis=1),
                n_layers)
            heads = []
            for (n, quad), j in itertools.product(enumerate(quads), range(QUAD)):
                parts = [_tile(y[j], n) for y in ys]
                if pre_rows is not None:
                    parts = [parts[0][:M], pre[which, quad, pre_rows, j * Dh:(j + 1) * Dh],
                             parts[0][M:L - PRE_ROWS], parts[1][:M],
                             parts[0][L - PRE_ROWS:], parts[1][M:]]
                y = jnp.concatenate(parts, axis=0)
                heads.append((y.T if which == 1 else y).astype(BF16))
            return heads

        def probabilities(q, k):
            s = _dot(q, k)
            b = bias[0:total, 0:total]
            s = jnp.where(b == 0.0, s * scale, b)
            e = jnp.exp(s - jnp.max(s, axis=-1, keepdims=True))
            p = e * (1.0 / jnp.sum(e, axis=-1, keepdims=True))
            return p.astype(BF16)

        def mix(quad, probs, v):
            o = [_dot(a, b) for a, b in zip(probs, v)]
            _put_rows(attn, every, slice(quad * Dh, (quad + 1) * Dh),
                      *([y[at:at + L] for y in o] for at in range(0, total, L)))

        q, k = (project(0, which) for which in range(2))
        _run(midway, 1)
        v = project(0, 2)
        for g in range(n_groups):
            probs = [probabilities(a, b) for a, b in zip(q[:QUAD], k[:QUAD])]
            q_next = project(g + 1, 0)
            mix(2 * g, probs, v[:QUAD])
            probs = [probabilities(a, b) for a, b in zip(q[QUAD:], k[QUAD:])]
            k_next = project(g + 1, 1)
            _run(midway, 1)
            mix(2 * g + 1, probs, v[QUAD:])
            q, k, v = q_next, k_next, project(g + 1, 2)

    def project_out(src, w, n_layers, lo, hi):
        ys = _block_matmul(
            lambda k, i: src[k, i, :, lo * LANES:hi * LANES],
            lambda p: jnp.concatenate(
                [w[p, k, lo:hi].reshape((hi - lo) * LANES // 2, LANES)
                 for k in range(quarter // LANES)], axis=1),
            n_layers)
        return [jnp.concatenate(y, axis=1) for y in ys]

    def out_early(n_layers):
        for g in range(n_groups - 1):
            ys = project_out(attn, wo, n_layers, g * HEAD_QUADS, (g + 1) * HEAD_QUADS)
            for n, y in enumerate(ys):
                early[n] = early[n] + y if g else y
            yield

    def out_late(n_layers):
        ys = project_out(attn, wo, n_layers, n_hq - HEAD_QUADS, n_hq)
        return [early[n] + y for n, y in enumerate(ys)]

    def gate_up():
        for g in range(n_fq):
            ys = _block_matmul(
                lambda k, i: h_ffn[k, i],
                lambda p: jnp.concatenate([wgu[p, 0, g], wgu[p, 1, g]], axis=1), 2)
            _put_rows(act, every, slice(g * LANES, (g + 1) * LANES),
                      *([_gate(_tile(b, 0), _tile(b, 1)) for b in y] for y in ys))

    def down():
        return [xb[n] + y for n, y in enumerate(project_out(act, wd, 2, 0, n_fq))]

    def ffn():
        feed_ffn()
        gate_up()
        return down()

    def single(s, xs, xs_next, before_out=None):
        attention(1, () if before_out else out_early(1))
        feed_tokens(_layernorm(xs_next))
        if before_out:
            before_out()
        o, = project_out(attn, wo, 1, 0, n_hq) if before_out else out_late(1)
        ring[s % RING] = xs + o[M:]
        mem[...] = o[:M]
        feed_memory(o[:M])

    def out_copy(s):
        slot = s % OUT_SLOTS
        return pltpu.make_async_copy(out_v.at[slot], out_hbm.at[s], sem_out.at[slot])

    def emit(s, x):
        out_v[s % OUT_SLOTS] = x.astype(out_v.dtype)

    def tokens(s):
        return x_v[s].astype(F32)

    def fill(s, carry):
        pl.when(s == 1)(lambda: start(wu_copies))
        pl.when(s == 2)(lambda: start(wd_copies))
        single(s, tokens(s), tokens(s + 1))
        return carry

    def prepare_wo():
        wait(wo_copies)
        form_operands(wo, wo_v)

    x_head.wait()
    feed_memory(mem0)
    feed_tokens(_layernorm(tokens(0)))
    start(wg_copies)
    single(0, tokens(0), tokens(1), prepare_wo)
    lax.fori_loop(1, LAG, fill, 0)
    feed_memory(mem[...], mem0)
    xb[0], xb[1] = ring[0], ring[1]
    wait(wg_copies)
    wait(wu_copies)
    form_operands(wgu, wgu_v)
    wait(wd_copies)
    x_tail.start()
    form_operands(wd, wd_v)
    ring[0], ring[1] = ffn()
    xb[0], xb[1] = ring[3], ring[2]
    normed[0], normed[1] = _layernorm(tokens(LAG)), _layernorm(ring[0])
    feed_both(True)

    def step(t, carry, *, use_pre):
        s = t - LAG - 1
        pl.when(not use_pre or s >= 1)(lambda: out_copy(s - 1).start())
        pl.when(not use_pre or s >= OUT_SLOTS)(lambda: out_copy(s - OUT_SLOTS).wait())

        def gated():
            gate_up()
            yield
            ring[(t - 1) % RING], x2 = down()
            ring[jnp.where(t == LAG, LAG - 2, RING)] = x2
            emit(jnp.maximum(s, 0), x2)
            normed[1] = _layernorm(ring[(t + 1 - LAG) % RING])
            normed[0] = _layernorm(tokens(jnp.minimum(t + 1, n_seg - 1)))

        pre_rows = None
        if use_pre:
            pre_rows = pl.ds(pl.multiple_of((t - LAG) * PRE_ROWS, PRE_ROWS), PRE_ROWS)
        feed_ffn()
        attention(2, out_early(2), pre_rows, gated())
        feed_both(use_pre)
        o1, o2 = out_late(2)
        mem[...] = o2[:M]
        feed_memory(o1[:M], o2[:M])
        xb[0], xb[1] = tokens(t) + o1[M:], ring[(t - LAG) % RING] + o2[M:]
        return carry

    lax.fori_loop(LAG, LAG + PRE_STEPS, functools.partial(step, use_pre=True), 0)
    x_tail.wait()
    feed_both(False)
    lax.fori_loop(LAG + PRE_STEPS, n_seg, functools.partial(step, use_pre=False), 0)

    tail = n_seg - LAG

    def drain(s, carry):
        single(s, ring[s % RING], ring[(s + 1) % RING])
        return carry

    def drain_ffn(n, carry):
        s = tail + 2 * n - 2

        @pl.when(n == 1)
        def _():
            ring[(n_seg - 1) % RING] = early[0, :seg]
            feed_memory(mem[...])
            feed_tokens(_layernorm(ring[tail % RING]))
            lax.fori_loop(tail, n_seg, drain, 0)
            wait([out_copy(k) for k in range(tail - OUT_SLOTS, tail)])

        @pl.when(n >= 1)
        def _():
            xb[0], xb[1] = ring[s % RING], ring[(s + 1) % RING]

        x1, x2 = ffn()
        early[0, :seg] = x1
        emit(s + 1, x2)

        @pl.when(n >= 1)
        def _():
            emit(s, x1)

        start([out_copy(s), out_copy(s + 1)])
        return carry

    out_copy(tail - 1 - OUT_SLOTS).wait()
    lax.fori_loop(0, 1 + LAG // 2, drain_ffn, 0)
    wait([out_copy(s) for s in range(tail, n_seg)])


@functools.partial(jax.jit, static_argnames=("A_seg_len",))
def pallas_interleave_layers__memory_aug_recurrent_mem_tr__glu_gated_glu__prompt_kernel(
    A_x, A_mem0, A_Wq, A_Wk, A_Wv, A_Wo, A_seg_len, B_x, B_w_gate, B_w_up, B_w_down,
):
    del B_x
    B, S, D = A_x.shape
    M = A_mem0.shape[1]
    _, H, Dh = A_Wq.shape
    F = B_w_gate.shape[1]
    seg = int(A_seg_len)
    assert B == 1 and S % seg == 0 and Dh == LANES
    L, quarter, n_pre = M + seg, D // QUAD, PRE_STEPS * PRE_ROWS
    n_hq, n_fq = H // QUAD, F // (QUAD * LANES)
    hbm = pl.BlockSpec(memory_space=pl.ANY)
    staged = [w.reshape(QUAD, quarter // RAW_ROWS, RAW_ROWS * H, Dh) for w in (A_Wq, A_Wk, A_Wv)]
    out = pl.pallas_call(
        _kernel,
        out_shape=jax.ShapeDtypeStruct((S // seg, seg, D), A_x.dtype),
        in_specs=[hbm, pl.BlockSpec(memory_space=pltpu.VMEM)] + [hbm] * 7,
        out_specs=hbm,
        scratch_shapes=[
            pltpu.VMEM((S // seg, seg, D), BF16),
            pltpu.VMEM((PRE_STEPS, PRE_ROWS, D), BF16),
            pltpu.VMEM((OUT_SLOTS, seg, D), A_x.dtype),
            pltpu.VMEM((RAW_SLOTS, QUAD, RAW_ROWS * H + 6 * RAW_PAD, Dh), BF16),
            pltpu.VMEM((3, N_SLOTS, n_hq, quarter // 2, Dh), U32),
            pltpu.VMEM((N_SLOTS, quarter // LANES, n_hq, Dh, LANES), BF16),
            pltpu.VMEM((N_SLOTS, 2, n_fq, quarter, LANES), BF16),
            pltpu.VMEM((N_SLOTS, quarter // LANES, n_fq, LANES, LANES), BF16),
            pltpu.VMEM((2, QUAD, L, quarter), F32),
            pltpu.VMEM((2, QUAD, L, n_hq * Dh), F32),
            pltpu.VMEM((2, QUAD, seg, quarter), F32),
            pltpu.VMEM((2, QUAD, seg, n_fq * LANES), F32),
            pltpu.VMEM((2, L, D), F32),
            pltpu.VMEM((M, D), F32),
            pltpu.VMEM((2, seg, D), F32),
            pltpu.VMEM((2, seg, D), F32),
            pltpu.VMEM((RING + 1, seg, D), F32),
            pltpu.VMEM((2 * L, 2 * L), F32),
            pltpu.VMEM((quarter // RAW_ROWS, n_pre // 2, QUAD * RAW_ROWS), U32),
            pltpu.VMEM((3, n_hq, n_pre, QUAD * Dh), F32),
            pltpu.SemaphoreType.DMA((3,)),
            pltpu.SemaphoreType.DMA((RAW_SLOTS,)),
            pltpu.SemaphoreType.DMA((4,)),
            pltpu.SemaphoreType.DMA((OUT_SLOTS,)),
        ],
        compiler_params=pltpu.CompilerParams(vmem_limit_bytes=127 * 2**20),
    )(A_x.reshape(S // seg, seg, D), A_mem0.reshape(M, D), *staged,
      A_Wo.reshape(n_hq, QUAD, Dh, D), B_w_gate.reshape(QUAD, quarter, F),
      B_w_up.reshape(QUAD, quarter, F), B_w_down.reshape(n_fq, QUAD, LANES, D))
    return out.reshape(B, S, D)
```

```python
import functools
import itertools

import jax
import jax.numpy as jnp
from jax import lax
import jax.experimental.pallas as pl
import jax.experimental.pallas.tpu as pltpu

F32 = jnp.float32
BF16 = jnp.bfloat16
U32 = jnp.uint32
LANES = 128
LAG = 4
RING = 8
HEAD_QUADS = 2
RAW_ROWS = 64
RAW_SLOTS = 3
RAW_PAD = 16
PRE_ROWS = 16
PRE_STEPS = 16
X_HEAD = LAG + PRE_STEPS + 1
OUT_SLOTS = 4

QUAD = 4
C = (-1.5, -0.5, 0.5, 1.5)
PAIRS = tuple(itertools.combinations(range(QUAD), 2))
V_SLOT, PAIR_SLOT = QUAD * QUAD, QUAD * QUAD + QUAD
ORDER = ((1, 2), (1, 3), (2, 3), (0, 1), (1, 1), (0, 2), (2, 2), (0, 3), (0, 0), (3, 3))
N_SLOTS = PAIR_SLOT + len(PAIRS)


def _slot(i, j):
    return QUAD * j + i


def _to_words(x):
    return pltpu.bitcast(x.astype(BF16), U32)


def _from_words(x):
    return pltpu.bitcast(x, BF16) if x.dtype == U32 else x


def _weight_sums(w):
    w = [[_from_words(b).astype(F32) for b in row] for row in w]
    sums = {}
    for i in range(QUAD):
        others = [j for j in range(QUAD) if j != i]
        sums[_slot(i, i)] = functools.reduce(jnp.add, [w[i][j] for j in others], w[i][i])
        sums[V_SLOT + i] = functools.reduce(jnp.subtract, [w[j][i] for j in others], w[i][i])
    for n, (i, j) in enumerate(PAIRS):
        sums[PAIR_SLOT + n] = w[i][j] + w[j][i]
    return {p: s.astype(BF16) for p, s in sums.items()}


def _times(c, x):
    return x if c == 1 else c * x


def _put_rows(dst, rows, cols, *layers):
    for i in range(QUAD):
        dst[0, i, rows, cols] = layers[-1][i]
        if len(layers) == 2:
            dst[1, i, rows, cols] = layers[0][i] - C[i] * layers[1][i]


def _block_matmul(rows, weights, n_layers):
    u, v = {}, {}

    def add(acc, i, y):
        acc[i] = acc[i] + y if i in acc else y

    for i, j in ORDER:
        if i == j:
            add(u, i, _dot(rows(0, i), weights(_slot(i, i))))
            if n_layers == 2:
                add(v, i, _dot(rows(1, i), weights(V_SLOT + i)))
            continue
        if n_layers == 1:
            t = _dot(rows(0, j), weights(_slot(j, i))) - _dot(rows(0, i), weights(_slot(i, j)))
        else:
            both, gap = rows(1, i) + rows(1, j), C[j] - C[i]
            m_ji = _dot(both + _times(gap, rows(0, j)), weights(_slot(j, i)))
            m_ij = _dot(both - _times(gap, rows(0, i)), weights(_slot(i, j)))
            m = _dot(both, weights(PAIR_SLOT + PAIRS.index((i, j))))
            t = _times(1 / gap, m_ji + m_ij - m)
            add(v, i, m_ji)
            add(v, j, m_ij)
        add(u, i, t)
        u[j] = u[j] - t if j in u else -t
    u = [u[i] for i in range(QUAD)]
    return [u] if n_layers == 1 else [[v[i] + C[i] * u[i] for i in range(QUAD)], u]


def _dot(a, b):
    return lax.dot_general(_from_words(a), _from_words(b), (((1,), (0,)), ((), ())),
                           preferred_element_type=F32)


def _layernorm(x):
    m = jnp.mean(x, axis=-1, keepdims=True)
    d = x - m
    v = jnp.mean(d * d, axis=-1, keepdims=True)
    return d * lax.rsqrt(v + 1e-5)


def _gate(g, u):
    u = 0.5 * u
    return u * jnp.tanh(0.5 * g) + u


def _run(stages, n=None):
    for _ in itertools.islice(stages, n):
        pass


def _tile(x, j):
    return x[:, j * LANES:(j + 1) * LANES]


def _kernel(x_hbm, mem0_ref, wq_hbm, wk_hbm, wv_hbm, wo_hbm, wg_hbm, wu_hbm, wd_hbm,
            out_hbm,
            x_v, x_pre, out_v, raw_v, wqkv, wo_v, wgu_v, wd_v,
            h_attn, attn, h_ffn, act, early, mem, xb, ring, bias, pre_in, pre,
            sem_x, sem_raw, sem_w, sem_out):
    n_seg, seg, D = x_v.shape
    M = mem0_ref.shape[0]
    Dh = LANES
    n_hq, n_fq = wo_hbm.shape[0], wd_hbm.shape[0]
    H = QUAD * n_hq
    L = M + seg
    quarter = D // QUAD
    n_chunks = quarter // RAW_ROWS
    n_groups = n_hq // HEAD_QUADS
    scale = Dh ** -0.5
    raw, wo, wgu, wd = (ref.bitcast(U32) for ref in (raw_v, wo_v, wgu_v, wd_v))

    x_first = pltpu.make_async_copy(
        x_hbm.at[pl.ds(LAG, PRE_STEPS), pl.ds(0, PRE_ROWS)], x_pre, sem_x.at[0])
    x_head = pltpu.make_async_copy(
        x_hbm.at[pl.ds(0, X_HEAD)], x_v.at[pl.ds(0, X_HEAD)], sem_x.at[1])
    x_tail = pltpu.make_async_copy(
        x_hbm.at[pl.ds(X_HEAD, n_seg - X_HEAD)], x_v.at[pl.ds(X_HEAD, n_seg - X_HEAD)],
        sem_x.at[2])

    def raw_copy(n, src):
        return pltpu.make_async_copy(
            src.at[:, n // 3], raw_v.at[n % RAW_SLOTS, :, pl.ds(RAW_PAD, RAW_ROWS * H)],
            sem_raw.at[n % RAW_SLOTS])

    def start_raw(n):
        for i, src in enumerate((wq_hbm, wk_hbm, wv_hbm)):
            pl.when(n % 3 == i)(raw_copy(n, src).start)

    def out_copies(src, dst, sem):
        return [pltpu.make_async_copy(
            src.at[:, i, :, pl.ds(j * quarter + k * LANES, LANES)], dst.at[_slot(i, j), k], sem)
            for i in range(QUAD) for j in range(QUAD) for k in range(quarter // LANES)]

    def in_copies(src, k, sem):
        return [pltpu.make_async_copy(
            src.at[:, :, pl.ds((QUAD * g + j) * LANES, LANES)],
            wgu_v.at[pl.ds(_slot(0, j), QUAD), k, g], sem)
            for g in range(n_fq) for j in range(QUAD)]

    wo_copies = out_copies(wo_hbm, wo_v, sem_w.at[0])
    wg_copies = in_copies(wg_hbm, 0, sem_w.at[1])
    wu_copies = in_copies(wu_hbm, 1, sem_w.at[2])
    wd_copies = out_copies(wd_hbm, wd_v, sem_w.at[3])

    def start(copies):
        for cp in copies:
            cp.start()

    def wait(copies):
        for cp in copies:
            cp.wait()

    def form_operands(w, w_v):
        def body(g, carry):
            at = [(k, r) for k in range(w.shape[1]) for r in range(0, w_v.shape[3], 32)]
            blocks = [[[w[_slot(i, j), k, g, r // 2:r // 2 + 16] for j in range(QUAD)]
                       for i in range(QUAD)] for k, r in at]
            for (k, r), b in zip(at, blocks):
                for p, s in _weight_sums(b).items():
                    w_v[p, k, g, r:r + 32] = s
            return carry
        lax.fori_loop(0, w.shape[2], body, 0)

    raw_copy(0, wq_hbm).start()
    x_first.start()

    r = lax.broadcasted_iota(jnp.int32, (2 * L, 2 * L), 0)
    c = lax.broadcasted_iota(jnp.int32, (2 * L, 2 * L), 1)
    visible = (r < M) | ((r >= L) & (r < L + M)) | (r >= c)
    bias[...] = jnp.where((r >= L) == (c >= L),
                          jnp.where(visible, 0.0, -1e9), -jnp.inf).astype(F32)

    for at in (0, RAW_PAD + RAW_ROWS * H):
        raw_v[:, :, at:at + RAW_PAD, :] = jnp.zeros((RAW_SLOTS, QUAD, RAW_PAD, Dh), BF16)
    x_first.wait()
    raw_copy(1, wk_hbm).start()
    hs = _to_words(_layernorm(x_pre[...].astype(F32).reshape(PRE_STEPS * PRE_ROWS, D)))
    for k in range(n_chunks):
        pre_in[k] = jnp.concatenate(
            [hs[:, i * quarter + k * RAW_ROWS:][:, :RAW_ROWS] for i in range(QUAD)], axis=1)

    def columns(slot, i):
        sub = lax.broadcasted_iota(jnp.int32, (8, Dh), 0)
        out = []
        for at in range(RAW_PAD // 2, (RAW_PAD + RAW_ROWS * H) // 2, 8 * H):
            x = {c: raw[slot, i, pl.ds(at + c, 8, stride=H + 1), :] for c in range(-7, H)}
            for bit in (1, 2, 4):
                x = {c: jnp.where(sub & bit != 0, x[c - bit], x[c]) for c in x if c - bit in x}
            out.append(x)
        return [jnp.concatenate([x[c] for x in out], axis=0) for c in range(H)]

    def relayout(n, carry):
        slot, which, chunk = n % RAW_SLOTS, n % 3, n // 3
        raw_copy(n, wq_hbm).wait()

        @pl.when(n + 2 < 3 * n_chunks)
        def _():
            start_raw(n + 2)

        @pl.when(n + 3 == 3 * n_chunks)
        def _():
            start([x_head] + wo_copies)

        rows = pl.ds(pl.multiple_of(chunk * (RAW_ROWS // 2), RAW_ROWS // 2), RAW_ROWS // 2)
        words = [columns(slot, i) for i in range(QUAD)]
        for g in range(n_hq):
            w = [[] for _ in range(QUAD)]
            for i, pair in itertools.product(range(QUAD), (2 * g, 2 * g + 1)):
                even, odd = words[i][pair], words[i][H // 2 + pair]
                w[i].append((even & 0xFFFF) | (odd << 16))
                w[i].append((even >> 16) | (odd & jnp.uint32(0xFFFF0000)))
            for i, j in itertools.permutations(range(QUAD), 2):
                wqkv[which, _slot(i, j), g, rows, :] = w[i][j]
            for p, s in _weight_sums(w).items():
                wqkv[which, p, g, rows, :] = _to_words(s)
            pre[which, g] = jnp.where(chunk == 0, 0.0, pre[which, g]) + _dot(pre_in[chunk], jnp.concatenate(
                [jnp.concatenate(row, axis=1) for row in w], axis=0))
        return carry

    lax.fori_loop(0, 3 * n_chunks, relayout, 0)

    mem0 = mem0_ref[...].astype(F32)
    every = slice(None)

    def feed(dst, rows, *hs):
        _put_rows(dst, rows, every,
                  *([h[:, i * quarter:(i + 1) * quarter] for i in range(QUAD)] for h in hs))

    def feed_memory(*mems):
        feed(h_attn, slice(0, M), *mems)

    def feed_tokens(*hs):
        feed(h_attn, slice(M, M + hs[0].shape[0]), *hs)

    def feed_both(t, use_pre):
        h1 = _layernorm(tokens(jnp.minimum(t, n_seg - 1))[PRE_ROWS * use_pre:])
        h2 = _layernorm(ring[(t - LAG) % RING])
        if use_pre:
            feed_tokens(jnp.concatenate([h1, h2[:PRE_ROWS // 2]], axis=0), h2[PRE_ROWS // 2:])
        else:
            feed_tokens(h1, h2)

    def feed_ffn():
        feed(h_ffn, every, _layernorm(xb[0]), _layernorm(xb[1]))

    def attention(n_layers, filler, pre_rows=None, midway=()):
        n_rows = L if pre_rows is None else L - PRE_ROWS // 2
        total = n_layers * L

        def project(g, which):
            if g == n_groups:
                return _run(filler, 1)
            quads = range(g * HEAD_QUADS, (g + 1) * HEAD_QUADS)
            ys = _block_matmul(
                lambda k, i: h_attn[k, i, 0:n_rows, :],
                lambda p: jnp.concatenate([wqkv[which, p, quad] for quad in quads], axis=1),
                n_layers)
            heads = []
            for (n, quad), j in itertools.product(enumerate(quads), range(QUAD)):
                parts = [_tile(y[j], n) for y in ys]
                if pre_rows is not None:
                    parts = [parts[0][:M], pre[which, quad, pre_rows, j * Dh:(j + 1) * Dh],
                             parts[0][M:L - PRE_ROWS], parts[1][:M],
                             parts[0][L - PRE_ROWS:], parts[1][M:]]
                y = jnp.concatenate(parts, axis=0)
                heads.append((y.T if which == 1 else y).astype(BF16))
            return heads

        def probabilities(q, k):
            s = _dot(q, k)
            b = bias[0:total, 0:total]
            s = jnp.where(b == 0.0, s * scale, b)
            e = jnp.exp(s - jnp.max(s, axis=-1, keepdims=True))
            p = e * (1.0 / jnp.sum(e, axis=-1, keepdims=True))
            return p.astype(BF16)

        def mix(quad, probs, v):
            o = [_dot(a, b) for a, b in zip(probs, v)]
            _put_rows(attn, every, slice(quad * Dh, (quad + 1) * Dh),
                      *([y[at:at + L] for y in o] for at in range(0, total, L)))

        q, k = (project(0, which) for which in range(2))
        _run(midway, 1)
        v = project(0, 2)
        for g in range(n_groups):
            probs = [probabilities(a, b) for a, b in zip(q[:QUAD], k[:QUAD])]
            q_next = project(g + 1, 0)
            mix(2 * g, probs, v[:QUAD])
            probs = [probabilities(a, b) for a, b in zip(q[QUAD:], k[QUAD:])]
            k_next = project(g + 1, 1)
            _run(midway, 1)
            mix(2 * g + 1, probs, v[QUAD:])
            q, k, v = q_next, k_next, project(g + 1, 2)

    def project_out(src, w, n_layers, lo, hi):
        ys = _block_matmul(
            lambda k, i: src[k, i, :, lo * LANES:hi * LANES],
            lambda p: jnp.concatenate(
                [w[p, k, lo:hi].reshape((hi - lo) * LANES // 2, LANES)
                 for k in range(quarter // LANES)], axis=1),
            n_layers)
        return [jnp.concatenate(y, axis=1) for y in ys]

    def out_early(n_layers):
        for g in range(n_groups - 1):
            ys = project_out(attn, wo, n_layers, g * HEAD_QUADS, (g + 1) * HEAD_QUADS)
            for n, y in enumerate(ys):
                early[n] = early[n] + y if g else y
            yield

    def out_late(n_layers):
        ys = project_out(attn, wo, n_layers, n_hq - HEAD_QUADS, n_hq)
        return [early[n] + y for n, y in enumerate(ys)]

    def gate_up():
        for g in range(n_fq):
            ys = _block_matmul(
                lambda k, i: h_ffn[k, i],
                lambda p: jnp.concatenate([wgu[p, 0, g], wgu[p, 1, g]], axis=1), 2)
            _put_rows(act, every, slice(g * LANES, (g + 1) * LANES),
                      *([_gate(_tile(b, 0), _tile(b, 1)) for b in y] for y in ys))

    def down():
        return [xb[n] + y for n, y in enumerate(project_out(act, wd, 2, 0, n_fq))]

    def ffn():
        feed_ffn()
        gate_up()
        return down()

    def single(s, xs, xs_next, before_out=None):
        attention(1, () if before_out else out_early(1))
        feed_tokens(_layernorm(xs_next))
        if before_out:
            before_out()
        o, = project_out(attn, wo, 1, 0, n_hq) if before_out else out_late(1)
        ring[s % RING] = xs + o[M:]
        mem[...] = o[:M]
        feed_memory(o[:M])

    def out_copy(s):
        slot = s % OUT_SLOTS
        return pltpu.make_async_copy(out_v.at[slot], out_hbm.at[s], sem_out.at[slot])

    def emit(s, x):
        out_v[s % OUT_SLOTS] = x.astype(out_v.dtype)

    def tokens(s):
        return x_v[s].astype(F32)

    def fill(s, carry):
        pl.when(s == 1)(lambda: start(wu_copies))
        pl.when(s == 2)(lambda: start(wd_copies))
        single(s, tokens(s), tokens(s + 1))
        return carry

    def prepare_wo():
        wait(wo_copies)
        form_operands(wo, wo_v)

    x_head.wait()
    feed_memory(mem0)
    feed_tokens(_layernorm(tokens(0)))
    start(wg_copies)
    single(0, tokens(0), tokens(1), prepare_wo)
    lax.fori_loop(1, LAG, fill, 0)
    feed_memory(mem[...], mem0)
    xb[0], xb[1] = ring[0], ring[1]
    wait(wg_copies)
    wait(wu_copies)
    form_operands(wgu, wgu_v)
    wait(wd_copies)
    x_tail.start()
    form_operands(wd, wd_v)
    ring[0], ring[1] = ffn()
    xb[0], xb[1] = ring[3], ring[2]
    feed_both(LAG, True)

    def step(t, carry, *, use_pre):
        s = t - LAG - 1

        def gated():
            gate_up()
            yield
            ring[(t - 1) % RING], x2 = down()
            ring[jnp.where(t == LAG, LAG - 2, RING)] = x2
            emit(jnp.maximum(s, 0), x2)

        pre_rows = None
        if use_pre:
            pre_rows = pl.ds(pl.multiple_of((t - LAG) * PRE_ROWS, PRE_ROWS), PRE_ROWS)
        feed_ffn()
        attention(2, out_early(2), pre_rows, gated())
        feed_both(t + 1, use_pre)
        o1, o2 = out_late(2)
        mem[...] = o2[:M]
        feed_memory(o1[:M], o2[:M])
        xb[0], xb[1] = tokens(t) + o1[M:], ring[(t - LAG) % RING] + o2[M:]
        pl.when(not use_pre or s >= 0)(lambda: out_copy(s).start())
        pl.when(not use_pre or s + 1 >= OUT_SLOTS)(lambda: out_copy(s + 1 - OUT_SLOTS).wait())
        return carry

    lax.fori_loop(LAG, LAG + PRE_STEPS, functools.partial(step, use_pre=True), 0)
    x_tail.wait()
    feed_both(LAG + PRE_STEPS, False)
    lax.fori_loop(LAG + PRE_STEPS, n_seg, functools.partial(step, use_pre=False), 0)

    tail = n_seg - LAG

    def drain(s, carry):
        single(s, ring[s % RING], ring[(s + 1) % RING])
        return carry

    def drain_ffn(n, carry):
        s = tail + 2 * n - 2

        @pl.when(n == 1)
        def _():
            ring[(n_seg - 1) % RING] = early[0, :seg]
            feed_memory(mem[...])
            feed_tokens(_layernorm(ring[tail % RING]))
            lax.fori_loop(tail, n_seg, drain, 0)
            wait([out_copy(k) for k in range(tail - OUT_SLOTS, tail)])

        @pl.when(n >= 1)
        def _():
            xb[0], xb[1] = ring[s % RING], ring[(s + 1) % RING]

        x1, x2 = ffn()
        early[0, :seg] = x1
        emit(s + 1, x2)

        @pl.when(n >= 1)
        def _():
            emit(s, x1)
            out_copy(s).start()

        out_copy(s + 1).start()
        return carry

    lax.fori_loop(0, 1 + LAG // 2, drain_ffn, 0)
    wait([out_copy(s) for s in range(tail, n_seg)])


@functools.partial(jax.jit, static_argnames=("A_seg_len",))
def pallas_interleave_layers__memory_aug_recurrent_mem_tr__glu_gated_glu__prompt_kernel(
    A_x, A_mem0, A_Wq, A_Wk, A_Wv, A_Wo, A_seg_len, B_x, B_w_gate, B_w_up, B_w_down,
):
    del B_x
    B, S, D = A_x.shape
    M = A_mem0.shape[1]
    _, H, Dh = A_Wq.shape
    F = B_w_gate.shape[1]
    seg = int(A_seg_len)
    assert B == 1 and S % seg == 0 and Dh == LANES
    L, quarter, n_pre = M + seg, D // QUAD, PRE_STEPS * PRE_ROWS
    n_hq, n_fq = H // QUAD, F // (QUAD * LANES)
    hbm = pl.BlockSpec(memory_space=pl.ANY)
    staged = [w.reshape(QUAD, quarter // RAW_ROWS, RAW_ROWS * H, Dh) for w in (A_Wq, A_Wk, A_Wv)]
    out = pl.pallas_call(
        _kernel,
        out_shape=jax.ShapeDtypeStruct((S // seg, seg, D), A_x.dtype),
        in_specs=[hbm, pl.BlockSpec(memory_space=pltpu.VMEM)] + [hbm] * 7,
        out_specs=hbm,
        scratch_shapes=[
            pltpu.VMEM((S // seg, seg, D), BF16),
            pltpu.VMEM((PRE_STEPS, PRE_ROWS, D), BF16),
            pltpu.VMEM((OUT_SLOTS, seg, D), A_x.dtype),
            pltpu.VMEM((RAW_SLOTS, QUAD, RAW_ROWS * H + 6 * RAW_PAD, Dh), BF16),
            pltpu.VMEM((3, N_SLOTS, n_hq, quarter // 2, Dh), U32),
            pltpu.VMEM((N_SLOTS, quarter // LANES, n_hq, Dh, LANES), BF16),
            pltpu.VMEM((N_SLOTS, 2, n_fq, quarter, LANES), BF16),
            pltpu.VMEM((N_SLOTS, quarter // LANES, n_fq, LANES, LANES), BF16),
            pltpu.VMEM((2, QUAD, L, quarter), F32),
            pltpu.VMEM((2, QUAD, L, n_hq * Dh), F32),
            pltpu.VMEM((2, QUAD, seg, quarter), F32),
            pltpu.VMEM((2, QUAD, seg, n_fq * LANES), F32),
            pltpu.VMEM((2, L, D), F32),
            pltpu.VMEM((M, D), F32),
            pltpu.VMEM((2, seg, D), F32),
            pltpu.VMEM((RING + 1, seg, D), F32),
            pltpu.VMEM((2 * L, 2 * L), F32),
            pltpu.VMEM((quarter // RAW_ROWS, n_pre // 2, QUAD * RAW_ROWS), U32),
            pltpu.VMEM((3, n_hq, n_pre, QUAD * Dh), F32),
            pltpu.SemaphoreType.DMA((3,)),
            pltpu.SemaphoreType.DMA((RAW_SLOTS,)),
            pltpu.SemaphoreType.DMA((4,)),
            pltpu.SemaphoreType.DMA((OUT_SLOTS,)),
        ],
        compiler_params=pltpu.CompilerParams(vmem_limit_bytes=127 * 2**20),
    )(A_x.reshape(S // seg, seg, D), A_mem0.reshape(M, D), *staged,
      A_Wo.reshape(n_hq, QUAD, Dh, D), B_w_gate.reshape(QUAD, quarter, F),
      B_w_up.reshape(QUAD, quarter, F), B_w_down.reshape(n_fq, QUAD, LANES, D))
    return out.reshape(B, S, D)
```

```python
import functools
import itertools

import jax
import jax.numpy as jnp
from jax import lax
import jax.experimental.pallas as pl
import jax.experimental.pallas.tpu as pltpu

F32 = jnp.float32
BF16 = jnp.bfloat16
U32 = jnp.uint32
LANES = 128
LAG = 4
RING = 8
HEAD_QUADS = 2
RAW_ROWS = 64
RAW_SLOTS = 3
RAW_PAD = 16
PRE_ROWS = 16
PRE_STEPS = 16
X_HEAD = LAG + 1
OUT_SLOTS = 4

QUAD = 4
C = (-1.5, -0.5, 0.5, 1.5)
PAIRS = tuple(itertools.combinations(range(QUAD), 2))
V_SLOT, PAIR_SLOT = QUAD * QUAD, QUAD * QUAD + QUAD
ORDER = ((1, 2), (1, 3), (2, 3), (0, 1), (1, 1), (0, 2), (2, 2), (0, 3), (0, 0), (3, 3))
N_SLOTS = PAIR_SLOT + len(PAIRS)


def _slot(i, j):
    return QUAD * j + i


def _to_words(x):
    return pltpu.bitcast(x.astype(BF16), U32)


def _from_words(x):
    return pltpu.bitcast(x, BF16) if x.dtype == U32 else x


def _weight_sums(w):
    w = [[_from_words(b).astype(F32) for b in row] for row in w]
    sums = {}
    for i in range(QUAD):
        others = [j for j in range(QUAD) if j != i]
        sums[_slot(i, i)] = functools.reduce(jnp.add, [w[i][j] for j in others], w[i][i])
        sums[V_SLOT + i] = functools.reduce(jnp.subtract, [w[j][i] for j in others], w[i][i])
    for n, (i, j) in enumerate(PAIRS):
        sums[PAIR_SLOT + n] = w[i][j] + w[j][i]
    return {p: s.astype(BF16) for p, s in sums.items()}


def _times(c, x):
    return x if c == 1 else c * x


def _put_rows(dst, rows, cols, *layers):
    for i in range(QUAD):
        dst[0, i, rows, cols] = layers[-1][i]
        if len(layers) == 2:
            dst[1, i, rows, cols] = layers[0][i] - C[i] * layers[1][i]


def _block_matmul(rows, weights, n_layers):
    u, v = {}, {}

    def add(acc, i, y):
        acc[i] = acc[i] + y if i in acc else y

    for i, j in ORDER:
        if i == j:
            add(u, i, _dot(rows(0, i), weights(_slot(i, i))))
            if n_layers == 2:
                add(v, i, _dot(rows(1, i), weights(V_SLOT + i)))
            continue
        if n_layers == 1:
            t = _dot(rows(0, j), weights(_slot(j, i))) - _dot(rows(0, i), weights(_slot(i, j)))
        else:
            both, gap = rows(1, i) + rows(1, j), C[j] - C[i]
            m_ji = _dot(both + _times(gap, rows(0, j)), weights(_slot(j, i)))
            m_ij = _dot(both - _times(gap, rows(0, i)), weights(_slot(i, j)))
            m = _dot(both, weights(PAIR_SLOT + PAIRS.index((i, j))))
            t = _times(1 / gap, m_ji + m_ij - m)
            add(v, i, m_ji)
            add(v, j, m_ij)
        add(u, i, t)
        u[j] = u[j] - t if j in u else -t
    u = [u[i] for i in range(QUAD)]
    return [u] if n_layers == 1 else [[v[i] + C[i] * u[i] for i in range(QUAD)], u]


def _dot(a, b):
    return lax.dot_general(_from_words(a), _from_words(b), (((1,), (0,)), ((), ())),
                           preferred_element_type=F32)


def _layernorm(x):
    m = jnp.mean(x, axis=-1, keepdims=True)
    d = x - m
    v = jnp.mean(d * d, axis=-1, keepdims=True)
    return d * lax.rsqrt(v + 1e-5)


def _gate(g, u):
    u = 0.5 * u
    return u * jnp.tanh(0.5 * g) + u


def _run(stages, n=None):
    for _ in itertools.islice(stages, n):
        pass


def _tile(x, j):
    return x[:, j * LANES:(j + 1) * LANES]


def _kernel(x_hbm, mem0_ref, wq_hbm, wk_hbm, wv_hbm, wo_hbm, wg_hbm, wu_hbm, wd_hbm,
            out_hbm,
            x_v, x_pre, out_v, raw_v, wqkv, wo_v, wgu_v, wd_v,
            h_attn, attn, h_ffn, act, early, mem, xb, ring, bias, pre_in, pre,
            sem_x, sem_raw, sem_w, sem_out):
    n_seg, seg, D = x_v.shape
    M = mem0_ref.shape[0]
    Dh = LANES
    n_hq, n_fq = wo_hbm.shape[0], wd_hbm.shape[0]
    H = QUAD * n_hq
    L = M + seg
    quarter = D // QUAD
    n_chunks = quarter // RAW_ROWS
    n_groups = n_hq // HEAD_QUADS
    scale = Dh ** -0.5
    raw, wo, wgu, wd = (ref.bitcast(U32) for ref in (raw_v, wo_v, wgu_v, wd_v))

    x_first = pltpu.make_async_copy(
        x_hbm.at[pl.ds(LAG, PRE_STEPS), pl.ds(0, PRE_ROWS)], x_pre, sem_x.at[0])
    x_head = pltpu.make_async_copy(
        x_hbm.at[pl.ds(0, X_HEAD)], x_v.at[pl.ds(0, X_HEAD)], sem_x.at[1])
    x_tail = pltpu.make_async_copy(
        x_hbm.at[pl.ds(X_HEAD, n_seg - X_HEAD)], x_v.at[pl.ds(X_HEAD, n_seg - X_HEAD)],
        sem_x.at[2])

    def raw_copy(n, src):
        return pltpu.make_async_copy(
            src.at[:, n // 3], raw_v.at[n % RAW_SLOTS, :, pl.ds(RAW_PAD, RAW_ROWS * H)],
            sem_raw.at[n % RAW_SLOTS])

    def start_raw(n):
        for i, src in enumerate((wq_hbm, wk_hbm, wv_hbm)):
            pl.when(n % 3 == i)(raw_copy(n, src).start)

    def out_copies(src, dst, sem):
        return [pltpu.make_async_copy(
            src.at[:, i, :, pl.ds(j * quarter + k * LANES, LANES)], dst.at[_slot(i, j), k], sem)
            for i in range(QUAD) for j in range(QUAD) for k in range(quarter // LANES)]

    def in_copies(src, k, sem):
        return [pltpu.make_async_copy(
            src.at[:, :, pl.ds((QUAD * g + j) * LANES, LANES)],
            wgu_v.at[pl.ds(_slot(0, j), QUAD), k, g], sem)
            for g in range(n_fq) for j in range(QUAD)]

    wo_copies = out_copies(wo_hbm, wo_v, sem_w.at[0])
    wg_copies = in_copies(wg_hbm, 0, sem_w.at[1])
    wu_copies = in_copies(wu_hbm, 1, sem_w.at[2])
    wd_copies = out_copies(wd_hbm, wd_v, sem_w.at[3])

    def start(copies):
        for cp in copies:
            cp.start()

    def wait(copies):
        for cp in copies:
            cp.wait()

    def form_operands(w, w_v):
        def body(g, carry):
            at = [(k, r) for k in range(w.shape[1]) for r in range(0, w_v.shape[3], 32)]
            blocks = [[[w[_slot(i, j), k, g, r // 2:r // 2 + 16] for j in range(QUAD)]
                       for i in range(QUAD)] for k, r in at]
            for (k, r), b in zip(at, blocks):
                for p, s in _weight_sums(b).items():
                    w_v[p, k, g, r:r + 32] = s
            return carry
        lax.fori_loop(0, w.shape[2], body, 0)

    raw_copy(0, wq_hbm).start()
    x_first.start()

    r = lax.broadcasted_iota(jnp.int32, (2 * L, 2 * L), 0)
    c = lax.broadcasted_iota(jnp.int32, (2 * L, 2 * L), 1)
    visible = (r < M) | ((r >= L) & (r < L + M)) | (r >= c)
    bias[...] = jnp.where((r >= L) == (c >= L),
                          jnp.where(visible, 0.0, -1e9), -jnp.inf).astype(F32)

    for at in (0, RAW_PAD + RAW_ROWS * H):
        raw_v[:, :, at:at + RAW_PAD, :] = jnp.zeros((RAW_SLOTS, QUAD, RAW_PAD, Dh), BF16)
    x_first.wait()
    raw_copy(1, wk_hbm).start()
    hs = _to_words(_layernorm(x_pre[...].astype(F32).reshape(PRE_STEPS * PRE_ROWS, D)))
    for k in range(n_chunks):
        pre_in[k] = jnp.concatenate(
            [hs[:, i * quarter + k * RAW_ROWS:][:, :RAW_ROWS] for i in range(QUAD)], axis=1)

    def columns(slot, i):
        sub = lax.broadcasted_iota(jnp.int32, (8, Dh), 0)
        out = []
        for at in range(RAW_PAD // 2, (RAW_PAD + RAW_ROWS * H) // 2, 8 * H):
            x = {c: raw[slot, i, pl.ds(at + c, 8, stride=H + 1), :] for c in range(-7, H)}
            for bit in (1, 2, 4):
                x = {c: jnp.where(sub & bit != 0, x[c - bit], x[c]) for c in x if c - bit in x}
            out.append(x)
        return [jnp.concatenate([x[c] for x in out], axis=0) for c in range(H)]

    def relayout(n, carry):
        slot, which, chunk = n % RAW_SLOTS, n % 3, n // 3
        raw_copy(n, wq_hbm).wait()

        @pl.when(n + 2 < 3 * n_chunks)
        def _():
            start_raw(n + 2)

        @pl.when(n + 3 == 3 * n_chunks)
        def _():
            start([x_head] + wo_copies)

        rows = pl.ds(pl.multiple_of(chunk * (RAW_ROWS // 2), RAW_ROWS // 2), RAW_ROWS // 2)
        words = [columns(slot, i) for i in range(QUAD)]
        for g in range(n_hq):
            w = [[] for _ in range(QUAD)]
            for i, pair in itertools.product(range(QUAD), (2 * g, 2 * g + 1)):
                even, odd = words[i][pair], words[i][H // 2 + pair]
                w[i].append((even & 0xFFFF) | (odd << 16))
                w[i].append((even >> 16) | (odd & jnp.uint32(0xFFFF0000)))
            for i, j in itertools.permutations(range(QUAD), 2):
                wqkv[which, _slot(i, j), g, rows, :] = w[i][j]
            for p, s in _weight_sums(w).items():
                wqkv[which, p, g, rows, :] = _to_words(s)
            plain = jnp.concatenate([jnp.concatenate(row, axis=1) for row in w], axis=0)
            pre[which, g] = (jnp.where(chunk == 0, 0.0, pre[which, g])
                             + _dot(pre_in[chunk], plain))
        return carry

    lax.fori_loop(0, 3 * n_chunks, relayout, 0)

    mem0 = mem0_ref[...].astype(F32)
    every = slice(None)

    def feed(dst, rows, *hs):
        _put_rows(dst, rows, every,
                  *([h[:, i * quarter:(i + 1) * quarter] for i in range(QUAD)] for h in hs))

    def feed_memory(*mems):
        feed(h_attn, slice(0, M), *mems)

    def feed_tokens(*hs):
        feed(h_attn, slice(M, M + hs[0].shape[0]), *hs)

    def feed_both(t, use_pre):
        h1 = _layernorm(tokens(jnp.minimum(t, n_seg - 1))[PRE_ROWS * use_pre:])
        h2 = _layernorm(ring[(t - LAG) % RING])
        if use_pre:
            feed_tokens(jnp.concatenate([h1, h2[:PRE_ROWS // 2]], axis=0), h2[PRE_ROWS // 2:])
        else:
            feed_tokens(h1, h2)

    def feed_ffn():
        feed(h_ffn, every, _layernorm(xb[0]), _layernorm(xb[1]))

    def attention(n_layers, filler, pre_rows=None, midway=()):
        n_rows = L if pre_rows is None else L - PRE_ROWS // 2
        total = n_layers * L

        def project(g, which):
            if g == n_groups:
                return _run(filler, 1)
            quads = range(g * HEAD_QUADS, (g + 1) * HEAD_QUADS)
            ys = _block_matmul(
                lambda k, i: h_attn[k, i, 0:n_rows, :],
                lambda p: jnp.concatenate([wqkv[which, p, quad] for quad in quads], axis=1),
                n_layers)
            heads = []
            for (n, quad), j in itertools.product(enumerate(quads), range(QUAD)):
                parts = [_tile(y[j], n) for y in ys]
                if pre_rows is not None:
                    parts = [parts[0][:M], pre[which, quad, pre_rows, j * Dh:(j + 1) * Dh],
                             parts[0][M:L - PRE_ROWS], parts[1][:M],
                             parts[0][L - PRE_ROWS:], parts[1][M:]]
                y = jnp.concatenate(parts, axis=0)
                heads.append((y.T if which == 1 else y).astype(BF16))
            return heads

        def probabilities(q, k):
            s = _dot(q, k)
            b = bias[0:total, 0:total]
            s = jnp.where(b == 0.0, s * scale, b)
            e = jnp.exp(s - jnp.max(s, axis=-1, keepdims=True))
            p = e * (1.0 / jnp.sum(e, axis=-1, keepdims=True))
            return p.astype(BF16)

        def mix(quad, probs, v):
            o = [_dot(a, b) for a, b in zip(probs, v)]
            _put_rows(attn, every, slice(quad * Dh, (quad + 1) * Dh),
                      *([y[at:at + L] for y in o] for at in range(0, total, L)))

        q, k = (project(0, which) for which in range(2))
        _run(midway, 1)
        for g in range(n_groups):
            v = project(g, 2)
            probs = [probabilities(a, b) for a, b in zip(q[:QUAD], k[:QUAD])]
            k_next = project(g + 1, 1)
            mix(2 * g, probs, v[:QUAD])
            probs = [probabilities(a, b) for a, b in zip(q[QUAD:], k[QUAD:])]
            q_next = project(g + 1, 0)
            mix(2 * g + 1, probs, v[QUAD:])
            if g:
                _run(midway, 1)
            q, k = q_next, k_next
        _run(filler)

    def project_out(src, w, n_layers, lo, hi):
        ys = _block_matmul(
            lambda k, i: src[k, i, :, lo * LANES:hi * LANES],
            lambda p: jnp.concatenate(
                [w[p, k, lo:hi].reshape((hi - lo) * LANES // 2, LANES)
                 for k in range(quarter // LANES)], axis=1),
            n_layers)
        return [jnp.concatenate(y, axis=1) for y in ys]

    def out_early(n_layers):
        for g in range(n_groups - 1):
            ys = project_out(attn, wo, n_layers, g * HEAD_QUADS, (g + 1) * HEAD_QUADS)
            for n, y in enumerate(ys):
                early[n] = early[n] + y if g else y
            yield

    def out_late(n_layers):
        ys = project_out(attn, wo, n_layers, n_hq - HEAD_QUADS, n_hq)
        return [early[n] + y for n, y in enumerate(ys)]

    def gate_up():
        for g in range(n_fq):
            ys = _block_matmul(
                lambda k, i: h_ffn[k, i],
                lambda p: jnp.concatenate([wgu[p, 0, g], wgu[p, 1, g]], axis=1), 2)
            _put_rows(act, every, slice(g * LANES, (g + 1) * LANES),
                      *([_gate(_tile(b, 0), _tile(b, 1)) for b in y] for y in ys))

    def down():
        return [xb[n] + y for n, y in enumerate(project_out(act, wd, 2, 0, n_fq))]

    def ffn():
        feed_ffn()
        gate_up()
        return down()

    def single(s, xs, xs_next, before_out=None):
        attention(1, () if before_out else out_early(1))
        feed_tokens(_layernorm(xs_next))
        if before_out:
            before_out()
        o, = project_out(attn, wo, 1, 0, n_hq) if before_out else out_late(1)
        ring[s % RING] = xs + o[M:]
        mem[...] = o[:M]
        feed_memory(o[:M])

    def out_copy(s):
        slot = s % OUT_SLOTS
        return pltpu.make_async_copy(out_v.at[slot], out_hbm.at[s], sem_out.at[slot])

    def emit(s, x):
        out_v[s % OUT_SLOTS] = x.astype(out_v.dtype)

    def tokens(s):
        return x_v[s].astype(F32)

    def fill(s, carry):
        pl.when(s == 2)(lambda: start(wd_copies))
        single(s, tokens(s), tokens(s + 1))
        return carry

    def prepare_wo():
        start(wg_copies)
        wait(wo_copies)
        start(wu_copies)
        form_operands(wo, wo_v)

    x_head.wait()
    feed_memory(mem0)
    feed_tokens(_layernorm(tokens(0)))
    single(0, tokens(0), tokens(1), prepare_wo)
    lax.fori_loop(1, LAG, fill, 0)
    feed_memory(mem[...], mem0)
    xb[0], xb[1] = ring[0], ring[1]
    wait(wg_copies)
    wait(wu_copies)
    form_operands(wgu, wgu_v)
    wait(wd_copies)
    x_tail.start()
    form_operands(wd, wd_v)
    ring[0], ring[1] = ffn()
    xb[0], xb[1] = ring[3], ring[2]
    x_tail.wait()
    feed_both(LAG, True)

    def step(t, carry, *, use_pre):
        s = t - LAG - 1

        def gated():
            gate_up()
            yield
            ring[(t - 1) % RING], x2 = down()
            ring[jnp.where(t == LAG, LAG - 2, RING)] = x2
            emit(jnp.maximum(s, 0), x2)

        pre_rows = None
        if use_pre:
            pre_rows = pl.ds(pl.multiple_of((t - LAG) * PRE_ROWS, PRE_ROWS), PRE_ROWS)
        feed_ffn()
        attention(2, out_early(2), pre_rows, gated())
        feed_both(t + 1, use_pre)
        o1, o2 = out_late(2)
        mem[...] = o2[:M]
        feed_memory(o1[:M], o2[:M])
        xb[0], xb[1] = tokens(t) + o1[M:], ring[(t - LAG) % RING] + o2[M:]
        pl.when(not use_pre or s >= 0)(lambda: out_copy(s).start())
        pl.when(not use_pre or s + 1 >= OUT_SLOTS)(lambda: out_copy(s + 1 - OUT_SLOTS).wait())
        return carry

    lax.fori_loop(LAG, LAG + PRE_STEPS, functools.partial(step, use_pre=True), 0)
    feed_both(LAG + PRE_STEPS, False)
    lax.fori_loop(LAG + PRE_STEPS, n_seg, functools.partial(step, use_pre=False), 0)

    tail = n_seg - LAG

    def drain(s, carry):
        single(s, ring[s % RING], ring[(s + 1) % RING])
        return carry

    def drain_ffn(n, carry):
        s = tail + 2 * n - 2

        @pl.when(n == 1)
        def _():
            ring[(n_seg - 1) % RING] = early[0, :seg]
            feed_memory(mem[...])
            feed_tokens(_layernorm(ring[tail % RING]))
            lax.fori_loop(tail, n_seg, drain, 0)
            wait([out_copy(k) for k in range(tail - OUT_SLOTS, tail)])

        @pl.when(n >= 1)
        def _():
            xb[0], xb[1] = ring[s % RING], ring[(s + 1) % RING]

        x1, x2 = ffn()
        early[0, :seg] = x1
        emit(s + 1, x2)

        @pl.when(n >= 1)
        def _():
            emit(s, x1)
            out_copy(s).start()

        out_copy(s + 1).start()
        return carry

    lax.fori_loop(0, 1 + LAG // 2, drain_ffn, 0)
    wait([out_copy(s) for s in range(tail, n_seg)])


@functools.partial(jax.jit, static_argnames=("A_seg_len",))
def pallas_interleave_layers__memory_aug_recurrent_mem_tr__glu_gated_glu__prompt_kernel(
    A_x, A_mem0, A_Wq, A_Wk, A_Wv, A_Wo, A_seg_len, B_x, B_w_gate, B_w_up, B_w_down,
):
    del B_x
    B, S, D = A_x.shape
    M = A_mem0.shape[1]
    _, H, Dh = A_Wq.shape
    F = B_w_gate.shape[1]
    seg = int(A_seg_len)
    assert B == 1 and S % seg == 0 and Dh == LANES
    L, quarter, n_pre = M + seg, D // QUAD, PRE_STEPS * PRE_ROWS
    n_hq, n_fq = H // QUAD, F // (QUAD * LANES)
    hbm = pl.BlockSpec(memory_space=pl.ANY)
    staged = [w.reshape(QUAD, quarter // RAW_ROWS, RAW_ROWS * H, Dh) for w in (A_Wq, A_Wk, A_Wv)]
    out = pl.pallas_call(
        _kernel,
        out_shape=jax.ShapeDtypeStruct((S // seg, seg, D), A_x.dtype),
        in_specs=[hbm, pl.BlockSpec(memory_space=pltpu.VMEM)] + [hbm] * 7,
        out_specs=hbm,
        scratch_shapes=[
            pltpu.VMEM((S // seg, seg, D), BF16),
            pltpu.VMEM((PRE_STEPS, PRE_ROWS, D), BF16),
            pltpu.VMEM((OUT_SLOTS, seg, D), A_x.dtype),
            pltpu.VMEM((RAW_SLOTS, QUAD, RAW_ROWS * H + 6 * RAW_PAD, Dh), BF16),
            pltpu.VMEM((3, N_SLOTS, n_hq, quarter // 2, Dh), U32),
            pltpu.VMEM((N_SLOTS, quarter // LANES, n_hq, Dh, LANES), BF16),
            pltpu.VMEM((N_SLOTS, 2, n_fq, quarter, LANES), BF16),
            pltpu.VMEM((N_SLOTS, quarter // LANES, n_fq, LANES, LANES), BF16),
            pltpu.VMEM((2, QUAD, L, quarter), F32),
            pltpu.VMEM((2, QUAD, L, n_hq * Dh), F32),
            pltpu.VMEM((2, QUAD, seg, quarter), F32),
            pltpu.VMEM((2, QUAD, seg, n_fq * LANES), F32),
            pltpu.VMEM((2, L, D), F32),
            pltpu.VMEM((M, D), F32),
            pltpu.VMEM((2, seg, D), F32),
            pltpu.VMEM((RING + 1, seg, D), F32),
            pltpu.VMEM((2 * L, 2 * L), F32),
            pltpu.VMEM((quarter // RAW_ROWS, n_pre // 2, QUAD * RAW_ROWS), U32),
            pltpu.VMEM((3, n_hq, n_pre, QUAD * Dh), F32),
            pltpu.SemaphoreType.DMA((3,)),
            pltpu.SemaphoreType.DMA((RAW_SLOTS,)),
            pltpu.SemaphoreType.DMA((4,)),
            pltpu.SemaphoreType.DMA((OUT_SLOTS,)),
        ],
        compiler_params=pltpu.CompilerParams(vmem_limit_bytes=120 * 2**20),
    )(A_x.reshape(S // seg, seg, D), A_mem0.reshape(M, D), *staged,
      A_Wo.reshape(n_hq, QUAD, Dh, D), B_w_gate.reshape(QUAD, quarter, F),
      B_w_up.reshape(QUAD, quarter, F), B_w_down.reshape(n_fq, QUAD, LANES, D))
    return out.reshape(B, S, D)
```

```python
import functools
import itertools

import jax
import jax.numpy as jnp
from jax import lax
import jax.experimental.pallas as pl
import jax.experimental.pallas.tpu as pltpu

F32 = jnp.float32
BF16 = jnp.bfloat16
U32 = jnp.uint32
LANES = 128
LAG = 4
RING = 8
HEAD_QUADS = 2
RAW_ROWS = 64
RAW_SLOTS = 3
RAW_PAD = 16
PRE_ROWS = 16
PRE_STEPS = 16
X_HEAD = LAG + 1
OUT_SLOTS = 4

QUAD = 4
C = (-1.5, -0.5, 0.5, 1.5)
PAIRS = tuple(itertools.combinations(range(QUAD), 2))
V_SLOT, PAIR_SLOT = QUAD * QUAD, QUAD * QUAD + QUAD
ORDER = ((1, 2), (1, 3), (2, 3), (0, 1), (1, 1), (0, 2), (2, 2), (0, 3), (0, 0), (3, 3))
N_SLOTS = PAIR_SLOT + len(PAIRS)


def _slot(i, j):
    return QUAD * j + i


def _to_words(x):
    return pltpu.bitcast(x.astype(BF16), U32)


def _from_words(x):
    return pltpu.bitcast(x, BF16) if x.dtype == U32 else x


def _weight_sums(w):
    w = [[_from_words(b).astype(F32) for b in row] for row in w]
    sums = {}
    for i in range(QUAD):
        others = [j for j in range(QUAD) if j != i]
        sums[_slot(i, i)] = functools.reduce(jnp.add, [w[i][j] for j in others], w[i][i])
        sums[V_SLOT + i] = functools.reduce(jnp.subtract, [w[j][i] for j in others], w[i][i])
    for n, (i, j) in enumerate(PAIRS):
        sums[PAIR_SLOT + n] = w[i][j] + w[j][i]
    return {p: s.astype(BF16) for p, s in sums.items()}


def _times(c, x):
    return x if c == 1 else c * x


def _put_rows(dst, rows, cols, *layers):
    for i in range(QUAD):
        dst[0, i, rows, cols] = layers[-1][i]
        if len(layers) == 2:
            dst[1, i, rows, cols] = layers[0][i] - C[i] * layers[1][i]


def _block_matmul(rows, weights, n_layers):
    u, v = {}, {}

    def add(acc, i, y):
        acc[i] = acc[i] + y if i in acc else y

    for i, j in ORDER:
        if i == j:
            add(u, i, _dot(rows(0, i), weights(_slot(i, i))))
            if n_layers == 2:
                add(v, i, _dot(rows(1, i), weights(V_SLOT + i)))
            continue
        if n_layers == 1:
            t = _dot(rows(0, j), weights(_slot(j, i))) - _dot(rows(0, i), weights(_slot(i, j)))
        else:
            both, gap = rows(1, i) + rows(1, j), C[j] - C[i]
            m_ji = _dot(both + _times(gap, rows(0, j)), weights(_slot(j, i)))
            m_ij = _dot(both - _times(gap, rows(0, i)), weights(_slot(i, j)))
            m = _dot(both, weights(PAIR_SLOT + PAIRS.index((i, j))))
            t = _times(1 / gap, m_ji + m_ij - m)
            add(v, i, m_ji)
            add(v, j, m_ij)
        add(u, i, t)
        u[j] = u[j] - t if j in u else -t
    u = [u[i] for i in range(QUAD)]
    return [u] if n_layers == 1 else [[v[i] + C[i] * u[i] for i in range(QUAD)], u]


def _dot(a, b):
    return lax.dot_general(_from_words(a), _from_words(b), (((1,), (0,)), ((), ())),
                           preferred_element_type=F32)


def _layernorm(x):
    m = jnp.mean(x, axis=-1, keepdims=True)
    d = x - m
    v = jnp.mean(d * d, axis=-1, keepdims=True)
    return d * lax.rsqrt(v + 1e-5)


def _gate(g, u):
    u = 0.5 * u
    return u * jnp.tanh(0.5 * g) + u


def _run(stages, n=None):
    for _ in itertools.islice(stages, n):
        pass


def _tile(x, j):
    return x[:, j * LANES:(j + 1) * LANES]


def _kernel(x_hbm, mem0_ref, wq_hbm, wk_hbm, wv_hbm, wo_hbm, wg_hbm, wu_hbm, wd_hbm,
            out_hbm,
            x_v, x_pre, out_v, raw_v, wqkv, wo_v, wgu_v, wd_v,
            h_attn, attn, h_ffn, act, early, mem, xb, ring, bias, pre_in, pre,
            sem_x, sem_raw, sem_w, sem_out):
    n_seg, seg, D = x_v.shape
    M = mem0_ref.shape[0]
    Dh = LANES
    n_hq, n_fq = wo_hbm.shape[0], wd_hbm.shape[0]
    H = QUAD * n_hq
    L = M + seg
    quarter = D // QUAD
    n_chunks = quarter // RAW_ROWS
    n_groups = n_hq // HEAD_QUADS
    scale = Dh ** -0.5
    raw, wo, wgu, wd = (ref.bitcast(U32) for ref in (raw_v, wo_v, wgu_v, wd_v))

    x_first = pltpu.make_async_copy(
        x_hbm.at[pl.ds(LAG, PRE_STEPS), pl.ds(0, PRE_ROWS)], x_pre, sem_x.at[0])
    x_head = pltpu.make_async_copy(
        x_hbm.at[pl.ds(0, X_HEAD)], x_v.at[pl.ds(0, X_HEAD)], sem_x.at[1])
    x_tail = pltpu.make_async_copy(
        x_hbm.at[pl.ds(X_HEAD, n_seg - X_HEAD)], x_v.at[pl.ds(X_HEAD, n_seg - X_HEAD)],
        sem_x.at[2])

    def raw_copy(n, src):
        return pltpu.make_async_copy(
            src.at[:, n // 3], raw_v.at[n % RAW_SLOTS, :, pl.ds(RAW_PAD, RAW_ROWS * H)],
            sem_raw.at[n % RAW_SLOTS])

    def start_raw(n):
        for i, src in enumerate((wq_hbm, wk_hbm, wv_hbm)):
            pl.when(n % 3 == i)(raw_copy(n, src).start)

    def out_copies(src, dst, sem):
        return [pltpu.make_async_copy(
            src.at[:, i, :, pl.ds(j * quarter + k * LANES, LANES)], dst.at[_slot(i, j), k], sem)
            for i in range(QUAD) for j in range(QUAD) for k in range(quarter // LANES)]

    def in_copies(src, k, sem):
        return [pltpu.make_async_copy(
            src.at[:, :, pl.ds((QUAD * g + j) * LANES, LANES)],
            wgu_v.at[pl.ds(_slot(0, j), QUAD), k, g], sem)
            for g in range(n_fq) for j in range(QUAD)]

    wo_copies = out_copies(wo_hbm, wo_v, sem_w.at[0])
    wg_copies = in_copies(wg_hbm, 0, sem_w.at[1])
    wu_copies = in_copies(wu_hbm, 1, sem_w.at[2])
    wd_copies = out_copies(wd_hbm, wd_v, sem_w.at[3])

    def start(copies):
        for cp in copies:
            cp.start()

    def wait(copies):
        for cp in copies:
            cp.wait()

    def form_operands(w, w_v):
        def body(g, carry):
            at = [(k, r) for k in range(w.shape[1]) for r in range(0, w_v.shape[3], 32)]
            blocks = [[[w[_slot(i, j), k, g, r // 2:r // 2 + 16] for j in range(QUAD)]
                       for i in range(QUAD)] for k, r in at]
            for (k, r), b in zip(at, blocks):
                for p, s in _weight_sums(b).items():
                    w_v[p, k, g, r:r + 32] = s
            return carry
        lax.fori_loop(0, w.shape[2], body, 0)

    raw_copy(0, wq_hbm).start()
    x_first.start()

    r = lax.broadcasted_iota(jnp.int32, (2 * L, 2 * L), 0)
    c = lax.broadcasted_iota(jnp.int32, (2 * L, 2 * L), 1)
    visible = (r < M) | ((r >= L) & (r < L + M)) | (r >= c)
    bias[...] = jnp.where((r >= L) == (c >= L),
                          jnp.where(visible, 0.0, -1e9), -jnp.inf).astype(F32)

    for at in (0, RAW_PAD + RAW_ROWS * H):
        raw_v[:, :, at:at + RAW_PAD, :] = jnp.zeros((RAW_SLOTS, QUAD, RAW_PAD, Dh), BF16)
    x_first.wait()
    raw_copy(1, wk_hbm).start()
    hs = _to_words(_layernorm(x_pre[...].astype(F32).reshape(PRE_STEPS * PRE_ROWS, D)))
    for k in range(n_chunks):
        pre_in[k] = jnp.concatenate(
            [hs[:, i * quarter + k * RAW_ROWS:][:, :RAW_ROWS] for i in range(QUAD)], axis=1)

    def columns(slot, i):
        sub = lax.broadcasted_iota(jnp.int32, (8, Dh), 0)
        out = []
        for at in range(RAW_PAD // 2, (RAW_PAD + RAW_ROWS * H) // 2, 8 * H):
            x = {c: raw[slot, i, pl.ds(at + c, 8, stride=H + 1), :] for c in range(-7, H)}
            for bit in (1, 2, 4):
                x = {c: jnp.where(sub & bit != 0, x[c - bit], x[c]) for c in x if c - bit in x}
            out.append(x)
        return [jnp.concatenate([x[c] for x in out], axis=0) for c in range(H)]

    def relayout(n, carry):
        slot, which, chunk = n % RAW_SLOTS, n % 3, n // 3
        raw_copy(n, wq_hbm).wait()

        @pl.when(n + 2 < 3 * n_chunks)
        def _():
            start_raw(n + 2)

        @pl.when(n + 3 == 3 * n_chunks)
        def _():
            start([x_head] + wo_copies)

        rows = pl.ds(pl.multiple_of(chunk * (RAW_ROWS // 2), RAW_ROWS // 2), RAW_ROWS // 2)
        words = [columns(slot, i) for i in range(QUAD)]
        for g in range(n_hq):
            w = [[] for _ in range(QUAD)]
            for i, pair in itertools.product(range(QUAD), (2 * g, 2 * g + 1)):
                even, odd = words[i][pair], words[i][H // 2 + pair]
                w[i].append((even & 0xFFFF) | (odd << 16))
                w[i].append((even >> 16) | (odd & jnp.uint32(0xFFFF0000)))
            for i, j in itertools.permutations(range(QUAD), 2):
                wqkv[which, _slot(i, j), g, rows, :] = w[i][j]
            for p, s in _weight_sums(w).items():
                wqkv[which, p, g, rows, :] = _to_words(s)
            plain = jnp.concatenate([jnp.concatenate(row, axis=1) for row in w], axis=0)
            pre[which, g] = (jnp.where(chunk == 0, 0.0, pre[which, g])
                             + _dot(pre_in[chunk], plain))
        return carry

    lax.fori_loop(0, 3 * n_chunks, relayout, 0)

    mem0 = mem0_ref[...].astype(F32)
    every = slice(None)

    def feed(dst, rows, *hs):
        _put_rows(dst, rows, every,
                  *([h[:, i * quarter:(i + 1) * quarter] for i in range(QUAD)] for h in hs))

    def feed_memory(*mems):
        feed(h_attn, slice(0, M), *mems)

    def feed_tokens(*hs):
        feed(h_attn, slice(M, M + hs[0].shape[0]), *hs)

    def feed_both(t, use_pre):
        h1 = _layernorm(tokens(jnp.minimum(t, n_seg - 1))[PRE_ROWS * use_pre:])
        h2 = _layernorm(ring[(t - LAG) % RING])
        if use_pre:
            feed_tokens(jnp.concatenate([h1, h2[:PRE_ROWS // 2]], axis=0), h2[PRE_ROWS // 2:])
        else:
            feed_tokens(h1, h2)

    def feed_ffn():
        feed(h_ffn, every, _layernorm(xb[0]), _layernorm(xb[1]))

    def attention(n_layers, filler, pre_rows=None, midway=()):
        n_rows = L if pre_rows is None else L - PRE_ROWS // 2
        total = n_layers * L

        def rounded(lhs):
            return lhs if total % 16 else lhs.astype(BF16)

        def project(g, which):
            if g == n_groups:
                return _run(filler, 1)
            quads = range(g * HEAD_QUADS, (g + 1) * HEAD_QUADS)
            ys = _block_matmul(
                lambda k, i: h_attn[k, i, 0:n_rows, :],
                lambda p: jnp.concatenate([wqkv[which, p, quad] for quad in quads], axis=1),
                n_layers)
            heads = []
            for (n, quad), j in itertools.product(enumerate(quads), range(QUAD)):
                parts = [_tile(y[j], n) for y in ys]
                if pre_rows is not None:
                    parts = [parts[0][:M], pre[which, quad, pre_rows, j * Dh:(j + 1) * Dh],
                             parts[0][M:L - PRE_ROWS], parts[1][:M],
                             parts[0][L - PRE_ROWS:], parts[1][M:]]
                y = jnp.concatenate(parts, axis=0)
                heads.append((rounded(y), y.T.astype(BF16), y.astype(BF16))[which])
            return heads

        def probabilities(q, k):
            s = _dot(q, k)
            b = bias[0:total, 0:total]
            s = jnp.where(b == 0.0, s * scale, b)
            e = jnp.exp(s - jnp.max(s, axis=-1, keepdims=True))
            p = e * (1.0 / jnp.sum(e, axis=-1, keepdims=True))
            return rounded(p)

        def mix(quad, probs, v):
            o = [_dot(a, b) for a, b in zip(probs, v)]
            _put_rows(attn, every, slice(quad * Dh, (quad + 1) * Dh),
                      *([y[at:at + L] for y in o] for at in range(0, total, L)))

        q, k = (project(0, which) for which in range(2))
        _run(midway, 1)
        for g in range(n_groups):
            v = project(g, 2)
            probs = [probabilities(a, b) for a, b in zip(q[:QUAD], k[:QUAD])]
            k_next = project(g + 1, 1)
            mix(2 * g, probs, v[:QUAD])
            probs = [probabilities(a, b) for a, b in zip(q[QUAD:], k[QUAD:])]
            q_next = project(g + 1, 0)
            mix(2 * g + 1, probs, v[QUAD:])
            if g:
                _run(midway, 1)
            q, k = q_next, k_next
        _run(filler)

    def project_out(src, w, n_layers, lo, hi):
        ys = _block_matmul(
            lambda k, i: src[k, i, :, lo * LANES:hi * LANES],
            lambda p: jnp.concatenate(
                [w[p, k, lo:hi].reshape((hi - lo) * LANES // 2, LANES)
                 for k in range(quarter // LANES)], axis=1),
            n_layers)
        return [jnp.concatenate(y, axis=1) for y in ys]

    def out_early(n_layers):
        for g in range(n_groups - 1):
            ys = project_out(attn, wo, n_layers, g * HEAD_QUADS, (g + 1) * HEAD_QUADS)
            for n, y in enumerate(ys):
                early[n] = early[n] + y if g else y
            yield

    def out_late(n_layers):
        ys = project_out(attn, wo, n_layers, n_hq - HEAD_QUADS, n_hq)
        return [early[n] + y for n, y in enumerate(ys)]

    def gate_up():
        for g in range(n_fq):
            ys = _block_matmul(
                lambda k, i: h_ffn[k, i],
                lambda p: jnp.concatenate([wgu[p, 0, g], wgu[p, 1, g]], axis=1), 2)
            _put_rows(act, every, slice(g * LANES, (g + 1) * LANES),
                      *([_gate(_tile(b, 0), _tile(b, 1)) for b in y] for y in ys))

    def down():
        return [xb[n] + y for n, y in enumerate(project_out(act, wd, 2, 0, n_fq))]

    def ffn():
        feed_ffn()
        gate_up()
        return down()

    def single(s, xs, xs_next, before_out=None):
        attention(1, () if before_out else out_early(1))
        feed_tokens(_layernorm(xs_next))
        if before_out:
            before_out()
        o, = project_out(attn, wo, 1, 0, n_hq) if before_out else out_late(1)
        ring[s % RING] = xs + o[M:]
        mem[...] = o[:M]
        feed_memory(o[:M])

    def out_copy(s):
        slot = s % OUT_SLOTS
        return pltpu.make_async_copy(out_v.at[slot], out_hbm.at[s], sem_out.at[slot])

    def emit(s, x):
        out_v[s % OUT_SLOTS] = x.astype(out_v.dtype)

    def tokens(s):
        return x_v[s].astype(F32)

    def fill(s, carry):
        pl.when(s == 2)(lambda: start(wd_copies))
        single(s, tokens(s), tokens(s + 1))
        return carry

    def prepare_wo():
        start(wg_copies)
        wait(wo_copies)
        start(wu_copies)
        form_operands(wo, wo_v)

    x_head.wait()
    feed_memory(mem0)
    feed_tokens(_layernorm(tokens(0)))
    single(0, tokens(0), tokens(1), prepare_wo)
    lax.fori_loop(1, LAG, fill, 0)
    feed_memory(mem[...], mem0)
    xb[0], xb[1] = ring[0], ring[1]
    wait(wg_copies)
    wait(wu_copies)
    form_operands(wgu, wgu_v)
    wait(wd_copies)
    x_tail.start()
    form_operands(wd, wd_v)
    ring[0], ring[1] = ffn()
    xb[0], xb[1] = ring[3], ring[2]
    x_tail.wait()
    feed_both(LAG, True)

    def step(t, carry, *, use_pre):
        s = t - LAG - 1

        def gated():
            gate_up()
            yield
            ring[(t - 1) % RING], x2 = down()
            ring[jnp.where(t == LAG, LAG - 2, RING)] = x2
            emit(jnp.maximum(s, 0), x2)

        pre_rows = None
        if use_pre:
            pre_rows = pl.ds(pl.multiple_of((t - LAG) * PRE_ROWS, PRE_ROWS), PRE_ROWS)
        feed_ffn()
        attention(2, out_early(2), pre_rows, gated())
        feed_both(t + 1, use_pre)
        o1, o2 = out_late(2)
        mem[...] = o2[:M]
        feed_memory(o1[:M], o2[:M])
        xb[0], xb[1] = tokens(t) + o1[M:], ring[(t - LAG) % RING] + o2[M:]
        pl.when(not use_pre or s >= 0)(lambda: out_copy(s).start())
        pl.when(not use_pre or s + 1 >= OUT_SLOTS)(lambda: out_copy(s + 1 - OUT_SLOTS).wait())
        return carry

    lax.fori_loop(LAG, LAG + PRE_STEPS, functools.partial(step, use_pre=True), 0)
    feed_both(LAG + PRE_STEPS, False)
    lax.fori_loop(LAG + PRE_STEPS, n_seg, functools.partial(step, use_pre=False), 0)

    tail = n_seg - LAG

    def drain(s, carry):
        single(s, ring[s % RING], ring[(s + 1) % RING])
        return carry

    def drain_ffn(n, carry):
        s = tail + 2 * n - 2

        @pl.when(n == 1)
        def _():
            ring[(n_seg - 1) % RING] = early[0, :seg]
            feed_memory(mem[...])
            feed_tokens(_layernorm(ring[tail % RING]))
            lax.fori_loop(tail, n_seg, drain, 0)
            wait([out_copy(k) for k in range(tail - OUT_SLOTS, tail)])

        @pl.when(n >= 1)
        def _():
            xb[0], xb[1] = ring[s % RING], ring[(s + 1) % RING]

        x1, x2 = ffn()
        early[0, :seg] = x1
        emit(s + 1, x2)

        @pl.when(n >= 1)
        def _():
            emit(s, x1)
            out_copy(s).start()

        out_copy(s + 1).start()
        return carry

    lax.fori_loop(0, 1 + LAG // 2, drain_ffn, 0)
    wait([out_copy(s) for s in range(tail, n_seg)])


@functools.partial(jax.jit, static_argnames=("A_seg_len",))
def pallas_interleave_layers__memory_aug_recurrent_mem_tr__glu_gated_glu__prompt_kernel(
    A_x, A_mem0, A_Wq, A_Wk, A_Wv, A_Wo, A_seg_len, B_x, B_w_gate, B_w_up, B_w_down,
):
    del B_x
    B, S, D = A_x.shape
    M = A_mem0.shape[1]
    _, H, Dh = A_Wq.shape
    F = B_w_gate.shape[1]
    seg = int(A_seg_len)
    assert B == 1 and S % seg == 0 and Dh == LANES
    L, quarter, n_pre = M + seg, D // QUAD, PRE_STEPS * PRE_ROWS
    n_hq, n_fq = H // QUAD, F // (QUAD * LANES)
    hbm = pl.BlockSpec(memory_space=pl.ANY)
    staged = [w.reshape(QUAD, quarter // RAW_ROWS, RAW_ROWS * H, Dh) for w in (A_Wq, A_Wk, A_Wv)]
    out = pl.pallas_call(
        _kernel,
        out_shape=jax.ShapeDtypeStruct((S // seg, seg, D), A_x.dtype),
        in_specs=[hbm, pl.BlockSpec(memory_space=pltpu.VMEM)] + [hbm] * 7,
        out_specs=hbm,
        scratch_shapes=[
            pltpu.VMEM((S // seg, seg, D), BF16),
            pltpu.VMEM((PRE_STEPS, PRE_ROWS, D), BF16),
            pltpu.VMEM((OUT_SLOTS, seg, D), A_x.dtype),
            pltpu.VMEM((RAW_SLOTS, QUAD, RAW_ROWS * H + 6 * RAW_PAD, Dh), BF16),
            pltpu.VMEM((3, N_SLOTS, n_hq, quarter // 2, Dh), U32),
            pltpu.VMEM((N_SLOTS, quarter // LANES, n_hq, Dh, LANES), BF16),
            pltpu.VMEM((N_SLOTS, 2, n_fq, quarter, LANES), BF16),
            pltpu.VMEM((N_SLOTS, quarter // LANES, n_fq, LANES, LANES), BF16),
            pltpu.VMEM((2, QUAD, L, quarter), F32),
            pltpu.VMEM((2, QUAD, L, n_hq * Dh), F32),
            pltpu.VMEM((2, QUAD, seg, quarter), F32),
            pltpu.VMEM((2, QUAD, seg, n_fq * LANES), F32),
            pltpu.VMEM((2, L, D), F32),
            pltpu.VMEM((M, D), F32),
            pltpu.VMEM((2, seg, D), F32),
            pltpu.VMEM((RING + 1, seg, D), F32),
            pltpu.VMEM((2 * L, 2 * L), F32),
            pltpu.VMEM((quarter // RAW_ROWS, n_pre // 2, QUAD * RAW_ROWS), U32),
            pltpu.VMEM((3, n_hq, n_pre, QUAD * Dh), F32),
            pltpu.SemaphoreType.DMA((3,)),
            pltpu.SemaphoreType.DMA((RAW_SLOTS,)),
            pltpu.SemaphoreType.DMA((4,)),
            pltpu.SemaphoreType.DMA((OUT_SLOTS,)),
        ],
        compiler_params=pltpu.CompilerParams(vmem_limit_bytes=120 * 2**20),
    )(A_x.reshape(S // seg, seg, D), A_mem0.reshape(M, D), *staged,
      A_Wo.reshape(n_hq, QUAD, Dh, D), B_w_gate.reshape(QUAD, quarter, F),
      B_w_up.reshape(QUAD, quarter, F), B_w_down.reshape(n_fq, QUAD, LANES, D))
    return out.reshape(B, S, D)
```
